```python
import os as _os
_os.environ.setdefault('JAX_PLATFORMS', 'cpu')
import jax
import jax.numpy as jnp

def _softmax(x, axis=-1):
    return jax.nn.softmax(x, axis=axis)

def _gelu(x):
    return jax.nn.gelu(x, approximate=True)

def _silu(x):
    return jax.nn.silu(x)

def _sigmoid(x):
    return jax.nn.sigmoid(x)

def _layernorm(x, axis=-1, eps=1e-05):
    m = jnp.mean(x, axis=axis, keepdims=True)
    v = jnp.var(x, axis=axis, keepdims=True)
    return (x - m) / jnp.sqrt(v + eps)

def _scatter_add(tgt, idx, src, axis=0):
    return tgt.at[idx].add(src)

def _segment_sum(src, seg, n):
    return jax.ops.segment_sum(src, seg, n)

class _Rng:

    def __init__(self, key):
        self._k = key

    def _next(self):
        self._k, sub = jax.random.split(self._k)
        return sub

    def normal(self, shape):
        return jax.random.normal(self._next(), shape, dtype=jnp.bfloat16)

    def randint(self, lo, hi, shape):
        return jax.random.randint(self._next(), shape, lo, hi, dtype=jnp.int32)

    def uniform(self, shape, lo=0.0, hi=1.0):
        return jax.random.uniform(self._next(), shape, jnp.bfloat16, lo, hi)

    def permutation(self, n):
        return jax.random.permutation(self._next(), n)
kernel_name = 'standalone__conformer_family_e_branchformer__speech'

def setup_inputs():
    _rng = _Rng(jax.random.key(int.from_bytes(__import__("os").urandom(4), "little")))
    _w = lambda a: (lambda t: t.astype(jnp.bfloat16) if jnp.issubdtype(t.dtype, jnp.floating) else t)(jnp.asarray(a))
    B, T, D, K = (2, 4000, 256, 31)
    return {'x': _w((lambda *s: _rng.normal(s) * 0.05)(B, T, D)), 'w_qkv': _w((lambda *s: _rng.normal(s) * 0.05)(D, 3 * D)), 'w_att_out': _w((lambda *s: _rng.normal(s) * 0.05)(D, D)), 'w_mlp_in': _w((lambda *s: _rng.normal(s) * 0.05)(D, 2 * D)), 'dw_csgu': _w((lambda *s: _rng.normal(s) * 0.05)(K, D)), 'w_mlp_out': _w((lambda *s: _rng.normal(s) * 0.05)(D, D)), 'dw_merge': _w((lambda *s: _rng.normal(s) * 0.05)(K, 2 * D)), 'w_merge': _w((lambda *s: _rng.normal(s) * 0.05)(2 * D, D))}

def reference(x, w_qkv, w_att_out, w_mlp_in, dw_csgu, w_mlp_out, dw_merge, w_merge):
    B, T, D = x.shape
    K = dw_csgu.shape[0]
    pad = K // 2
    xa = _layernorm(x, axis=-1)
    qkv = jnp.einsum('btd,de->bte', xa, w_qkv)
    q, k, v = (qkv[..., :D].copy(), qkv[..., D:2 * D].copy(), qkv[..., 2 * D:].copy())
    scores = jnp.einsum('btd,bsd->bts', q, k) * D ** (-0.5)
    p = _softmax(scores, axis=-1)
    attn = jnp.einsum('bts,bsd->btd', p, v)
    glob = jnp.einsum('btd,de->bte', attn, w_att_out)
    xc = _layernorm(x, axis=-1)
    h = _gelu(jnp.einsum('btd,de->bte', xc, w_mlp_in))
    u, g = (h[..., :D].copy(), h[..., D:].copy())
    g = _layernorm(g, axis=-1)
    gp = jnp.pad(g, ((0, 0), (pad, pad), (0, 0)))
    gc = jnp.zeros_like(g)
    for i in range(K):
        gc = gc + gp[:, i:i + T, :] * dw_csgu[i][None, None, :]
    loc = jnp.einsum('btd,de->bte', u * gc, w_mlp_out)
    m = jnp.concatenate([glob, loc], axis=-1)
    mp = jnp.pad(m, ((0, 0), (pad, pad), (0, 0)))
    mc = jnp.zeros_like(m)
    for i in range(K):
        mc = mc + mp[:, i:i + T, :] * dw_merge[i][None, None, :]
    m = m + mc
    return x + jnp.einsum('btc,cd->btd', m, w_merge)
```

```python
import functools
NITER = 18
SKIP = ''
STOP = ''
CV = 10
import jax
import jax.numpy as jnp
from jax import lax
import jax.experimental.pallas as pl
import jax.experimental.pallas.tpu as pltpu

F32 = jnp.float32
BF16 = jnp.bfloat16
U32 = jnp.uint32
LOG2E = 1.4426950408889634
NT_DIMS = (((1,), (1,)), ((), ()))
SLOT = 448
LAG = 16


def _pk(x):
    return pltpu.bitcast(x, U32)


def _upk(x):
    return pltpu.bitcast(x, BF16)


def _ln(x, eps=1e-5):
    m = jnp.mean(x, axis=-1, keepdims=True)
    xc = x - m
    v = jnp.mean(xc * xc, axis=-1, keepdims=True)
    return xc * lax.rsqrt(v + eps)


def _gelu(x):
    c = 0.7978845608028654
    hx = 0.5 * x
    return hx + hx * jnp.tanh(x * (c + (c * 0.044715) * (x * x)))


def _ds(base, off, n, align):
    if isinstance(base, int):
        return pl.ds(base + off, n)
    a = align
    while off % a:
        a //= 2
    return pl.ds(pl.multiple_of(base + off, a), n) if a > 1 else pl.ds(base + off, n)


def _conv(buf_ref, g, w_ref, wg, base, off, nrows, K):
    outs = []
    nv = nrows // 8
    v0 = 0
    while v0 < nv:
        V = min(CV, nv - v0)
        acc = None
        for p in range(8):
            taps = list(range(p, K, 8))
            nq = V + len(taps) - 1
            slab = buf_ref[g, _ds(base, off + 8 * v0 + p - K // 2, 8 * nq, 32), :].reshape(nq, 8, 128)
            for qi, i in enumerate(taps):
                term = slab[qi:qi + V] * w_ref[wg, i][None]
                acc = term if acc is None else acc + term
        outs.append(acc.reshape(8 * V, 128))
        v0 += V
    return jnp.concatenate(outs, axis=0) if len(outs) > 1 else outs[0]


class Tile:
    def __init__(self, t, NT, NS, TQ, TP, T):
        if isinstance(t, int):
            b = t // NT
            first, last = t % NT == 0, t % NT == NT - 1
            self.prev = (NS if first else t - 1) * SLOT
            self.next = (NS if last else t + 1) * SLOT
        else:
            b = (t >= NT).astype(jnp.int32)
            first = jnp.logical_or(t == 0, t == NT)
            last = jnp.logical_or(t == NT - 1, t == NS - 1)
            self.prev = jnp.where(first, NS, t - 1) * SLOT
            self.next = jnp.where(last, NS, t + 1) * SLOT
        self.cb = t * SLOT
        self.fb = t * TQ
        self.ab = t * (TQ // 2) + b * ((TP - T) // 2)
        self.kb = b * (TP // 2)


def kernel(x_hbm, wqkv_hbm, wao_hbm, wmi_hbm, dwc_hbm, wmo_hbm, dwm_hbm, wm_hbm, o_hbm,
           x_buf, o_buf, xa_ref, wa_p, wvo_p, wmi_p, wmo_p, wm_p, dw_f, g_buf, m_buf, u_ref,
           s_ref, mx_ref, q_ref, mp_ref, lp_ref, acc_ref, y_ref,
           wqkv_ref, wao_ref, wmi_ref, dwc_ref, wmo_ref, dwm_ref, wm_ref,
           zoff, sem_x, sem_w, sem_out,
           *, B, T, D, K, TQ, TP, CK):
    NT = T // TQ
    NS = B * NT
    G = D // 128
    NC = TP // CK
    LT = CK // 128
    assert B == 2
    last = [None]
    JUNK = NS * SLOT + 64

    def tile(t):
        return Tile(t, NT, NS, TQ, TP, T)

    def x_copy(t):
        n = TQ if t <= NT else B * T - t * TQ
        return pltpu.make_async_copy(x_hbm.at[pl.ds(t * TQ, n), :], x_buf.at[pl.ds(LAG + t * TQ, n), :], sem_x.at[t])

    w_pairs = [(wqkv_hbm.at[:, 0:2 * D], wqkv_ref.at[:, 0:2 * D]), (wmi_hbm, wmi_ref), (wao_hbm, wao_ref), (dwc_hbm, dwc_ref),
               (wmo_hbm, wmo_ref), (dwm_hbm, dwm_ref), (wm_hbm, wm_ref), (wqkv_hbm.at[:, 2 * D:3 * D], wqkv_ref.at[:, 2 * D:3 * D])]

    def w_copy(k):
        return pltpu.make_async_copy(w_pairs[k][0], w_pairs[k][1], sem_w.at[k])

    def dma_start(op):
        if op[1] == 'x':
            x_copy(int(op[2:])).start()
        elif op == 'swr':
            for k in range(2, len(w_pairs)):
                w_copy(k).start()
        else:
            w_copy(int(op[2:])).start()

    PRO = 'sx0 sw0 sx1 | x0 n0 w0 x1 sx2 sw1 sx3 A n1 q K K K x2 w1 x3 sx4 sx5 sx6 sx7 sw3 sw4 p1 n2 n3 H0 H1 K x4 x5 x6 x7 w3 w4 sx8 sx9 sw2 sw5 sw6 sw7 sx10 p3 p4 K Zg n4 n5 n6 n7 K K K K K K L0 x8 x9 w2 w5 w6 w7 x10 sx11 n8 n9 p5 p6 K p2 K K K K'.split()
    for op in PRO[:PRO.index('|')]:
        dma_start(op)
    PRO = PRO[PRO.index('|') + 1:]

    zoff[0] = 0
    z16 = jnp.zeros((16, 128), F32)
    for b in range(B):
        for gi in range(G):
            g_buf[gi, b * NT * SLOT:b * NT * SLOT + 16, :] = z16
            g_buf[gi, ((b + 1) * NT - 1) * SLOT + 416:((b + 1) * NT - 1) * SLOT + 432, :] = z16
        for gi in range(2 * G):
            m_buf[gi, b * NT * SLOT:b * NT * SLOT + 16, :] = z16
            m_buf[gi, b * NT * SLOT + 16:b * NT * SLOT + 32, :] = z16
            m_buf[gi, ((b + 1) * NT - 1) * SLOT + 432:((b + 1) * NT - 1) * SLOT + 448, :] = z16
        xa_ref[b * TP // 2 + T // 2:(b + 1) * TP // 2, :] = jnp.zeros(((TP - T) // 2, D), U32)
    x_buf[0:LAG, :] = jnp.zeros((LAG, D), BF16)

    def prep_a():
        a = lax.dot_general(wqkv_ref[:, 0:D], wqkv_ref[:, D:2 * D], NT_DIMS, preferred_element_type=F32)
        wa_p[...] = _pk((a * (D ** -0.5 * LOG2E)).astype(BF16))

    def prep(k):
        if k == 1:
            wmi_p[...] = _pk(wmi_ref[...])
        elif k == 2:
            wvo_p[...] = _pk(jnp.dot(wqkv_ref[:, 2 * D:3 * D], wao_ref[...], preferred_element_type=F32).astype(BF16))
        elif k == 4:
            wmo_p[...] = _pk(wmo_ref[...])
        elif k == 6:
            wm_p[...] = _pk(wm_ref[...])
        elif k in (3, 5):
            dw = (dwc_ref if k == 3 else dwm_ref)[...].astype(F32)
            g0 = 2 * G if k == 3 else 0
            for gi in range(dw.shape[1] // 128):
                for i in range(K):
                    dw_f[g0 + gi, i] = jnp.broadcast_to(dw[i:i + 1, gi * 128:(gi + 1) * 128], (8, 128))

    def ln_tile(t):
        return _pk(_ln(x_buf[_ds(t.fb, LAG, TQ, 16), :].astype(F32)).astype(BF16))

    def ln_store(t, xa):
        xa_ref[_ds(t.ab, 0, TQ // 2, 8), :] = xa

    def xq_of(t):
        return _upk(xa_ref[_ds(t.ab, 0, TQ // 2, 8), :])

    def xa_chunk(t, j):
        return _upk(xa_ref[_ds(t.kb, j * CK // 2, CK // 2, 16), :])

    def qproj(t):
        qf = jnp.dot(xq_of(t), _upk(wa_p[...]), preferred_element_type=F32)
        last[0] = qf[0:16, 0:128]
        q_ref[0:TQ // 2, :] = _pk(qf.astype(BF16))

    def l1(t):
        h = _gelu(jnp.dot(xq_of(t), _upk(wmi_p[...]), preferred_element_type=F32))
        u_ref[_ds(t.fb, 0, TQ, 16), :] = h[:, :D]
        g = _ln(h[:, D:])
        for gi in range(G):
            g_buf[gi, _ds(t.prev, 16 + TQ, 16, 32), :] = g[0:16, gi * 128:(gi + 1) * 128]
        for gi in range(G):
            g_buf[gi, _ds(t.cb, 16, TQ, 32), :] = g[:, gi * 128:(gi + 1) * 128]
        for gi in range(G):
            g_buf[gi, _ds(t.next, 0, 16, 32), :] = g[TQ - 16:TQ, gi * 128:(gi + 1) * 128]

    def m_store(t, g0, v):
        for gi in range(G):
            m_buf[g0 + gi, _ds(t.cb, 32, TQ, 32), :] = v[:, gi * 128:(gi + 1) * 128]
        for gi in range(G):
            m_buf[g0 + gi, _ds(t.next, 0, 32, 32), :] = v[TQ - 32:TQ, gi * 128:(gi + 1) * 128]

    def l2(t):
        gc = jnp.concatenate([_conv(g_buf, gi, dw_f, 2 * G + gi, t.cb, 16, TQ, K) for gi in range(G)], axis=-1)
        u = u_ref[_ds(t.fb, 0, TQ, 16), :]
        loc = jnp.dot((u * gc).astype(BF16), _upk(wmo_p[...]), preferred_element_type=F32)
        m_store(t, G, loc)

    def merge_half(half, pieces):
        lhs = []
        for (t, off, nrows, yo) in pieces:
            r = 32 - LAG + off
            ms = [m_buf[gi, _ds(t.cb, r, nrows, 32), :] + _conv(m_buf, gi, dw_f, gi, t.cb, r, nrows, K)
                  for gi in range(half * G, (half + 1) * G)]
            lhs.append(jnp.concatenate(ms, axis=-1))
        lhs = lhs[0] if len(lhs) == 1 else jnp.concatenate(lhs, axis=0)
        return jnp.dot(lhs.astype(BF16), _upk(wm_p[half * D // 2:(half + 1) * D // 2, :]), preferred_element_type=F32)

    def merge_a(pieces):
        y = merge_half(1, pieces)
        r = 0
        for (t, off, nrows, yo) in pieces:
            y_ref[yo:yo + nrows, :] = x_buf[_ds(t.fb, off, nrows, 16), :].astype(F32) + y[r:r + nrows]
            r += nrows

    def merge_b(pieces):
        y = merge_half(0, pieces)
        r = 0
        for (t, off, nrows, yo) in pieces:
            o_buf[_ds(t.fb, off, nrows, 16), :] = (y_ref[yo:yo + nrows, :] + y[r:r + nrows]).astype(BF16)
            r += nrows

    def p1_chunk(t, j):
        sj = lax.dot_general(_upk(q_ref[0:TQ // 2, :]), xa_chunk(t, j), NT_DIMS, preferred_element_type=F32)
        last[0] = sj[0:16, 0:128]
        mloc = None
        for lt in range(LT):
            c0 = j * CK + lt * 128
            st = sj[:, lt * 128:(lt + 1) * 128]
            if c0 + 128 > T:
                col = lax.broadcasted_iota(jnp.int32, (TQ, 128), 1)
                st = jnp.where(col < T - c0, st, -1e30)
            s_ref[:, c0:c0 + 128] = st
            mloc = st if mloc is None else jnp.maximum(mloc, st)
        if j == 0:
            mp_ref[0:TQ] = mloc
        elif j < NC - 1:
            mp_ref[0:TQ] = jnp.maximum(mp_ref[0:TQ], mloc)
        else:
            return jnp.maximum(mp_ref[0:TQ], mloc)

    def p1_fin(mpart):
        m = jnp.max(mpart, axis=-1, keepdims=True)
        mx_ref[0:TQ] = jnp.broadcast_to(m, (TQ, 128))

    def p2_chunk(t, j):
        ps = []
        lloc = None
        for lt in range(LT):
            c0 = j * CK + lt * 128
            p = jnp.exp2(s_ref[:, c0:c0 + 128] - mx_ref[0:TQ])
            lloc = p if lloc is None else lloc + p
            ps.append(p)
        pv = jnp.dot(jnp.concatenate(ps, axis=-1).astype(BF16), xa_chunk(t, j), preferred_element_type=F32)
        last[0] = pv[0:16, 0:128]
        if j == 0:
            lp_ref[0:TQ] = lloc
            acc_ref[...] = pv
        else:
            lp_ref[0:TQ] += lloc
            acc_ref[...] += pv

    def p2_fin(t):
        l = jnp.sum(lp_ref[0:TQ], axis=-1, keepdims=True)
        o = (acc_ref[...] * (1.0 / l)).astype(BF16)
        glob = jnp.dot(o, _upk(wvo_p[...]), preferred_element_type=F32)
        m_store(t, 0, glob)

    def anchor(buf):
        zrow = pl.multiple_of(zoff[0], 8)
        buf[0, pl.ds(zrow + JUNK, 8), :] = last[0][0:8]

    def anchor_x():
        zrow = pl.multiple_of(zoff[0], 16)
        x_buf[pl.ds(zrow + B * T + LAG, 16), 0:128] = last[0].astype(BF16)

    def out_copy(base, off, n):
        return pltpu.make_async_copy(o_buf.at[_ds(base, off, n, 16), :], o_hbm.at[_ds(base, off - LAG, n, 16), :], sem_out)

    DEF = 'q Z H V V V K V K V K V K Mb V K V K V K V K Ma V K V K V K V K L Zx V K V K N K K G'
    ORDER = DEF.split()
    ORDERP = 'q Z Zg V V V K V K V K V K V K Mb V K V K V K V K Ma V K V K V K V K L V K K K G'.split()
    ORDERL = 'V Z V V V V V V V V V Mb V V V V V V Ma G'.split()

    def step(order, pb, pa, t0, tp, th, tn):
        assert order.count('V') == NC and (tp is None or order.count('K') == NC)
        mpart = None
        jv = jk = 0
        for op in order:
            if op in SKIP.split(','):
                continue
            if op == 'q':
                qproj(tp)
            elif op == 'V':
                p2_chunk(t0, jv)
                jv += 1
            elif op == 'K':
                assert jk < jv
                mpart = p1_chunk(tp, jk)
                jk += 1
            elif op == 'Z':
                anchor(m_buf)
            elif op == 'Zg':
                anchor(g_buf)
            elif op == 'Zx':
                anchor_x()
            elif op == 'Ma':
                merge_a(pa)
            elif op == 'Mb':
                merge_b(pb)
            elif op == 'H':
                l1(th)
            elif op == 'L':
                l2(tp)
            elif op == 'N':
                ln_store(tn, ln_tile(tn))
            elif op == 'G':
                p2_fin(t0)
            else:
                raise ValueError(op)
        if tp is not None:
            p1_fin(mpart)

    def do_ln(t):
        ln_store(tile(t), ln_tile(tile(t)))

    jk = 0
    nln = 0
    for op in PRO:
        if op == 'STOP':
            return
        if op[0] == 's':
            dma_start(op)
        elif op[0] == 'x':
            x_copy(int(op[1:])).wait()
        elif op[0] == 'n':
            do_ln(int(op[1:]))
            nln = int(op[1:]) + 1
        elif op[0] == 'w':
            w_copy(int(op[1:])).wait()
        elif op[0] == 'p':
            prep(int(op[1:]))
        elif op == 'A':
            prep_a()
        elif op == 'q':
            qproj(tile(0))
        elif op == 'K':
            assert nln * TQ >= min((jk + 1) * CK, T)
            mpart = p1_chunk(tile(0), jk)
            jk += 1
        elif op[0] == 'H':
            l1(tile(int(op[1:])))
        elif op == 'L0':
            l2(tile(0))
        elif op == 'Zg':
            anchor(g_buf)
        elif op == 'Zx':
            anchor_x()
        else:
            raise ValueError(op)
    assert jk == NC
    p1_fin(mpart)
    if STOP == 'pro':
        x_copy(NT + 1).wait()
        return

    def body(s, c):
        @pl.when(s == 1)
        def _():
            x_copy(NT + 1).wait()

        w = jnp.maximum(s - 1, 0)
        step(ORDER, [(tile(w), 0, TQ, 0)], [(tile(s), 0, TQ, 0)], tile(s), tile(s + 1), tile(s + 2),
             tile(jnp.minimum(s + NT, NS - 1)))
        fb = w * TQ

        @pl.when(s > 0)
        def _():
            out_copy(fb, LAG, TQ - LAG).start()

        @pl.when(jnp.logical_and(s > 1, s != NT + 1))
        def _():
            out_copy(fb, 0, LAG).start()
        return c
    lax.fori_loop(0, NITER, body, 0)

    z = zoff[0]
    t9 = tile(NT - 1)

    @pl.when(z == 0)
    def _():
        dyn = (lambda t: tile(z + t)) if '1' == '1' else tile
        step(ORDERP, [(dyn(NS - 3), 0, TQ, 0)], [(dyn(NS - 2), 0, TQ, 0), (t9, TQ, LAG, TQ + LAG)],
             dyn(NS - 2), dyn(NS - 1), None, None)
        out_copy(0, (NS - 3) * TQ, TQ).start()

    @pl.when(z < 1)
    def _():
        tl = tile(NS - 1)
        step(ORDERL, [(tile(NS - 2), 0, TQ, 0), (t9, TQ, LAG, TQ + LAG)], [(tl, 0, TQ + LAG, 0)], tl, None, None, None)
        out_copy(0, (NS - 2) * TQ, TQ).start()
        out_copy(0, NT * TQ, LAG).start()
        merge_b([(tl, 0, TQ + LAG, 0)])
        out_copy(0, (NS - 1) * TQ, TQ + LAG).start()

    for s in range(1, NITER):
        out_copy(0, LAG, TQ - LAG).wait()
        if s != 1 and s != NT + 1:
            out_copy(0, LAG, LAG).wait()
    out_copy(0, (NS - 3) * TQ, TQ).wait()
    out_copy(0, (NS - 2) * TQ, TQ).wait()
    out_copy(0, (NS - 1) * TQ, TQ + LAG).wait()
    out_copy(0, NT * TQ, LAG).wait()


@jax.jit
def pallas_standalone__conformer_family_e_branchformer__speech_kernel(
    x, w_qkv, w_att_out, w_mlp_in, dw_csgu, w_mlp_out, dw_merge, w_merge):
    B, T, D = x.shape
    K = dw_csgu.shape[0]
    TQ = 400
    TP = 4096
    CK = 256
    G = D // 128
    NT = T // TQ
    RB = (B * NT + 1) * SLOT
    out = pl.pallas_call(
        functools.partial(kernel, B=B, T=T, D=D, K=K, TQ=TQ, TP=TP, CK=CK),
        in_specs=[pl.BlockSpec(memory_space=pl.ANY)] * 8,
        out_specs=pl.BlockSpec(memory_space=pl.ANY),
        out_shape=jax.ShapeDtypeStruct((B * T, D), x.dtype),
        scratch_shapes=[
            pltpu.VMEM((B * T + 32, D), BF16),
            pltpu.VMEM((B * T + 32, D), BF16),
            pltpu.VMEM((B * TP // 2, D), U32),
            pltpu.VMEM((D // 2, D), U32),
            pltpu.VMEM((D // 2, D), U32),
            pltpu.VMEM((D // 2, 2 * D), U32),
            pltpu.VMEM((D // 2, D), U32),
            pltpu.VMEM((D, D), U32),
            pltpu.VMEM((3 * G, 32, 8, 128), F32),
            pltpu.VMEM((G, RB, 128), F32),
            pltpu.VMEM((2 * G, RB, 128), F32),
            pltpu.VMEM((B * T, D), F32),
            pltpu.VMEM((TQ, TP), F32),
            pltpu.VMEM((TQ + 16, 128), F32),
            pltpu.VMEM((TQ // 2 + 8, D), U32),
            pltpu.VMEM((TQ + 16, 128), F32),
            pltpu.VMEM((TQ + 16, 128), F32),
            pltpu.VMEM((TQ, D), F32),
            pltpu.VMEM((TQ + 2 * LAG, D), F32),
            pltpu.VMEM(w_qkv.shape, BF16),
            pltpu.VMEM(w_att_out.shape, BF16),
            pltpu.VMEM(w_mlp_in.shape, BF16),
            pltpu.VMEM(dw_csgu.shape, BF16),
            pltpu.VMEM(w_mlp_out.shape, BF16),
            pltpu.VMEM(dw_merge.shape, BF16),
            pltpu.VMEM(w_merge.shape, BF16),
            pltpu.SMEM((1,), jnp.int32),
            pltpu.SemaphoreType.DMA((NT + 2,)),
            pltpu.SemaphoreType.DMA((8,)),
            pltpu.SemaphoreType.DMA,
        ],
        compiler_params=pltpu.CompilerParams(vmem_limit_bytes=110 * 1024 * 1024),
    )(x.reshape(B * T, D), w_qkv, w_att_out, w_mlp_in, dw_csgu, w_mlp_out, dw_merge, w_merge)
    return out.reshape(B, T, D)
```

```python
import functools
NITER = 18
SKIP = ''
STOP = ''
CV = 10
RSQ = 1
REM = 2
import jax
import jax.numpy as jnp
from jax import lax
import jax.experimental.pallas as pl
import jax.experimental.pallas.tpu as pltpu

F32 = jnp.float32
BF16 = jnp.bfloat16
U32 = jnp.uint32
LOG2E = 1.4426950408889634
NT_DIMS = (((1,), (1,)), ((), ()))
SLOT = 448
LAG = 16

PRO0 = 'sx0 sw0 sx1 | x0 sx2 sw1 sx3 n0 w0 x1 sx4 sx5 A n1 q K K K x2 w1 x3 sx6 sx7 sw3 sw4 sx8 sx9 p1 n2 n3 H0 H1 K x4 x5 x6 x7 w3 w4 sw2 sw5 sw6 sw7 sx10 p3 p4 K Zg n4 n5 n6 n7 K K K K K K L0 x8 x9 w2 w5 w6 w7 x10 sx11 n8 n9 p5 p6 K K K K K p2 n10'.split()
GRP = {}
_g, _prev = -1, False
for _op in PRO0:
    _is_wait = _op[0] in 'xw'
    if _is_wait:
        if not _prev:
            _g += 1
        GRP[_op] = _g
    _prev = _is_wait
GRP['x11'] = _g + 1


def _pk(x):
    return pltpu.bitcast(x, U32)


def _upk(x):
    return pltpu.bitcast(x, BF16)


def _ln(x, eps=1e-5):
    m = jnp.mean(x, axis=-1, keepdims=True)
    xc = x - m
    v = jnp.mean(xc * xc, axis=-1, keepdims=True)
    if RSQ == 0:
        return xc * lax.rsqrt(v + eps)
    return xc * jnp.exp2(jnp.log(v + eps) * (-0.5 * LOG2E))


def _gelu(x):
    c = 0.7978845608028654
    hx = 0.5 * x
    return hx + hx * jnp.tanh(x * (c + (c * 0.044715) * (x * x)))


def _ds(base, off, n, align):
    if isinstance(base, int):
        return pl.ds(base + off, n)
    a = align
    while off % a:
        a //= 2
    return pl.ds(pl.multiple_of(base + off, a), n) if a > 1 else pl.ds(base + off, n)


def _conv(buf_ref, g, w_ref, wg, base, off, nrows, K):
    outs = []
    nv = nrows // 8
    v0 = 0
    while v0 < nv:
        V = min(CV, nv - v0)
        acc = None
        for p in range(8):
            taps = list(range(p, K, 8))
            nq = V + len(taps) - 1
            slab = buf_ref[g, _ds(base, off + 8 * v0 + p - K // 2, 8 * nq, 32), :].reshape(nq, 8, 128)
            for qi, i in enumerate(taps):
                term = slab[qi:qi + V] * w_ref[wg, i][None]
                acc = term if acc is None else acc + term
        outs.append(acc.reshape(8 * V, 128))
        v0 += V
    return jnp.concatenate(outs, axis=0) if len(outs) > 1 else outs[0]


class Tile:
    def __init__(self, t, NT, NS, TQ, TP, T):
        if isinstance(t, int):
            b = t // NT
            first, last = t % NT == 0, t % NT == NT - 1
            self.prev = (NS if first else t - 1) * SLOT
            self.next = (NS if last else t + 1) * SLOT
        else:
            b = (t >= NT).astype(jnp.int32)
            first = jnp.logical_or(t == 0, t == NT)
            last = jnp.logical_or(t == NT - 1, t == NS - 1)
            self.prev = jnp.where(first, NS, t - 1) * SLOT
            self.next = jnp.where(last, NS, t + 1) * SLOT
        self.cb = t * SLOT
        self.fb = t * TQ
        self.ab = t * (TQ // 2) + b * ((TP - T) // 2)
        self.kb = b * (TP // 2)


def kernel(x_hbm, wqkv_hbm, wao_hbm, wmi_hbm, dwc_hbm, wmo_hbm, dwm_hbm, wm_hbm, o_hbm,
           x_buf, o_buf, xa_ref, wa_p, wvo_p, wmi_p, wmo_p, wm_p, dw_f, g_buf, m_buf, u_ref,
           s_ref, mx_ref, q_ref, mp_ref, lp_ref, acc_ref, y_ref,
           wqkv_ref, wao_ref, wmi_ref, dwc_ref, wmo_ref, dwm_ref, wm_ref,
           zoff, sem_in, sem_out,
           *, B, T, D, K, TQ, TP, CK):
    NT = T // TQ
    NS = B * NT
    G = D // 128
    NC = TP // CK
    LT = CK // 128
    assert B == 2
    last = [None]
    last_e = [None]
    JUNK = NS * SLOT + 64

    def tile(t):
        return Tile(t, NT, NS, TQ, TP, T)

    def x_copy(t):
        r0 = t * TQ if t <= NT else (NT + 2) * TQ
        n = TQ if t < NT else (2 * TQ if t == NT else B * T - r0)
        return pltpu.make_async_copy(x_hbm.at[pl.ds(r0, n), :], x_buf.at[pl.ds(LAG + r0, n), :], sem_in.at[GRP['x%d' % t]])

    w_pairs = [(wqkv_hbm.at[:, 0:2 * D], wqkv_ref.at[:, 0:2 * D]), (wmi_hbm, wmi_ref), (wao_hbm, wao_ref), (dwc_hbm, dwc_ref),
               (wmo_hbm, wmo_ref), (dwm_hbm, dwm_ref), (wm_hbm, wm_ref), (wqkv_hbm.at[:, 2 * D:3 * D], wqkv_ref.at[:, 2 * D:3 * D])]

    def w_copy(k):
        return pltpu.make_async_copy(w_pairs[k][0], w_pairs[k][1], sem_in.at[GRP['w%d' % k]])

    def dma_start(op):
        if STOP == 'pro' and op == 'sx11':
            return
        if op[1] == 'x':
            x_copy(int(op[2:])).start()
        elif op == 'swr':
            for k in range(2, len(w_pairs)):
                w_copy(k).start()
        else:
            w_copy(int(op[2:])).start()

    PRO = list(PRO0)
    for op in PRO[:PRO.index('|')]:
        dma_start(op)
    PRO = PRO[PRO.index('|') + 1:]

    zoff[0] = 0
    z16 = jnp.zeros((16, 128), F32)
    for b in range(B):
        for gi in range(G):
            g_buf[gi, b * NT * SLOT:b * NT * SLOT + 16, :] = z16
            g_buf[gi, ((b + 1) * NT - 1) * SLOT + 416:((b + 1) * NT - 1) * SLOT + 432, :] = z16
        for gi in range(2 * G):
            m_buf[gi, b * NT * SLOT:b * NT * SLOT + 16, :] = z16
            m_buf[gi, b * NT * SLOT + 16:b * NT * SLOT + 32, :] = z16
            m_buf[gi, ((b + 1) * NT - 1) * SLOT + 432:((b + 1) * NT - 1) * SLOT + 448, :] = z16
        xa_ref[b * TP // 2 + T // 2:(b + 1) * TP // 2, :] = jnp.zeros(((TP - T) // 2, D), U32)
    x_buf[0:LAG, :] = jnp.zeros((LAG, D), BF16)
    q_ref[TQ // 2:, :] = jnp.zeros((q_ref.shape[0] - TQ // 2, D), U32)

    def prep_a():
        a = lax.dot_general(wqkv_ref[:, 0:D], wqkv_ref[:, D:2 * D], NT_DIMS, preferred_element_type=F32)
        wa_p[...] = _pk((a * (D ** -0.5 * LOG2E)).astype(BF16))

    def prep(k):
        if k == 1:
            wmi_p[...] = _pk(wmi_ref[...])
        elif k == 2:
            wvo_p[...] = _pk(jnp.dot(wqkv_ref[:, 2 * D:3 * D], wao_ref[...], preferred_element_type=F32).astype(BF16))
        elif k == 4:
            wmo_p[...] = _pk(wmo_ref[...])
        elif k == 6:
            wm_p[...] = _pk(wm_ref[...])
        elif k in (3, 5):
            dw = (dwc_ref if k == 3 else dwm_ref)[...].astype(F32)
            g0 = 2 * G if k == 3 else 0
            for gi in range(dw.shape[1] // 128):
                for i in range(K):
                    dw_f[g0 + gi, i] = jnp.broadcast_to(dw[i:i + 1, gi * 128:(gi + 1) * 128], (8, 128))

    def ln_tile(t):
        return _pk(_ln(x_buf[_ds(t.fb, LAG, TQ, 16), :].astype(F32)).astype(BF16))

    def ln_store(t, xa):
        xa_ref[_ds(t.ab, 0, TQ // 2, 8), :] = xa

    def xq_of(t):
        return _upk(xa_ref[_ds(t.ab, 0, TQ // 2, 8), :])

    def xa_chunk(t, j):
        return _upk(xa_ref[_ds(t.kb, j * CK // 2, CK // 2, 16), :])

    def qproj(t):
        qf = jnp.dot(xq_of(t), _upk(wa_p[...]), preferred_element_type=F32)
        last[0] = qf[0:16, 0:128]
        q_ref[0:TQ // 2, :] = _pk(qf.astype(BF16))

    def l1(t):
        h = _gelu(jnp.dot(xq_of(t), _upk(wmi_p[...]), preferred_element_type=F32))
        u_ref[_ds(t.fb, 0, TQ, 16), :] = h[:, :D]
        g = _ln(h[:, D:])
        for gi in range(G):
            g_buf[gi, _ds(t.prev, 16 + TQ, 16, 32), :] = g[0:16, gi * 128:(gi + 1) * 128]
        for gi in range(G):
            g_buf[gi, _ds(t.cb, 16, TQ, 32), :] = g[:, gi * 128:(gi + 1) * 128]
        for gi in range(G):
            g_buf[gi, _ds(t.next, 0, 16, 32), :] = g[TQ - 16:TQ, gi * 128:(gi + 1) * 128]

    def m_store(t, g0, v):
        for gi in range(G):
            m_buf[g0 + gi, _ds(t.cb, 32, TQ, 32), :] = v[:, gi * 128:(gi + 1) * 128]
        for gi in range(G):
            m_buf[g0 + gi, _ds(t.next, 0, 32, 32), :] = v[TQ - 32:TQ, gi * 128:(gi + 1) * 128]

    def l2(t):
        gc = jnp.concatenate([_conv(g_buf, gi, dw_f, 2 * G + gi, t.cb, 16, TQ, K) for gi in range(G)], axis=-1)
        u = u_ref[_ds(t.fb, 0, TQ, 16), :]
        loc = jnp.dot((u * gc).astype(BF16), _upk(wmo_p[...]), preferred_element_type=F32)
        m_store(t, G, loc)

    def merge_half(half, pieces):
        lhs = []
        for (t, off, nrows, yo) in pieces:
            r = 32 - LAG + off
            ms = [m_buf[gi, _ds(t.cb, r, nrows, 32), :] + _conv(m_buf, gi, dw_f, gi, t.cb, r, nrows, K)
                  for gi in range(half * G, (half + 1) * G)]
            lhs.append(jnp.concatenate(ms, axis=-1))
        lhs = lhs[0] if len(lhs) == 1 else jnp.concatenate(lhs, axis=0)
        return jnp.dot(lhs.astype(BF16), _upk(wm_p[half * D // 2:(half + 1) * D // 2, :]), preferred_element_type=F32)

    def merge_a(pieces):
        y = merge_half(1, pieces)
        r = 0
        for (t, off, nrows, yo) in pieces:
            y_ref[yo:yo + nrows, :] = x_buf[_ds(t.fb, off, nrows, 16), :].astype(F32) + y[r:r + nrows]
            r += nrows

    def merge_b(pieces):
        y = merge_half(0, pieces)
        r = 0
        for (t, off, nrows, yo) in pieces:
            o_buf[_ds(t.fb, off, nrows, 16), :] = (y_ref[yo:yo + nrows, :] + y[r:r + nrows]).astype(BF16)
            r += nrows

    def p1_chunk(t, j, pos):
        q = _upk(q_ref[0:TQ // 2, :])
        if (j + 1) * CK <= T or REM == 0:
            sj = lax.dot_general(q, xa_chunk(t, j), NT_DIMS, preferred_element_type=F32)
            sts = [sj[:, lt * 128:(lt + 1) * 128] for lt in range(LT)]
            if (j + 1) * CK > T:
                col = lax.broadcasted_iota(jnp.int32, (TQ, 128), 1)
                sts[-1] = jnp.where(col < T % 128, sts[-1], -jnp.inf)
        else:
            nfull = (T - j * CK) // 128
            nrem = T - j * CK - nfull * 128
            assert nfull + 1 == LT and nrem % 16 == 0
            kf = _upk(xa_ref[_ds(t.kb, j * CK // 2, nfull * 64, 16), :])
            if REM == 1:
                sj = lax.dot_general(q, kf, NT_DIMS, preferred_element_type=F32)
            else:
                sj = jnp.concatenate([lax.dot_general(q[0:208], kf, NT_DIMS, preferred_element_type=F32),
                                      lax.dot_general(q[208:TQ], kf, NT_DIMS, preferred_element_type=F32)], axis=0)
            sts = [sj[:, lt * 128:(lt + 1) * 128] for lt in range(nfull)]
            kr = _upk(xa_ref[_ds(t.kb, j * CK // 2 + nfull * 64, nrem // 2, 16), :])
            st = lax.dot_general(kr, _upk(q_ref[...]), NT_DIMS, preferred_element_type=F32)
            st = jnp.concatenate([st, jnp.full((128 - nrem, st.shape[1]), -jnp.inf, F32)], axis=0)
            sts.append(st.T[0:TQ])
        last[0] = sj[0:16, 0:128]
        mloc = None
        for lt in range(LT):
            c0 = j * CK + lt * 128
            s_ref[:, c0:c0 + 128] = sts[lt]
            mloc = sts[lt] if mloc is None else jnp.maximum(mloc, sts[lt])
        if pos == 0:
            mp_ref[0:TQ] = mloc
        elif pos < NC - 1:
            mp_ref[0:TQ] = jnp.maximum(mp_ref[0:TQ], mloc)
        else:
            return jnp.maximum(mp_ref[0:TQ], mloc)

    def p1_fin(mpart):
        m = jnp.max(mpart, axis=-1, keepdims=True)
        mx_ref[0:TQ] = jnp.broadcast_to(m, (TQ, 128))

    def p2_chunk(t, j, pos, r0=0, n=TQ):
        ps = []
        lloc = None
        for lt in range(LT):
            c0 = j * CK + lt * 128
            p = jnp.exp2(s_ref[r0:r0 + n, c0:c0 + 128] - mx_ref[r0:r0 + n])
            lloc = p if lloc is None else lloc + p
            ps.append(p)
        pv = jnp.dot(jnp.concatenate(ps, axis=-1).astype(BF16), xa_chunk(t, j), preferred_element_type=F32)
        last[0] = pv[0:16, 0:128]
        last_e[0] = lloc[0:16]
        if pos == 0:
            lp_ref[r0:r0 + n] = lloc
            acc_ref[r0:r0 + n] = pv
        else:
            lp_ref[r0:r0 + n] += lloc
            acc_ref[r0:r0 + n] += pv

    def p2_fin(t, r0=0, n=TQ):
        l = jnp.sum(lp_ref[r0:r0 + n], axis=-1, keepdims=True)
        o = (acc_ref[r0:r0 + n] * (1.0 / l)).astype(BF16)
        glob = jnp.dot(o, _upk(wvo_p[...]), preferred_element_type=F32)
        if n == TQ:
            m_store(t, 0, glob)
        else:
            for gi in range(G):
                m_buf[gi, _ds(t.cb, 32 + r0, n, 32), :] = glob[:, gi * 128:(gi + 1) * 128]

    def anchor(buf):
        zrow = pl.multiple_of(zoff[0], 8)
        buf[0, pl.ds(zrow + JUNK, 8), :] = last[0][0:8]

    def anchor_l():
        zrow = pl.multiple_of(zoff[0], 8)
        lp_ref[pl.ds(zrow + TQ, 8), :] = last[0][0:8]

    def anchor_m():
        zrow = pl.multiple_of(zoff[0], 8)
        mx_ref[pl.ds(zrow + TQ, 8), :] = last[0][0:8]

    def anchor_x():
        zrow = pl.multiple_of(zoff[0], 16)
        x_buf[pl.ds(zrow + B * T + LAG, 16), 0:128] = last[0].astype(BF16)

    def out_copy(base, off, n):
        return pltpu.make_async_copy(o_buf.at[_ds(base, off, n, 16), :], o_hbm.at[_ds(base, off - LAG, n, 16), :], sem_out)

    DEF = 'H q Z V V V K V K V K V K Mb V K D V K V K V K Ma V K V K V K L V Zx K V K V Zl K N K K G'
    ORDER = DEF.split()
    ORDERP = 'q Z Zg V V V K V K V K V K V K Mb V K V K V K V K Ma V K V K V K V K L V Zl K K K G'.split()
    ORDERL = 'A Z A A A A A A A A A A A Mb A A A A Zl Mc Ga | B Z S B B R Zm B S B B R Zm B B B B B B B B B B Zl M1 Gb M2'.split()

    RPOS = 3
    CORD = list(range(NC - 1))
    CORD.insert(RPOS, NC - 1)
    CORDP = list(range(NC - 1))
    CORDP.insert(NC - 3, NC - 1)

    def step(order, pb, pa, t0, tp, th, tn, dma=None, pc=None):
        assert order.count('V') == NC and (tp is None or order.count('K') == NC)
        mpart = None
        jv = jk = 0
        for op in order:
            if op in SKIP.split(','):
                continue
            if op == 'q':
                qproj(tp)
            elif op == 'V':
                p2_chunk(t0, CORD[jv], jv)
                jv += 1
            elif op == 'K':
                assert jk < jv
                mpart = p1_chunk(tp, CORD[jk], jk)
                jk += 1
            elif op == 'Z':
                anchor(m_buf)
            elif op == 'Zg':
                anchor(g_buf)
            elif op == 'Zx':
                anchor_x()
            elif op == 'Zl':
                anchor_l()
            elif op == 'Ma':
                merge_a(pa)
            elif op == 'Mc':
                merge_a(pc)
            elif op == 'Mb':
                merge_b(pb)
            elif op == 'H':
                l1(th)
            elif op == 'L':
                l2(tp)
            elif op == 'N':
                xa_n = ln_tile(tn)
            elif op == 'G':
                p2_fin(t0)
            elif op == 'D':
                dma()
            else:
                raise ValueError(op)
        if tp is not None:
            p1_fin(mpart)
        if tn is not None:
            ln_store(tn, xa_n)

    def do_ln(t):
        ln_store(tile(t), ln_tile(tile(t)))

    jk = 0
    nln = 0
    for op in PRO:
        if op == 'STOP':
            return
        if op[0] == 's':
            dma_start(op)
        elif op[0] == 'x':
            x_copy(int(op[1:])).wait()
        elif op[0] == 'n':
            do_ln(int(op[1:]))
            nln = max(nln, min(int(op[1:]) + 1, NT))
        elif op[0] == 'w':
            w_copy(int(op[1:])).wait()
        elif op[0] == 'p':
            prep(int(op[1:]))
        elif op == 'A':
            prep_a()
        elif op == 'q':
            qproj(tile(0))
        elif op == 'K':
            assert nln * TQ >= min((CORDP[jk] + 1) * CK, T)
            mpart = p1_chunk(tile(0), CORDP[jk], jk)
            jk += 1
        elif op[0] == 'H':
            l1(tile(int(op[1:])))
        elif op == 'L0':
            l2(tile(0))
        elif op == 'Zg':
            anchor(g_buf)
        elif op == 'Zx':
            anchor_x()
        else:
            raise ValueError(op)
    assert jk == NC
    p1_fin(mpart)
    if STOP == 'pro':
        return

    def body(s, c):
        @pl.when(s == 1)
        def _():
            x_copy(NT + 1).wait()

        w = jnp.maximum(s - 1, 0)
        fb = w * TQ

        def dma():
            @pl.when(s > 0)
            def _():
                out_copy(fb, LAG, TQ - LAG).start()

            @pl.when(jnp.logical_and(s > 1, s != NT + 1))
            def _():
                out_copy(fb, 0, LAG).start()

        step(ORDER, [(tile(w), 0, TQ, 0)], [(tile(s), 0, TQ, 0)], tile(s), tile(s + 1), tile(s + 2),
             tile(jnp.minimum(s + NT + 1, NS - 1)), dma)
        return c
    lax.fori_loop(0, NITER, body, 0)

    z = zoff[0]
    t9 = tile(NT - 1)

    tl = tile(NS - 1)
    Y2 = TQ + 3 * LAG

    @pl.when(z == 0)
    def _():
        dyn = (lambda t: tile(z + t)) if '1' == '1' else tile
        step(ORDERP, [(dyn(NS - 3), 0, TQ, 0)], [(dyn(NS - 2), 0, TQ, 0), (t9, TQ, LAG, TQ + LAG)],
             dyn(NS - 2), dyn(NS - 1), None, None, pc=[(dyn(NS - 1), 0, TQ + LAG, Y2)])
        out_copy(0, (NS - 3) * TQ, TQ).start()

    RA = 288

    cnt = {'A': 0, 'B': 0}

    def last_block(ops):
        dyn = (lambda t: tile(z + t)) if '1' == '1' else tile
        tl = dyn(NS - 1)
        for op in ops:
            if op == 'A':
                p2_chunk(tl, cnt['A'], cnt['A'], 0, RA)
                cnt['A'] += 1
            elif op == 'B':
                p2_chunk(tl, cnt['B'], cnt['B'], RA, TQ - RA)
                cnt['B'] += 1
            elif op == 'Z':
                anchor(m_buf)
            elif op == 'Ze':
                last[0] = last_e[0]
                anchor(m_buf)
            elif op == 'Zl':
                anchor_l()
            elif op == 'Zm':
                anchor_m()
            elif op == 'S':
                saved = last[0]
            elif op == 'R':
                last[0] = saved
            elif op == 'Mb':
                merge_b([(dyn(NS - 2), 0, TQ, 0), (t9, TQ, LAG, TQ + LAG)])
                out_copy(0, (NS - 2) * TQ, TQ).start()
                out_copy(0, NT * TQ, LAG).start()
            elif op == 'Mc':
                merge_a([(tl, 0, TQ + LAG, Y2)])
            elif op == 'Ga':
                p2_fin(tl, 0, RA)
            elif op == 'Gb':
                p2_fin(tl, RA, TQ - RA)
            elif op == 'M1':
                merge_b([(tl, 0, RA, Y2)])
                out_copy(0, (NS - 1) * TQ, RA).start()
            elif op == 'M2':
                merge_b([(tl, RA, TQ + LAG - RA, Y2 + RA)])
                out_copy(0, (NS - 1) * TQ + RA, TQ + LAG - RA).start()
            else:
                raise ValueError(op)

    for bi, ops in enumerate(' '.join(ORDERL).split('|')):
        pl.when(z < 1 + bi)(functools.partial(last_block, ops.split()))
    assert cnt['A'] == NC and cnt['B'] == NC

    nrows = (NITER - 1) * (TQ - LAG) + sum(LAG for s in range(2, NITER) if s != NT + 1) + 3 * TQ + 2 * LAG
    out_copy(0, LAG, nrows).wait()


@jax.jit
def pallas_standalone__conformer_family_e_branchformer__speech_kernel(
    x, w_qkv, w_att_out, w_mlp_in, dw_csgu, w_mlp_out, dw_merge, w_merge):
    B, T, D = x.shape
    K = dw_csgu.shape[0]
    TQ = 400
    TP = 4096
    CK = 256
    G = D // 128
    NT = T // TQ
    RB = (B * NT + 1) * SLOT
    out = pl.pallas_call(
        functools.partial(kernel, B=B, T=T, D=D, K=K, TQ=TQ, TP=TP, CK=CK),
        in_specs=[pl.BlockSpec(memory_space=pl.ANY)] * 8,
        out_specs=pl.BlockSpec(memory_space=pl.ANY),
        out_shape=jax.ShapeDtypeStruct((B * T, D), x.dtype),
        scratch_shapes=[
            pltpu.VMEM((B * T + 32, D), BF16),
            pltpu.VMEM((B * T + 32, D), BF16),
            pltpu.VMEM((B * TP // 2, D), U32),
            pltpu.VMEM((D // 2, D), U32),
            pltpu.VMEM((D // 2, D), U32),
            pltpu.VMEM((D // 2, 2 * D), U32),
            pltpu.VMEM((D // 2, D), U32),
            pltpu.VMEM((D, D), U32),
            pltpu.VMEM((3 * G, 32, 8, 128), F32),
            pltpu.VMEM((G, RB, 128), F32),
            pltpu.VMEM((2 * G, RB, 128), F32),
            pltpu.VMEM((B * T, D), F32),
            pltpu.VMEM((TQ, TP), F32),
            pltpu.VMEM((TQ + 16, 128), F32),
            pltpu.VMEM((256, D), U32),
            pltpu.VMEM((TQ + 16, 128), F32),
            pltpu.VMEM((TQ + 16, 128), F32),
            pltpu.VMEM((TQ, D), F32),
            pltpu.VMEM((2 * TQ + 4 * LAG, D), F32),
            pltpu.VMEM(w_qkv.shape, BF16),
            pltpu.VMEM(w_att_out.shape, BF16),
            pltpu.VMEM(w_mlp_in.shape, BF16),
            pltpu.VMEM(dw_csgu.shape, BF16),
            pltpu.VMEM(w_mlp_out.shape, BF16),
            pltpu.VMEM(dw_merge.shape, BF16),
            pltpu.VMEM(w_merge.shape, BF16),
            pltpu.SMEM((1,), jnp.int32),
            pltpu.SemaphoreType.DMA((max(GRP.values()) + 1,)),
            pltpu.SemaphoreType.DMA,
        ],
        compiler_params=pltpu.CompilerParams(vmem_limit_bytes=110 * 1024 * 1024, disable_bounds_checks=True),
    )(x.reshape(B * T, D), w_qkv, w_att_out, w_mlp_in, dw_csgu, w_mlp_out, dw_merge, w_merge)
    return out.reshape(B, T, D)
```

```python
import functools
NITER = 18
SKIP = ''
STOP = ''
CV = 10
STR = 1
RSQ = 1
REM = 2
import jax
import jax.numpy as jnp
from jax import lax
import jax.experimental.pallas as pl
import jax.experimental.pallas.tpu as pltpu

F32 = jnp.float32
BF16 = jnp.bfloat16
U32 = jnp.uint32
LOG2E = 1.4426950408889634
NT_DIMS = (((1,), (1,)), ((), ()))
SLOT = 448
LAG = 16

PRO0 = 'sx0 sw0 sx1 | x0 sx2 sw1 sx3 n0 w0 x1 sx4 sx5 A n1 q K K K c0+3 x2 w1 x3 sx6 sx7 sw3 sw4 sx8 sx9 p1 n2 n3 H0 H1 K c3+3 x4 x5 x6 x7 w3 w4 sw2 sw5 sw6 sw7 sx10 p3 p4 K Zg n4 n5 n6 n7 K K K K K K L0 c6+6 x8 x9 w2 w5 w6 w7 x10 sx11 n8 n9 p5 p6 K K K K K p2 n10 c12+2'.split()
GRP = {}
_g, _prev = -1, False
for _op in PRO0:
    _is_wait = _op[0] in 'xw'
    if _is_wait:
        if not _prev:
            _g += 1
        GRP[_op] = _g
    _prev = _is_wait
GRP['x11'] = _g + 1


def PAIRSEQ(a, b):
    v = 0
    if v == 0:
        return [(a, 1), (a, 4), (a, 5), (a, 7), (b, 1), (b, 7), (b, 5), (b, 4),
                (a, 2), (a, 3), (b, 2), (b, 3), (a, 61), (a, 62), (b, 61), (b, 62)]
    return [(a, 61), (a, 62), (b, 61), (b, 62), (a, 2), (a, 3), (b, 2), (b, 3),
            (a, 1), (a, 4), (a, 5), (a, 7), (b, 1), (b, 7), (b, 5), (b, 4)]


def _pk(x):
    return pltpu.bitcast(x, U32)


def _upk(x):
    return pltpu.bitcast(x, BF16)


def _ln(x, eps=1e-5):
    m = jnp.mean(x, axis=-1, keepdims=True)
    xc = x - m
    v = jnp.mean(xc * xc, axis=-1, keepdims=True)
    if RSQ == 0:
        return xc * lax.rsqrt(v + eps)
    return xc * jnp.exp2(jnp.log(v + eps) * (-0.5 * LOG2E))


def _gelu(x):
    c = 0.7978845608028654
    hx = 0.5 * x
    return hx + hx * jnp.tanh(x * (c + (c * 0.044715) * (x * x)))


def _ds(base, off, n, align):
    if isinstance(base, int):
        return pl.ds(base + off, n)
    a = align
    while off % a:
        a //= 2
    return pl.ds(pl.multiple_of(base + off, a), n) if a > 1 else pl.ds(base + off, n)


def _conv(buf_ref, g, w_ref, wg, base, off, nrows, K):
    outs = []
    nv = nrows // 8
    v0 = 0
    while v0 < nv:
        V = min(CV, nv - v0)
        acc = None
        for p in range(8):
            taps = list(range(p, K, 8))
            nq = V + len(taps) - 1
            slab = buf_ref[g, _ds(base, off + 8 * v0 + p - K // 2, 8 * nq, 32), :].reshape(nq, 8, 128)
            for qi, i in enumerate(taps):
                term = slab[qi:qi + V] * w_ref[wg, i][None]
                acc = term if acc is None else acc + term
        outs.append(acc.reshape(8 * V, 128))
        v0 += V
    return jnp.concatenate(outs, axis=0) if len(outs) > 1 else outs[0]


class Tile:
    def __init__(self, t, NT, NS, TQ, TP, T):
        if isinstance(t, int):
            b = t // NT
            first, last = t % NT == 0, t % NT == NT - 1
            self.prev = (NS if first else t - 1) * SLOT
            self.next = (NS if last else t + 1) * SLOT
        else:
            b = (t >= NT).astype(jnp.int32)
            first = jnp.logical_or(t == 0, t == NT)
            last = jnp.logical_or(t == NT - 1, t == NS - 1)
            self.prev = jnp.where(first, NS, t - 1) * SLOT
            self.next = jnp.where(last, NS, t + 1) * SLOT
        self.cb = t * SLOT
        self.fb = t * TQ
        self.ab = t * (TQ // 2) + b * ((TP - T) // 2)
        self.kb = b * (TP // 2)
        self.cbk = b * (16 * 64)


def kernel(x_hbm, wqkv_hbm, wao_hbm, wmi_hbm, dwc_hbm, wmo_hbm, dwm_hbm, wm_hbm, o_hbm,
           x_buf, o_buf, xa_ref, wa_p, wvo_p, wmi_p, wmo_p, wm_p, dw_f, g_buf, m_buf, u_ref,
           s_ref, mx_ref, q_ref, qc_ref, kc_ref, mp_ref, lp_ref, acc_ref, y_ref,
           wqkv_ref, wao_ref, wmi_ref, dwc_ref, wmo_ref, dwm_ref, wm_ref,
           zoff, sem_in, sem_out,
           *, B, T, D, K, TQ, TP, CK):
    NT = T // TQ
    NS = B * NT
    G = D // 128
    NC = TP // CK
    LT = CK // 128
    assert B == 2
    last = [None]
    last_e = [None]
    JUNK = NS * SLOT + 64

    def tile(t):
        return Tile(t, NT, NS, TQ, TP, T)

    def x_copy(t):
        r0 = t * TQ if t <= NT else (NT + 2) * TQ
        n = TQ if t < NT else (2 * TQ if t == NT else B * T - r0)
        return pltpu.make_async_copy(x_hbm.at[pl.ds(r0, n), :], x_buf.at[pl.ds(LAG + r0, n), :], sem_in.at[GRP['x%d' % t]])

    w_pairs = [(wqkv_hbm.at[:, 0:2 * D], wqkv_ref.at[:, 0:2 * D]), (wmi_hbm, wmi_ref), (wao_hbm, wao_ref), (dwc_hbm, dwc_ref),
               (wmo_hbm, wmo_ref), (dwm_hbm, dwm_ref), (wm_hbm, wm_ref), (wqkv_hbm.at[:, 2 * D:3 * D], wqkv_ref.at[:, 2 * D:3 * D])]

    def w_copy(k):
        return pltpu.make_async_copy(w_pairs[k][0], w_pairs[k][1], sem_in.at[GRP['w%d' % k]])

    def dma_start(op):
        if STOP == 'pro' and op == 'sx11':
            return
        if op[1] == 'x':
            x_copy(int(op[2:])).start()
        elif op == 'swr':
            for k in range(2, len(w_pairs)):
                w_copy(k).start()
        else:
            w_copy(int(op[2:])).start()

    PRO = list(PRO0)
    for op in PRO[:PRO.index('|')]:
        dma_start(op)
    PRO = PRO[PRO.index('|') + 1:]

    zoff[0] = 0
    z16 = jnp.zeros((16, 128), F32)
    for b in range(B):
        for gi in range(G):
            g_buf[gi, b * NT * SLOT:b * NT * SLOT + 16, :] = z16
            g_buf[gi, ((b + 1) * NT - 1) * SLOT + 416:((b + 1) * NT - 1) * SLOT + 432, :] = z16
        for gi in range(2 * G):
            m_buf[gi, b * NT * SLOT:b * NT * SLOT + 16, :] = z16
            m_buf[gi, b * NT * SLOT + 16:b * NT * SLOT + 32, :] = z16
            m_buf[gi, ((b + 1) * NT - 1) * SLOT + 432:((b + 1) * NT - 1) * SLOT + 448, :] = z16
        xa_ref[b * TP // 2 + T // 2:(b + 1) * TP // 2, :] = jnp.zeros(((TP - T) // 2, D), U32)
    x_buf[0:LAG, :] = jnp.zeros((LAG, D), BF16)
    q_ref[TQ // 2:, :] = jnp.zeros((q_ref.shape[0] - TQ // 2, D), U32)

    def prep_a():
        a = lax.dot_general(wqkv_ref[:, 0:D], wqkv_ref[:, D:2 * D], NT_DIMS, preferred_element_type=F32)
        wa_p[...] = _pk((a * (D ** -0.5 * LOG2E)).astype(BF16))

    def prep(k):
        if k == 1:
            wmi_p[...] = _pk(wmi_ref[...])
        elif k == 2:
            wvo_p[...] = _pk(jnp.dot(wqkv_ref[:, 2 * D:3 * D], wao_ref[...], preferred_element_type=F32).astype(BF16))
        elif k == 4:
            wmo_p[...] = _pk(wmo_ref[...])
        elif k == 6:
            wm_p[...] = _pk(wm_ref[...])
        elif k in (3, 5):
            dw = (dwc_ref if k == 3 else dwm_ref)[...].astype(F32)
            g0 = 2 * G if k == 3 else 0
            for gi in range(dw.shape[1] // 128):
                for i in range(K):
                    dw_f[g0 + gi, i] = jnp.broadcast_to(dw[i:i + 1, gi * 128:(gi + 1) * 128], (8, 128))

    def ln_tile(t):
        return _pk(_ln(x_buf[_ds(t.fb, LAG, TQ, 16), :].astype(F32)).astype(BF16))

    def ln_store(t, xa):
        xa_ref[_ds(t.ab, 0, TQ // 2, 8), :] = xa

    def xq_of(t):
        return _upk(xa_ref[_ds(t.ab, 0, TQ // 2, 8), :])

    def xa_chunk(t, j):
        return _upk(xa_ref[_ds(t.kb, j * CK // 2, CK // 2, 16), :])

    R1 = 208
    R2 = TQ - R1

    def qproj(t, combos=True):
        qf = jnp.dot(xq_of(t), _upk(wa_p[...]), preferred_element_type=F32)
        last[0] = qf[0:16, 0:128]
        q_ref[0:TQ // 2, :] = _pk(qf.astype(BF16))
        if STR and combos:
            a11, a12 = qf[0:R1, 0:128], qf[0:R1, 128:256]
            a21, a22 = qf[R1:TQ, 0:128], qf[R1:TQ, 128:256]
            cat = lambda u, v: jnp.concatenate([u, v], axis=0)
            qc_ref[0:R1 // 2, 0:384] = _pk(jnp.concatenate(
                [cat(a11[0:R2] + a22, a11[R2:]), a11 + a12, cat(a12[0:R2] - a22, a12[R2:])], axis=1).astype(BF16))
            qc_ref[0:R2 // 2, 384:640] = _pk(jnp.concatenate([a21 + a22, a21 - a11[0:R2]], axis=1).astype(BF16))

    def kcomb(kb, cbk, c0, n):
        for c in range(n):
            xk = _upk(xa_ref[_ds(kb + c0 * 128, c * 128, 128, 16), :]).astype(F32)
            alo, ahi, blo, bhi = xk[0:128, 0:128], xk[0:128, 128:256], xk[128:256, 0:128], xk[128:256, 128:256]
            v = jnp.concatenate([alo + bhi, blo - bhi, ahi - alo, alo + blo, ahi + bhi], axis=1)
            kc_ref[_ds(cbk + c0 * 64, c * 64, 64, 32), :] = _pk(v.astype(BF16))

    def l1(t):
        hp = jnp.dot(xq_of(t), _upk(wmi_p[...]), preferred_element_type=F32)
        last[0] = hp[0:16, 0:128]
        h = _gelu(hp)
        u_ref[_ds(t.fb, 0, TQ, 16), :] = h[:, :D]
        g = _ln(h[:, D:])
        for gi in range(G):
            g_buf[gi, _ds(t.prev, 16 + TQ, 16, 32), :] = g[0:16, gi * 128:(gi + 1) * 128]
        for gi in range(G):
            g_buf[gi, _ds(t.cb, 16, TQ, 32), :] = g[:, gi * 128:(gi + 1) * 128]
        for gi in range(G):
            g_buf[gi, _ds(t.next, 0, 16, 32), :] = g[TQ - 16:TQ, gi * 128:(gi + 1) * 128]

    def m_store(t, g0, v):
        for gi in range(G):
            m_buf[g0 + gi, _ds(t.cb, 32, TQ, 32), :] = v[:, gi * 128:(gi + 1) * 128]
        for gi in range(G):
            m_buf[g0 + gi, _ds(t.next, 0, 32, 32), :] = v[TQ - 32:TQ, gi * 128:(gi + 1) * 128]

    def l2(t):
        gc = jnp.concatenate([_conv(g_buf, gi, dw_f, 2 * G + gi, t.cb, 16, TQ, K) for gi in range(G)], axis=-1)
        u = u_ref[_ds(t.fb, 0, TQ, 16), :]
        loc = jnp.dot((u * gc).astype(BF16), _upk(wmo_p[...]), preferred_element_type=F32)
        m_store(t, G, loc)

    def merge_half(half, pieces):
        lhs = []
        for (t, off, nrows, yo) in pieces:
            r = 32 - LAG + off
            ms = [m_buf[gi, _ds(t.cb, r, nrows, 32), :] + _conv(m_buf, gi, dw_f, gi, t.cb, r, nrows, K)
                  for gi in range(half * G, (half + 1) * G)]
            lhs.append(jnp.concatenate(ms, axis=-1))
        lhs = lhs[0] if len(lhs) == 1 else jnp.concatenate(lhs, axis=0)
        return jnp.dot(lhs.astype(BF16), _upk(wm_p[half * D // 2:(half + 1) * D // 2, :]), preferred_element_type=F32)

    def merge_a(pieces):
        y = merge_half(1, pieces)
        r = 0
        for (t, off, nrows, yo) in pieces:
            y_ref[yo:yo + nrows, :] = x_buf[_ds(t.fb, off, nrows, 16), :].astype(F32) + y[r:r + nrows]
            r += nrows

    def merge_b(pieces):
        y = merge_half(0, pieces)
        r = 0
        for (t, off, nrows, yo) in pieces:
            o_buf[_ds(t.fb, off, nrows, 16), :] = (y_ref[yo:yo + nrows, :] + y[r:r + nrows]).astype(BF16)
            r += nrows

    def p1_strassen(t, j, pos):
        nt = lambda a, b: lax.dot_general(a, b, NT_DIMS, preferred_element_type=F32)
        kc = lambda i: _upk(kc_ref[_ds(t.cbk, j * 64, 64, 32), i * 128:(i + 1) * 128])
        b11 = _upk(xa_ref[_ds(t.kb, j * 128, 64, 16), 0:128])
        b22 = _upk(xa_ref[_ds(t.kb, j * 128 + 64, 64, 16), 128:256])
        m1 = nt(_upk(qc_ref[0:R1 // 2, 0:128]), kc(0))
        m4 = nt(_upk(q_ref[R1 // 2:TQ // 2, 128:256]), kc(2))
        m5 = nt(_upk(qc_ref[0:R1 // 2, 128:256]), b22)
        m7 = nt(_upk(qc_ref[0:R1 // 2, 256:384]), kc(4))
        m2 = nt(_upk(qc_ref[0:R2 // 2, 384:512]), b11)
        m3 = nt(_upk(q_ref[0:R1 // 2, 0:128]), kc(1))
        m6 = nt(_upk(qc_ref[0:R2 // 2, 512:640]), kc(3))
        last[0] = m1[0:16]
        c11 = m1 + (m7 - m5)
        c11 = jnp.concatenate([c11[0:R2] + m4, c11[R2:]], axis=0)
        c12 = m3 + m5
        c21 = m2 + m4
        c22 = (m1[0:R2] - m2) + (m3[0:R2] + m6)
        c0 = j * CK
        s_ref[0:R1, c0:c0 + 128] = c11
        s_ref[0:R1, c0 + 128:c0 + 256] = c12
        s_ref[R1:TQ, c0:c0 + 128] = c21
        s_ref[R1:TQ, c0 + 128:c0 + 256] = c22
        mloc = jnp.concatenate([jnp.maximum(c11, c12), jnp.maximum(c21, c22)], axis=0)
        if pos == 0:
            mp_ref[0:TQ] = mloc
        elif pos < NC - 1:
            mp_ref[0:TQ] = jnp.maximum(mp_ref[0:TQ], mloc)
        else:
            return jnp.maximum(mp_ref[0:TQ], mloc)

    def p1_pair(t, js, pos):
        nt = lambda a, b: lax.dot_general(a, b, NT_DIMS, preferred_element_type=F32)
        kc = lambda j, i: _upk(kc_ref[_ds(t.cbk, j * 64, 64, 32), i * 128:(i + 1) * 128])
        b11 = lambda j: _upk(xa_ref[_ds(t.kb, j * 128, 64, 16), 0:128])
        b22 = lambda j: _upk(xa_ref[_ds(t.kb, j * 128 + 64, 64, 16), 128:256])
        f = {
            1: lambda j: nt(_upk(qc_ref[0:R1 // 2, 0:128]), kc(j, 0)),
            4: lambda j: nt(_upk(q_ref[R1 // 2:TQ // 2, 128:256]), kc(j, 2)),
            5: lambda j: nt(_upk(qc_ref[0:R1 // 2, 128:256]), b22(j)),
            7: lambda j: nt(_upk(qc_ref[0:R1 // 2, 256:384]), kc(j, 4)),
            2: lambda j: nt(_upk(qc_ref[0:R2 // 2, 384:512]), b11(j)),
            3: lambda j: nt(_upk(q_ref[0:R1 // 2, 0:128]), kc(j, 1)),
            61: lambda j: nt(_upk(qc_ref[0:R2 // 4, 512:640]), kc(j, 3)),
            62: lambda j: nt(_upk(qc_ref[R2 // 4:R2 // 2, 512:640]), kc(j, 3)),
        }
        a, b = js
        m = {}
        for (j, k) in PAIRSEQ(a, b):
            m[(j, k)] = f[k](j)
        last[0] = m[(a, 1)][0:16]
        mloc = None
        for j in js:
            m1, m2, m3, m4, m5, m7 = (m[(j, k)] for k in (1, 2, 3, 4, 5, 7))
            m6 = jnp.concatenate([m[(j, 61)], m[(j, 62)]], axis=0)
            c11 = m1 + (m7 - m5)
            c11 = jnp.concatenate([c11[0:R2] + m4, c11[R2:]], axis=0)
            c12 = m3 + m5
            c21 = m2 + m4
            c22 = ((m1[0:R2] - m2) + m3[0:R2]) + m6
            c0 = j * CK
            s_ref[0:R1, c0:c0 + 128] = c11
            s_ref[0:R1, c0 + 128:c0 + 256] = c12
            s_ref[R1:TQ, c0:c0 + 128] = c21
            s_ref[R1:TQ, c0 + 128:c0 + 256] = c22
            ml = jnp.concatenate([jnp.maximum(c11, c12), jnp.maximum(c21, c22)], axis=0)
            mloc = ml if mloc is None else jnp.maximum(mloc, ml)
        if pos == 0:
            mp_ref[0:TQ] = mloc
        elif pos < NC - 2:
            mp_ref[0:TQ] = jnp.maximum(mp_ref[0:TQ], mloc)
        else:
            return jnp.maximum(mp_ref[0:TQ], mloc)

    def p1_chunk(t, j, pos, strassen=True):
        if STR and strassen and (j + 1) * CK <= T:
            return p1_strassen(t, j, pos)
        q = _upk(q_ref[0:TQ // 2, :])
        if (j + 1) * CK <= T or REM == 0:
            sj = lax.dot_general(q, xa_chunk(t, j), NT_DIMS, preferred_element_type=F32)
            sts = [sj[:, lt * 128:(lt + 1) * 128] for lt in range(LT)]
            if (j + 1) * CK > T:
                col = lax.broadcasted_iota(jnp.int32, (TQ, 128), 1)
                sts[-1] = jnp.where(col < T % 128, sts[-1], -jnp.inf)
        else:
            nfull = (T - j * CK) // 128
            nrem = T - j * CK - nfull * 128
            assert nfull + 1 == LT and nrem % 16 == 0
            kf = _upk(xa_ref[_ds(t.kb, j * CK // 2, nfull * 64, 16), :])
            if REM == 1:
                sj = lax.dot_general(q, kf, NT_DIMS, preferred_element_type=F32)
            else:
                sj = jnp.concatenate([lax.dot_general(q[0:208], kf, NT_DIMS, preferred_element_type=F32),
                                      lax.dot_general(q[208:TQ], kf, NT_DIMS, preferred_element_type=F32)], axis=0)
            sts = [sj[:, lt * 128:(lt + 1) * 128] for lt in range(nfull)]
            kr = _upk(xa_ref[_ds(t.kb, j * CK // 2 + nfull * 64, nrem // 2, 16), :])
            st = lax.dot_general(kr, _upk(q_ref[...]), NT_DIMS, preferred_element_type=F32)
            st = jnp.concatenate([st, jnp.full((128 - nrem, st.shape[1]), -jnp.inf, F32)], axis=0)
            sts.append(st.T[0:TQ])
        last[0] = sj[0:16, 0:128]
        mloc = None
        for lt in range(LT):
            c0 = j * CK + lt * 128
            s_ref[:, c0:c0 + 128] = sts[lt]
            mloc = sts[lt] if mloc is None else jnp.maximum(mloc, sts[lt])
        if pos == 0:
            mp_ref[0:TQ] = mloc
        elif pos < NC - 1:
            mp_ref[0:TQ] = jnp.maximum(mp_ref[0:TQ], mloc)
        else:
            return jnp.maximum(mp_ref[0:TQ], mloc)

    def p1_fin(mpart):
        m = jnp.max(mpart, axis=-1, keepdims=True)
        mx_ref[0:TQ] = jnp.broadcast_to(m, (TQ, 128))

    def p2_chunk(t, j, pos, r0=0, n=TQ):
        ps = []
        lloc = None
        for lt in range(LT):
            c0 = j * CK + lt * 128
            p = jnp.exp2(s_ref[r0:r0 + n, c0:c0 + 128] - mx_ref[r0:r0 + n])
            lloc = p if lloc is None else lloc + p
            ps.append(p)
        pv = jnp.dot(jnp.concatenate(ps, axis=-1).astype(BF16), xa_chunk(t, j), preferred_element_type=F32)
        last[0] = pv[0:16, 0:128]
        last_e[0] = lloc[0:16]
        if pos == 0:
            lp_ref[r0:r0 + n] = lloc
            acc_ref[r0:r0 + n] = pv
        else:
            lp_ref[r0:r0 + n] += lloc
            acc_ref[r0:r0 + n] += pv

    def p2_fin(t, r0=0, n=TQ):
        l = jnp.sum(lp_ref[r0:r0 + n], axis=-1, keepdims=True)
        o = (acc_ref[r0:r0 + n] * (1.0 / l)).astype(BF16)
        glob = jnp.dot(o, _upk(wvo_p[...]), preferred_element_type=F32)
        if n == TQ:
            m_store(t, 0, glob)
        else:
            for gi in range(G):
                m_buf[gi, _ds(t.cb, 32 + r0, n, 32), :] = glob[:, gi * 128:(gi + 1) * 128]

    def anchor(buf):
        zrow = pl.multiple_of(zoff[0], 8)
        buf[0, pl.ds(zrow + JUNK, 8), :] = last[0][0:8]

    def anchor_l():
        zrow = pl.multiple_of(zoff[0], 8)
        lp_ref[pl.ds(zrow + TQ, 8), :] = last[0][0:8]

    def anchor_m():
        zrow = pl.multiple_of(zoff[0], 8)
        mx_ref[pl.ds(zrow + TQ, 8), :] = last[0][0:8]

    def anchor_x():
        zrow = pl.multiple_of(zoff[0], 16)
        x_buf[pl.ds(zrow + B * T + LAG, 16), 0:128] = last[0].astype(BF16)

    def out_copy(base, off, n):
        return pltpu.make_async_copy(o_buf.at[_ds(base, off, n, 16), :], o_hbm.at[_ds(base, off - LAG, n, 16), :], sem_out)

    DEF = 'C H Z q V V V V V V Mb K Ks KK D KK V V V V V Ma KK KK V V V V V Zl L KK Zx KK N KK G'
    ORDER = DEF.split()
    ORDERP = 'q Z Zg V V V V V V V Mb K KK KK V V V V V Ma KK KK V V V V Zl Ks L KK KK KK G'.split()
    ORDERL = 'A Z A A A A A A A A A A A Mb A A A A Zl Mc Ga | B Z S B B R Zm B S B B R Zm B B B B B B B B B B Zl M1 Gb M2'.split()

    RPOS = 3
    CORD = list(range(NC - 1))
    CORD.insert(RPOS, NC - 1)
    CORDP = list(range(NC - 1))
    CORDP.insert(NC - 3, NC - 1)

    def step(order, pb, pa, t0, tp, th, tn, dma=None, pc=None, cc=None):
        CORD = []
        nxt = 0
        for op in order:
            if op == 'KK':
                CORD += [nxt, nxt + 1]
                nxt += 2
            elif op == 'Ks':
                CORD.append(NC - 2)
            elif op == 'K':
                CORD.append(NC - 1)
        assert order.count('V') == NC and sorted(CORD) == list(range(NC))
        mpart = None
        jv = jk = 0
        for op in order:
            if op in SKIP.split(','):
                continue
            if op == 'q':
                qproj(tp)
            elif op == 'V':
                p2_chunk(t0, CORD[jv], jv)
                jv += 1
            elif op == 'K':
                assert jk < jv
                mpart = p1_chunk(tp, CORD[jk], jk)
                jk += 1
            elif op == 'KK':
                assert jk + 1 < jv and CORD[jk] < NC - 1 and CORD[jk + 1] < NC - 1
                mpart = p1_pair(tp, (CORD[jk], CORD[jk + 1]), jk)
                jk += 2
            elif op == 'Ks':
                assert jk < jv
                mpart = p1_chunk(tp, CORD[jk], jk, False)
                jk += 1
            elif op == 'Z':
                anchor(m_buf)
            elif op == 'Zg':
                anchor(g_buf)
            elif op == 'Zx':
                anchor_x()
            elif op == 'Zl':
                anchor_l()
            elif op == 'Ma':
                merge_a(pa)
            elif op == 'Mc':
                merge_a(pc)
            elif op == 'Mb':
                merge_b(pb)
            elif op == 'H':
                l1(th)
            elif op == 'L':
                l2(tp)
            elif op == 'N':
                xa_n = ln_tile(tn)
            elif op == 'G':
                p2_fin(t0)
            elif op == 'D':
                dma()
            elif op == 'C':
                kcomb(TP // 2, 16 * 64, cc, 2)
            else:
                raise ValueError(op)
        if tp is not None:
            p1_fin(mpart)
        if tn is not None:
            ln_store(tn, xa_n)

    def do_ln(t):
        ln_store(tile(t), ln_tile(tile(t)))

    jk = 0
    nln = 0
    for op in PRO:
        if op == 'STOP':
            return
        if op[0] == 's':
            dma_start(op)
        elif op[0] == 'x':
            x_copy(int(op[1:])).wait()
        elif op[0] == 'n':
            do_ln(int(op[1:]))
            nln = max(nln, min(int(op[1:]) + 1, NT))
        elif op[0] == 'w':
            w_copy(int(op[1:])).wait()
        elif op[0] == 'p':
            prep(int(op[1:]))
        elif op == 'A':
            prep_a()
        elif op == 'q':
            qproj(tile(0), False)
        elif op == 'K':
            assert nln * TQ >= min((CORDP[jk] + 1) * CK, T)
            mpart = p1_chunk(tile(0), CORDP[jk], jk, False)
            jk += 1
        elif op[0] == 'H':
            l1(tile(int(op[1:])))
        elif op == 'L0':
            l2(tile(0))
        elif op == 'Zg':
            anchor(g_buf)
        elif op == 'Zx':
            anchor_x()
        elif op == 'Za':
            zrow = pl.multiple_of(zoff[0], 8)
            xa_ref[pl.ds(zrow + B * TP // 2, 8), 0:128] = pltpu.bitcast(last[0][0:8], U32)
        elif op[0] == 'c':
            c0, n = map(int, op[1:].split('+'))
            assert nln * TQ >= (c0 + n) * CK
            kcomb(0, 0, c0, n)
        else:
            raise ValueError(op)
    assert jk == NC
    p1_fin(mpart)
    if STOP == 'pro':
        return

    def body(s, c):
        @pl.when(s == 1)
        def _():
            x_copy(NT + 1).wait()

        w = jnp.maximum(s - 1, 0)
        fb = w * TQ

        def dma():
            @pl.when(s > 0)
            def _():
                out_copy(fb, LAG, TQ - LAG).start()

            @pl.when(jnp.logical_and(s > 1, s != NT + 1))
            def _():
                out_copy(fb, 0, LAG).start()

        step(ORDER, [(tile(w), 0, TQ, 0)], [(tile(s), 0, TQ, 0)], tile(s), tile(s + 1), tile(s + 2),
             tile(jnp.minimum(s + NT + 1, NS - 1)), dma, cc=jnp.clip(2 * s - 4, 0, NC - 4))
        return c
    lax.fori_loop(0, NITER, body, 0)

    z = zoff[0]
    t9 = tile(NT - 1)

    tl = tile(NS - 1)
    Y2 = TQ + 3 * LAG

    @pl.when(z == 0)
    def _():
        dyn = (lambda t: tile(z + t)) if '1' == '1' else tile
        step(ORDERP, [(dyn(NS - 3), 0, TQ, 0)], [(dyn(NS - 2), 0, TQ, 0), (t9, TQ, LAG, TQ + LAG)],
             dyn(NS - 2), dyn(NS - 1), None, None, pc=[(dyn(NS - 1), 0, TQ + LAG, Y2)])
        out_copy(0, (NS - 3) * TQ, TQ).start()

    RA = 288

    cnt = {'A': 0, 'B': 0}

    def last_block(ops):
        dyn = (lambda t: tile(z + t)) if '1' == '1' else tile
        tl = dyn(NS - 1)
        for op in ops:
            if op == 'A':
                p2_chunk(tl, cnt['A'], cnt['A'], 0, RA)
                cnt['A'] += 1
            elif op == 'B':
                p2_chunk(tl, cnt['B'], cnt['B'], RA, TQ - RA)
                cnt['B'] += 1
            elif op == 'Z':
                anchor(m_buf)
            elif op == 'Ze':
                last[0] = last_e[0]
                anchor(m_buf)
            elif op == 'Zl':
                anchor_l()
            elif op == 'Zm':
                anchor_m()
            elif op == 'S':
                saved = last[0]
            elif op == 'R':
                last[0] = saved
            elif op == 'Mb':
                merge_b([(dyn(NS - 2), 0, TQ, 0), (t9, TQ, LAG, TQ + LAG)])
                out_copy(0, (NS - 2) * TQ, TQ).start()
                out_copy(0, NT * TQ, LAG).start()
            elif op == 'Mc':
                merge_a([(tl, 0, TQ + LAG, Y2)])
            elif op == 'Ga':
                p2_fin(tl, 0, RA)
            elif op == 'Gb':
                p2_fin(tl, RA, TQ - RA)
            elif op == 'M1':
                merge_b([(tl, 0, RA, Y2)])
                out_copy(0, (NS - 1) * TQ, RA).start()
            elif op == 'M2':
                merge_b([(tl, RA, TQ + LAG - RA, Y2 + RA)])
                out_copy(0, (NS - 1) * TQ + RA, TQ + LAG - RA).start()
            else:
                raise ValueError(op)

    for bi, ops in enumerate(' '.join(ORDERL).split('|')):
        pl.when(z < 1 + bi)(functools.partial(last_block, ops.split()))
    assert cnt['A'] == NC and cnt['B'] == NC

    nrows = (NITER - 1) * (TQ - LAG) + sum(LAG for s in range(2, NITER) if s != NT + 1) + 3 * TQ + 2 * LAG
    out_copy(0, LAG, nrows).wait()


@jax.jit
def pallas_standalone__conformer_family_e_branchformer__speech_kernel(
    x, w_qkv, w_att_out, w_mlp_in, dw_csgu, w_mlp_out, dw_merge, w_merge):
    B, T, D = x.shape
    K = dw_csgu.shape[0]
    TQ = 400
    TP = 4096
    CK = 256
    G = D // 128
    NT = T // TQ
    RB = (B * NT + 1) * SLOT
    out = pl.pallas_call(
        functools.partial(kernel, B=B, T=T, D=D, K=K, TQ=TQ, TP=TP, CK=CK),
        in_specs=[pl.BlockSpec(memory_space=pl.ANY)] * 8,
        out_specs=pl.BlockSpec(memory_space=pl.ANY),
        out_shape=jax.ShapeDtypeStruct((B * T, D), x.dtype),
        scratch_shapes=[
            pltpu.VMEM((B * T + 32, D), BF16),
            pltpu.VMEM((B * T + 32, D), BF16),
            pltpu.VMEM((B * TP // 2 + 16, D), U32),
            pltpu.VMEM((D // 2, D), U32),
            pltpu.VMEM((D // 2, D), U32),
            pltpu.VMEM((D // 2, 2 * D), U32),
            pltpu.VMEM((D // 2, D), U32),
            pltpu.VMEM((D, D), U32),
            pltpu.VMEM((3 * G, 32, 8, 128), F32),
            pltpu.VMEM((G, RB, 128), F32),
            pltpu.VMEM((2 * G, RB, 128), F32),
            pltpu.VMEM((B * T, D), F32),
            pltpu.VMEM((TQ, TP), F32),
            pltpu.VMEM((TQ + 16, 128), F32),
            pltpu.VMEM((256, D), U32),
            pltpu.VMEM((128, 640), U32),
            pltpu.VMEM((B * 16 * 64, 640), U32),
            pltpu.VMEM((TQ + 16, 128), F32),
            pltpu.VMEM((TQ + 16, 128), F32),
            pltpu.VMEM((TQ, D), F32),
            pltpu.VMEM((2 * TQ + 4 * LAG, D), F32),
            pltpu.VMEM(w_qkv.shape, BF16),
            pltpu.VMEM(w_att_out.shape, BF16),
            pltpu.VMEM(w_mlp_in.shape, BF16),
            pltpu.VMEM(dw_csgu.shape, BF16),
            pltpu.VMEM(w_mlp_out.shape, BF16),
            pltpu.VMEM(dw_merge.shape, BF16),
            pltpu.VMEM(w_merge.shape, BF16),
            pltpu.SMEM((1,), jnp.int32),
            pltpu.SemaphoreType.DMA((max(GRP.values()) + 1,)),
            pltpu.SemaphoreType.DMA,
        ],
        compiler_params=pltpu.CompilerParams(vmem_limit_bytes=110 * 1024 * 1024, disable_bounds_checks=True),
    )(x.reshape(B * T, D), w_qkv, w_att_out, w_mlp_in, dw_csgu, w_mlp_out, dw_merge, w_merge)
    return out.reshape(B, T, D)
```

```python
import functools
NITER = 18 - 1
SKIP = ''
STOP = ''
CV = 10
CQ = 4
MPV = 2
VSEQ = [int(c) for c in '3415726']
STR = 1
RSQ = 1
REM = 2
import jax
import jax.numpy as jnp
from jax import lax
import jax.experimental.pallas as pl
import jax.experimental.pallas.tpu as pltpu

F32 = jnp.float32
BF16 = jnp.bfloat16
U32 = jnp.uint32
LOG2E = 1.4426950408889634
NT_DIMS = (((1,), (1,)), ((), ()))
SLOT = 448
LAG = 16

PRO0 = 'sx0 sw0 | x0 sx1 sw1 sx2 n0 w0 sx3 sx4 A q K K x1 w1 x2 sx5 sw3 sw4 sx6 sx7 p1 n1 n2 H0 K H1 K x3 x4 x5 w3 w4 sw2 sw5 sw6 sw7 sx8 p3 p4 K Zg n3 n4 n5 K K K K K K L0 x6 x7 w2 w5 w6 w7 x8 sx9 n6 n7 p5 p6 K H2 K K K K p2'.split()
GRP = {}
_g, _prev = -1, False
for _op in PRO0:
    _is_wait = _op[0] in 'xw'
    if _is_wait:
        if not _prev:
            _g += 1
        GRP[_op] = _g
    _prev = _is_wait
GRP['x9'] = _g + 1


def _pk(x):
    return pltpu.bitcast(x, U32)


def _upk(x):
    return pltpu.bitcast(x, BF16)


def _ln(x, eps=1e-5):
    m = jnp.mean(x, axis=-1, keepdims=True)
    xc = x - m
    v = jnp.mean(xc * xc, axis=-1, keepdims=True)
    if RSQ == 0:
        return xc * lax.rsqrt(v + eps)
    return xc * jnp.exp2(jnp.log(v + eps) * (-0.5 * LOG2E))


def _gelu(x):
    c = 0.7978845608028654
    hx = 0.5 * x
    return hx + hx * jnp.tanh(x * (c + (c * 0.044715) * (x * x)))


def _ds(base, off, n, align):
    if isinstance(base, int):
        return pl.ds(base + off, n)
    a = align
    while off % a:
        a //= 2
    return pl.ds(pl.multiple_of(base + off, a), n) if a > 1 else pl.ds(base + off, n)


def _conv(buf_ref, g, w_ref, wg, base, off, nrows, K):
    outs = []
    nv = nrows // 8
    v0 = 0
    while v0 < nv:
        V = min(CV, nv - v0)
        acc = None
        for p in range(8):
            taps = list(range(p, K, 8))
            nq = V + len(taps) - 1
            slab = buf_ref[g, _ds(base, off + 8 * v0 + p - K // 2, 8 * nq, 32), :].reshape(nq, 8, 128)
            for qi, i in enumerate(taps):
                term = slab[qi:qi + V] * w_ref[wg, i][None]
                acc = term if acc is None else acc + term
        outs.append(acc.reshape(8 * V, 128))
        v0 += V
    return jnp.concatenate(outs, axis=0) if len(outs) > 1 else outs[0]


def _conv2(buf_ref, g, ge, w_ref, wg, base, off, nrows, K):
    nq = nrows // 32
    outs = []
    q0 = 0
    while q0 < nq:
        Q = min(CQ, nq - q0)
        am = a0 = a1 = None
        for i in [p + 8 * h for p in range(8) for h in range(2)]:
            r = off + 32 * q0 + i - K // 2 + 16
            xs = buf_ref[g, _ds(base, r, 32 * Q - 16, 32), :]
            xs = jnp.concatenate([xs[32 * k:32 * k + 16] for k in range(Q)], axis=0).reshape(2 * Q, 8, 128)
            t = xs * w_ref[wg, 32 + i][None]
            am = t if am is None else am + t
            if i + 16 < K:
                es = buf_ref[ge, _ds(base, r, 32 * Q, 32), :]
                e2 = jnp.concatenate([es[32 * k + 16:32 * k + 32] for k in range(Q)], axis=0).reshape(2 * Q, 8, 128)
                t = e2 * w_ref[wg, i + 16][None]
                a1 = t if a1 is None else a1 + t
            else:
                es = buf_ref[ge, _ds(base, r, 32 * Q - 16, 32), :]
            e1 = jnp.concatenate([es[32 * k:32 * k + 16] for k in range(Q)], axis=0).reshape(2 * Q, 8, 128)
            t = e1 * w_ref[wg, i][None]
            a0 = t if a0 is None else a0 + t
        y0 = (am - a0).reshape(16 * Q, 128)
        y1 = (am + a1).reshape(16 * Q, 128)
        for k in range(Q):
            outs += [y0[16 * k:16 * k + 16], y1[16 * k:16 * k + 16]]
        q0 += Q
    if nrows % 32:
        outs.append(_conv(buf_ref, g, w_ref, wg, base, off + 32 * nq, nrows - 32 * nq, K))
    return jnp.concatenate(outs, axis=0) if len(outs) > 1 else outs[0]


class Tile:
    def __init__(self, t, NT, NS, TQ, TP, T):
        if isinstance(t, int):
            b = t // NT
            first, last = t % NT == 0, t % NT == NT - 1
            self.prev = (NS if first else t - 1) * SLOT
            self.next = (NS if last else t + 1) * SLOT
        else:
            b = (t >= NT).astype(jnp.int32)
            first = jnp.logical_or(t == 0, t == NT)
            last = jnp.logical_or(t == NT - 1, t == NS - 1)
            self.prev = jnp.where(first, NS, t - 1) * SLOT
            self.next = jnp.where(last, NS, t + 1) * SLOT
        self.cb = t * SLOT
        self.fb = t * TQ
        self.ab = t * (TQ // 2) + b * ((TP - T) // 2)
        self.kb = b * (TP // 2)
        self.cbk = b * (16 * 64)


def kernel(x_hbm, wqkv_hbm, wao_hbm, wmi_hbm, dwc_hbm, wmo_hbm, dwm_hbm, wm_hbm, o_hbm,
           x_buf, o_buf, xa_ref, wa_p, wvo_p, wmi_p, wmo_p, wm_p, dw_f, g_buf, m_buf, u_ref,
           s_ref, mx_ref, q_ref, qc_ref, kc_ref, mp_ref, lp_ref, acc_ref, acc7_ref, y_ref,
           wqkv_ref, wao_ref, wmi_ref, dwc_ref, wmo_ref, dwm_ref, wm_ref,
           zoff, sem_in, sem_out,
           *, B, T, D, K, TQ, TP, CK):
    NT = T // TQ
    NS = B * NT
    G = D // 128
    NC = TP // CK
    LT = CK // 128
    assert B == 2
    last = [None]
    last_e = [None]
    JUNK = NS * SLOT + 64

    def tile(t):
        return Tile(t, NT, NS, TQ, TP, T)

    NU = TP // 512

    def x_copy(u):
        r0 = u * 512 if u < NU else (T if u == NU else T + 512)
        n = min(512, T - r0) if u < NU else (512 if u == NU else T - 512)
        return pltpu.make_async_copy(x_hbm.at[pl.ds(r0, n), :], x_buf.at[pl.ds(LAG + r0, n), :], sem_in.at[GRP['x%d' % u]])

    w_pairs = [(wqkv_hbm.at[:, 0:2 * D], wqkv_ref.at[:, 0:2 * D]), (wmi_hbm, wmi_ref), (wao_hbm, wao_ref), (dwc_hbm, dwc_ref),
               (wmo_hbm, wmo_ref), (dwm_hbm, dwm_ref), (wm_hbm, wm_ref), (wqkv_hbm.at[:, 2 * D:3 * D], wqkv_ref.at[:, 2 * D:3 * D])]

    def w_copy(k):
        return pltpu.make_async_copy(w_pairs[k][0], w_pairs[k][1], sem_in.at[GRP['w%d' % k]])

    def dma_start(op):
        if STOP == 'pro' and op == 'sx9':
            return
        if op[1] == 'x':
            x_copy(int(op[2:])).start()
        elif op == 'swr':
            for k in range(2, len(w_pairs)):
                w_copy(k).start()
        else:
            w_copy(int(op[2:])).start()

    PRO = list(PRO0)
    for op in PRO[:PRO.index('|')]:
        dma_start(op)
    PRO = PRO[PRO.index('|') + 1:]

    zoff[0] = 0
    z16 = jnp.zeros((16, 128), F32)
    for b in range(B):
        for gi in range(G):
            g_buf[gi, b * NT * SLOT:b * NT * SLOT + 16, :] = z16
            g_buf[gi, ((b + 1) * NT - 1) * SLOT + 416:((b + 1) * NT - 1) * SLOT + 432, :] = z16
        for gi in range(2 * G):
            m_buf[gi, b * NT * SLOT:b * NT * SLOT + 16, :] = z16
            m_buf[gi, b * NT * SLOT + 16:b * NT * SLOT + 32, :] = z16
            m_buf[2 * G + gi, b * NT * SLOT + 16:b * NT * SLOT + 32, :] = z16
            m_buf[gi, ((b + 1) * NT - 1) * SLOT + 432:((b + 1) * NT - 1) * SLOT + 448, :] = z16
    x_buf[0:LAG, :] = jnp.zeros((LAG, D), BF16)
    x_buf[LAG + B * T:LAG + B * T + TP - T, :] = jnp.zeros((TP - T, D), BF16)
    q_ref[TQ // 2:, :] = jnp.zeros((q_ref.shape[0] - TQ // 2, D), U32)

    def prep_a():
        a = lax.dot_general(wqkv_ref[:, 0:D], wqkv_ref[:, D:2 * D], NT_DIMS, preferred_element_type=F32)
        wa_p[...] = _pk((a * (D ** -0.5 * LOG2E)).astype(BF16))

    def prep(k):
        if k == 1:
            wmi_p[...] = _pk(wmi_ref[...])
        elif k == 2:
            wvo_p[...] = _pk(jnp.dot(wqkv_ref[:, 2 * D:3 * D], wao_ref[...], preferred_element_type=F32).astype(BF16))
        elif k == 4:
            wmo_p[...] = _pk(wmo_ref[...])
        elif k == 6:
            wm_p[...] = _pk(wm_ref[...])
        elif k in (3, 5):
            dw = (dwc_ref if k == 3 else dwm_ref)[...].astype(F32)
            g0 = 2 * G if k == 3 else 0
            if k == 5:
                row = lax.broadcasted_iota(jnp.int32, dw.shape, 0)
                dw = jnp.where(row == K // 2, dw + 1.0, dw)
            for gi in range(dw.shape[1] // 128):
                for i in range(K):
                    dw_f[g0 + gi, i] = jnp.broadcast_to(dw[i:i + 1, gi * 128:(gi + 1) * 128], (8, 128))
                for i in range(16):
                    v = dw_f[g0 + gi, i]
                    dw_f[g0 + gi, 32 + i] = v + dw_f[g0 + gi, i + 16] if i + 16 < K else v

    def ln_unit(base, off, n):
        xk = _ln(x_buf[_ds(base, off, n, 16), :].astype(F32))
        if n < 512:
            xk = jnp.concatenate([xk, jnp.zeros((512 - n, D), F32)], axis=0)
        vs = []
        for c in range(2):
            r = c * 256
            alo, ahi = xk[r:r + 128, 0:128], xk[r:r + 128, 128:256]
            blo, bhi = xk[r + 128:r + 256, 0:128], xk[r + 128:r + 256, 128:256]
            vs.append(jnp.concatenate([alo + bhi, ahi - bhi, blo - alo, alo + ahi, blo + bhi], axis=1))
        return _pk(xk.astype(BF16)), _pk(jnp.concatenate(vs, axis=0).astype(BF16))

    def xq_of(t):
        return _upk(xa_ref[_ds(t.ab, 0, TQ // 2, 8), :])

    def xa_chunk(t, j):
        return _upk(xa_ref[_ds(t.kb, j * CK // 2, CK // 2, 16), :])

    R1 = 208
    R2 = TQ - R1

    def qproj(t, combos=True):
        qf = jnp.dot(xq_of(t), _upk(wa_p[...]), preferred_element_type=F32)
        last[0] = qf[0:16, 0:128]
        q_ref[0:TQ // 2, :] = _pk(qf.astype(BF16))
        if STR and combos:
            a11, a12 = qf[0:R1, 0:128], qf[0:R1, 128:256]
            a21, a22 = qf[R1:TQ, 0:128], qf[R1:TQ, 128:256]
            cat = lambda u, v: jnp.concatenate([u, v], axis=0)
            qc_ref[0:R1 // 2, 0:384] = _pk(jnp.concatenate(
                [cat(a11[0:R2] + a22, a11[R2:]), a12 - a11, cat(a12[0:R2] + a22, a12[R2:])], axis=1).astype(BF16))
            qc_ref[0:R2 // 2, 384:640] = _pk(jnp.concatenate([a21 - a22, a11[0:R2] + a21], axis=1).astype(BF16))

    def l1(t):
        hp = jnp.dot(xq_of(t), _upk(wmi_p[...]), preferred_element_type=F32)
        last[0] = hp[0:16, 0:128]
        h = _gelu(hp)
        u_ref[_ds(t.fb, 0, TQ, 16), :] = h[:, :D]
        g = _ln(h[:, D:])
        halo = jnp.concatenate([g_buf[gi, _ds(t.cb, 0, 16, 32), :] for gi in range(G)], axis=1)
        e = jnp.concatenate([g[0:16] - halo, g[16:] - g[:TQ - 16], -g[TQ - 16:]], axis=0)
        for gi in range(G):
            g_buf[gi, _ds(t.prev, 16 + TQ, 16, 32), :] = g[0:16, gi * 128:(gi + 1) * 128]
            g_buf[G + gi, _ds(t.prev, 16 + TQ, 16, 32), :] = e[0:16, gi * 128:(gi + 1) * 128]
        for gi in range(G):
            g_buf[gi, _ds(t.cb, 16, TQ, 32), :] = g[:, gi * 128:(gi + 1) * 128]
            g_buf[G + gi, _ds(t.cb, 16, TQ + 16, 32), :] = e[:, gi * 128:(gi + 1) * 128]
        for gi in range(G):
            g_buf[gi, _ds(t.next, 0, 16, 32), :] = g[TQ - 16:TQ, gi * 128:(gi + 1) * 128]

    def m_store(t, g0, v, r0=0):
        n = v.shape[0]
        halo = jnp.concatenate([m_buf[g0 + gi, _ds(t.cb, 16 + r0, 16, 32), :] for gi in range(G)], axis=1)
        parts = [v[0:16] - halo, v[16:] - v[:n - 16]]
        if r0 + n == TQ:
            parts.append(-v[n - 16:])
        e = jnp.concatenate(parts, axis=0)
        for gi in range(G):
            m_buf[g0 + gi, _ds(t.cb, 32 + r0, n, 32), :] = v[:, gi * 128:(gi + 1) * 128]
            m_buf[2 * G + g0 + gi, _ds(t.cb, 32 + r0, e.shape[0], 32), :] = e[:, gi * 128:(gi + 1) * 128]
        if n == TQ:
            for gi in range(G):
                m_buf[g0 + gi, _ds(t.next, 0, 32, 32), :] = v[TQ - 32:TQ, gi * 128:(gi + 1) * 128]
                m_buf[2 * G + g0 + gi, _ds(t.next, 16, 16, 32), :] = e[TQ - 16:TQ, gi * 128:(gi + 1) * 128]

    def l2(t):
        gc = jnp.concatenate([_conv2(g_buf, gi, G + gi, dw_f, 2 * G + gi, t.cb, 16, TQ, K) for gi in range(G)], axis=-1)
        u = u_ref[_ds(t.fb, 0, TQ, 16), :]
        loc = jnp.dot((u * gc).astype(BF16), _upk(wmo_p[...]), preferred_element_type=F32)
        m_store(t, G, loc)

    def merge_half(half, pieces):
        lhs = []
        for (t, off, nrows, yo) in pieces:
            r = 32 - LAG + off
            ms = [_conv2(m_buf, gi, 2 * G + gi, dw_f, gi, t.cb, r, nrows, K)
                  for gi in range(half * G, (half + 1) * G)]
            lhs.append(jnp.concatenate(ms, axis=-1))
        lhs = lhs[0] if len(lhs) == 1 else jnp.concatenate(lhs, axis=0)
        return jnp.dot(lhs.astype(BF16), _upk(wm_p[half * D // 2:(half + 1) * D // 2, :]), preferred_element_type=F32)

    def merge_a(pieces):
        y = merge_half(1, pieces)
        r = 0
        for (t, off, nrows, yo) in pieces:
            y_ref[yo:yo + nrows, :] = x_buf[_ds(t.fb, off, nrows, 16), :].astype(F32) + y[r:r + nrows]
            r += nrows

    def merge_b(pieces):
        y = merge_half(0, pieces)
        r = 0
        for (t, off, nrows, yo) in pieces:
            o_buf[_ds(t.fb, off, nrows, 16), :] = (y_ref[yo:yo + nrows, :] + y[r:r + nrows]).astype(BF16)
            r += nrows

    def p1_pair(t, js, pos):
        nt = lambda a, b: lax.dot_general(_upk(a), _upk(b), NT_DIMS, preferred_element_type=F32)
        kc = lambda j, i: kc_ref[_ds(t.cbk, j * 64, 64, 32), i * 128:(i + 1) * 128]
        b11 = lambda j: xa_ref[_ds(t.kb, j * 128, 64, 16), 0:128]
        b22 = lambda j: xa_ref[_ds(t.kb, j * 128 + 64, 64, 16), 128:256]
        h1, h2, hs = R1 // 2, R2 // 2, 48
        f = {
            1: lambda j: nt(qc_ref[0:h1, 0:128], kc(j, 0)),
            11: lambda j: nt(qc_ref[0:hs, 0:128], kc(j, 0)),
            12: lambda j: nt(qc_ref[hs:h1, 0:128], kc(j, 0)),
            2: lambda j: nt(q_ref[0:h1, 0:128], kc(j, 4)),
            3: lambda j: nt(qc_ref[0:h2, 384:512], b11(j)),
            4: lambda j: nt(qc_ref[0:h1, 128:256], b22(j)),
            5: lambda j: nt(q_ref[h1:TQ // 2, 128:256], kc(j, 3)),
            6: lambda j: nt(qc_ref[0:h2, 512:640], kc(j, 2)),
            7: lambda j: nt(qc_ref[0:h1, 256:384], kc(j, 1)),
            71: lambda j: nt(qc_ref[0:hs, 256:384], kc(j, 1)),
            72: lambda j: nt(qc_ref[hs:h1, 256:384], kc(j, 1)),
        }
        a, b = js
        cat0 = lambda u, v: jnp.concatenate([u, v], axis=0)

        def mx_upd(ml, final=False):
            if final:
                return jnp.maximum(mp_ref[0:TQ], ml)
            mp_ref[0:TQ] = jnp.maximum(mp_ref[0:TQ], ml)

        assert pos > 0
        for j, order in ((a, (2, 4, 3, 5)), (b, (3, 5, 2, 4))):
            m = {k: f[k](j) for k in order}
            if j == a:
                last[0] = m[2][0:16]
            c0 = j * CK
            c12 = m[2] + m[4]
            c21 = m[3] + m[5]
            s_ref[0:R1, c0 + 128:c0 + 256] = c12
            s_ref[R1:TQ, c0:c0 + 128] = c21
            s_ref[0:R1, c0:c0 + 128] = cat0(m[4][0:R2] - m[5], m[4][R2:])
            s_ref[R1:TQ, c0 + 128:c0 + 256] = m[3] - m[2][0:R2]
            if MPV == 0:
                mx_upd(cat0(c12, c21))
        reload = lambda j: cat0(s_ref[0:R1, j * CK + 128:j * CK + 256], s_ref[R1:TQ, j * CK:j * CK + 128])
        reload2 = lambda j: cat0(s_ref[0:R1, j * CK:j * CK + 128], s_ref[R1:TQ, j * CK + 128:j * CK + 256])
        m1, m7, m6, m6b = f[1](a), f[7](a), f[6](a), f[6](b)
        c0 = a * CK
        c11 = s_ref[0:R1, c0:c0 + 128] + (m1 + m7)
        c22 = s_ref[R1:TQ, c0 + 128:c0 + 256] + (m1[0:R2] + m6)
        s_ref[0:R1, c0:c0 + 128] = c11
        s_ref[R1:TQ, c0 + 128:c0 + 256] = c22
        if MPV == 0:
            mx_upd(cat0(c11, c22))
        elif MPV == 1:
            mx_upd(jnp.maximum(cat0(c11, c22), reload(a)))
        c0 = b * CK
        s_ref[R1:TQ, c0 + 128:c0 + 256] += m6b
        m11, m71, m12, m72 = f[11](b), f[71](b), f[12](b), f[72](b)
        m1, m7 = cat0(m11, m12), cat0(m71, m72)
        c11 = s_ref[0:R1, c0:c0 + 128] + (m1 + m7)
        c22 = s_ref[R1:TQ, c0 + 128:c0 + 256] + m1[0:R2]
        s_ref[0:R1, c0:c0 + 128] = c11
        s_ref[R1:TQ, c0 + 128:c0 + 256] = c22
        ml = cat0(c11, c22)
        if MPV >= 1:
            ml = jnp.maximum(ml, reload(b))
        if MPV == 2:
            ml = jnp.maximum(ml, jnp.maximum(reload(a), reload2(a)))
        return mx_upd(ml, pos >= NC - 2)

    def p1_chunk(t, j, pos, strassen=True):
        q = _upk(q_ref[0:TQ // 2, :])
        if (j + 1) * CK <= T or REM == 0:
            sj = lax.dot_general(q, xa_chunk(t, j), NT_DIMS, preferred_element_type=F32)
            sts = [sj[:, lt * 128:(lt + 1) * 128] for lt in range(LT)]
            if (j + 1) * CK > T:
                col = lax.broadcasted_iota(jnp.int32, (TQ, 128), 1)
                sts[-1] = jnp.where(col < T % 128, sts[-1], -jnp.inf)
        else:
            nfull = (T - j * CK) // 128
            nrem = T - j * CK - nfull * 128
            assert nfull + 1 == LT and nrem % 16 == 0
            kf = _upk(xa_ref[_ds(t.kb, j * CK // 2, nfull * 64, 16), :])
            if REM == 1:
                sj = lax.dot_general(q, kf, NT_DIMS, preferred_element_type=F32)
            else:
                sj = jnp.concatenate([lax.dot_general(q[0:208], kf, NT_DIMS, preferred_element_type=F32),
                                      lax.dot_general(q[208:TQ], kf, NT_DIMS, preferred_element_type=F32)], axis=0)
            sts = [sj[:, lt * 128:(lt + 1) * 128] for lt in range(nfull)]
            kr = _upk(xa_ref[_ds(t.kb, j * CK // 2 + nfull * 64, nrem // 2, 16), :])
            st = lax.dot_general(kr, _upk(q_ref[...]), NT_DIMS, preferred_element_type=F32)
            st = jnp.concatenate([st, jnp.full((128 - nrem, st.shape[1]), -jnp.inf, F32)], axis=0)
            sts.append(st.T[0:TQ])
        last[0] = sj[0:16, 0:128]
        mloc = None
        for lt in range(LT):
            c0 = j * CK + lt * 128
            s_ref[:, c0:c0 + 128] = sts[lt]
            mloc = sts[lt] if mloc is None else jnp.maximum(mloc, sts[lt])
        if pos == 0:
            mp_ref[0:TQ] = mloc
        elif pos < NC - 1:
            mp_ref[0:TQ] = jnp.maximum(mp_ref[0:TQ], mloc)
        else:
            return jnp.maximum(mp_ref[0:TQ], mloc)

    def p1_fin(mpart, scaled=True):
        m = jnp.max(mpart, axis=-1, keepdims=True)
        if scaled:
            lam = jnp.sum(jnp.exp2(mpart - m), axis=-1, keepdims=True)
            m = m + jnp.log(lam) * LOG2E
        mx_ref[0:TQ] = jnp.broadcast_to(m, (TQ, 128))

    def p2_group(t, js, first):
        cat0 = lambda u, v: jnp.concatenate([u, v], axis=0)
        L = {k: [] for k in range(1, 8)}
        l1 = l2 = None
        for j in js:
            c0 = j * CK
            a11 = jnp.exp2(s_ref[0:R1, c0:c0 + 128] - mx_ref[0:R1])
            a12 = jnp.exp2(s_ref[0:R1, c0 + 128:c0 + 256] - mx_ref[0:R1])
            a21 = jnp.exp2(s_ref[R1:TQ, c0:c0 + 128] - mx_ref[R1:TQ])
            a22 = jnp.exp2(s_ref[R1:TQ, c0 + 128:c0 + 256] - mx_ref[R1:TQ])
            s1 = a11 + a12
            s2 = a21 + a22
            l1 = s1 if l1 is None else l1 + s1
            l2 = s2 if l2 is None else l2 + s2
            L[1].append(cat0(a11[0:R2] + a22, a11[R2:]))
            L[2].append(s2)
            L[3].append(a11)
            L[4].append(a22)
            L[5].append(s1)
            L[6].append(a21 - a11[0:R2])
            L[7].append(cat0(a12[0:R2] - a22, a12[R2:]))
        kc = lambda j, i: kc_ref[_ds(t.cbk, j * 64, 64, 32), i * 128:(i + 1) * 128]
        W = {
            1: lambda j: kc(j, 0),
            2: lambda j: xa_ref[_ds(t.kb, j * 128, 64, 16), 0:128],
            3: lambda j: kc(j, 1),
            4: lambda j: kc(j, 2),
            5: lambda j: xa_ref[_ds(t.kb, j * 128 + 64, 64, 16), 128:256],
            6: lambda j: kc(j, 3),
            7: lambda j: kc(j, 4),
        }
        for k in VSEQ:
            lhs = jnp.concatenate(L[k], axis=1).astype(BF16)
            rhs = _upk(jnp.concatenate([W[k](j) for j in js], axis=0))
            mk = jnp.dot(lhs, rhs, preferred_element_type=F32)
            last[0] = mk[0:16]
            n = mk.shape[0]
            if first:
                acc7_ref[k, 0:n] = mk
            else:
                acc7_ref[k, 0:n] += mk
        lloc = cat0(l1, l2)
        if first:
            lp_ref[0:TQ] = lloc
        else:
            lp_ref[0:TQ] += lloc

    def p2_fin7(t):
        l = jnp.sum(lp_ref[0:TQ], axis=-1, keepdims=True)
        m1, m3, m5, m7 = (acc7_ref[k, 0:R1] for k in (1, 3, 5, 7))
        m2, m4, m6 = (acc7_ref[k, 0:R2] for k in (2, 4, 6))
        c11 = m1 + (m7 - m5)
        c11 = jnp.concatenate([c11[0:R2] + m4, c11[R2:]], axis=0)
        c12 = m3 + m5
        c21 = m2 + m4
        c22 = (m1[0:R2] - m2) + (m3[0:R2] + m6)
        acc = jnp.concatenate([jnp.concatenate([c11, c12], axis=1), jnp.concatenate([c21, c22], axis=1)], axis=0)
        o = (acc * (1.0 / l)).astype(BF16)
        glob = jnp.dot(o, _upk(wvo_p[...]), preferred_element_type=F32)
        m_store(t, 0, glob)

    def p2_chunk(t, j, pos, r0=0, n=TQ):
        ps = []
        lloc = None
        for lt in range(LT):
            c0 = j * CK + lt * 128
            p = jnp.exp2(s_ref[r0:r0 + n, c0:c0 + 128] - mx_ref[r0:r0 + n])
            lloc = p if lloc is None else lloc + p
            ps.append(p)
        pv = jnp.dot(jnp.concatenate(ps, axis=-1).astype(BF16), xa_chunk(t, j), preferred_element_type=F32)
        last[0] = pv[0:16, 0:128]
        last_e[0] = lloc[0:16]
        if pos == 0:
            lp_ref[r0:r0 + n] = lloc
            acc_ref[r0:r0 + n] = pv
        else:
            lp_ref[r0:r0 + n] += lloc
            acc_ref[r0:r0 + n] += pv

    def p2_fin(t, r0=0, n=TQ):
        l = jnp.sum(lp_ref[r0:r0 + n], axis=-1, keepdims=True)
        o = (acc_ref[r0:r0 + n] * (1.0 / l)).astype(BF16)
        glob = jnp.dot(o, _upk(wvo_p[...]), preferred_element_type=F32)
        m_store(t, 0, glob, r0)

    def anchor(buf):
        zrow = pl.multiple_of(zoff[0], 8)
        buf[0, pl.ds(zrow + JUNK, 8), :] = last[0][0:8]

    def anchor_l():
        zrow = pl.multiple_of(zoff[0], 8)
        lp_ref[pl.ds(zrow + TQ, 8), :] = last[0][0:8]

    def anchor_m():
        zrow = pl.multiple_of(zoff[0], 8)
        mx_ref[pl.ds(zrow + TQ, 8), :] = last[0][0:8]

    def anchor_x():
        zrow = pl.multiple_of(zoff[0], 16)
        x_buf[pl.ds(zrow + B * T + LAG + TP - T, 16), 0:128] = last[0].astype(BF16)

    def out_copy(base, off, n):
        return pltpu.make_async_copy(o_buf.at[_ds(base, off, n, 16), :], o_hbm.at[_ds(base, off - LAG, n, 16), :], sem_out)

    DEF = 'q Z Zg W W Mb K Ks D W Ma W Zl L H KK KK KK Zx KK KK N KK KK Ns G7'
    ORDER = DEF.split()
    ORDERP = 'q Z Zg W W Mb K Ks W Ma W Zl L KK KK KK KK KK KK KK G7'.split()
    ORDERL = 'A Z A A A A A A A A A A A Mb A A A A Zl Mc Ga | B Z S B B R Zm B S B B R Zm B B B B B B B B B B Zl M1 Gb M2'.split()

    RPOS = 3
    CORD = list(range(NC - 1))
    CORD.insert(RPOS, NC - 1)
    CORDP = list(range(NC - 1))
    CORDP.insert(NC - 3, NC - 1)

    def step(order, pb, pa, t0, tp, th, tn, dma=None, pc=None, cc=None):
        CORD = []
        nxt = 0
        for op in order:
            if op == 'KK':
                CORD += [nxt, nxt + 1]
                nxt += 2
            elif op == 'Ks':
                CORD.append(NC - 2)
            elif op == 'K':
                CORD.append(NC - 1)
        assert order.count('V') + 4 * order.count('W') == NC and sorted(CORD) == list(range(NC))
        mpart = None
        jv = jk = 0
        for op in order:
            if op in SKIP.split(','):
                continue
            if op == 'q':
                qproj(tp)
            elif op == 'V':
                p2_chunk(t0, CORD[jv], jv)
                jv += 1
            elif op == 'W':
                p2_group(t0, CORD[jv:jv + 4], jv == 0)
                jv += 4
            elif op == 'G7':
                p2_fin7(t0)
            elif op == 'K':
                assert jk < jv
                mpart = p1_chunk(tp, CORD[jk], jk)
                jk += 1
            elif op == 'KK':
                assert jk + 1 < jv and CORD[jk] < NC - 1 and CORD[jk + 1] < NC - 1
                mpart = p1_pair(tp, (CORD[jk], CORD[jk + 1]), jk)
                jk += 2
            elif op == 'Ks':
                assert jk < jv
                mpart = p1_chunk(tp, CORD[jk], jk, False)
                jk += 1
            elif op == 'Z':
                anchor(m_buf)
            elif op == 'Zg':
                anchor(g_buf)
            elif op == 'Zx':
                anchor_x()
            elif op == 'Zl':
                anchor_l()
            elif op == 'Ma':
                merge_a(pa)
            elif op == 'Mc':
                merge_a(pc)
            elif op == 'Mb':
                merge_b(pb)
            elif op == 'H':
                l1(th)
            elif op == 'L':
                l2(tp)
            elif op == 'N':
                xa_n, kc_n = ln_unit(tn * 512, LAG + T, 512)
            elif op == 'Ns':
                xa_ref[_ds(tn * 256, TP // 2, 256, 256), :] = xa_n
                kc_ref[_ds(tn * 128, 16 * 64, 128, 128), :] = kc_n
            elif op == 'G':
                p2_fin(t0)
            elif op == 'D':
                dma()

            else:
                raise ValueError(op)
        if tp is not None:
            p1_fin(mpart)

    def do_ln(u):
        xa_ref[u * 256:(u + 1) * 256, :], kc_ref[u * 128:(u + 1) * 128, :] = ln_unit(0, LAG + u * 512, min(512, T - u * 512))

    jk = 0
    nln = 0
    for op in PRO:
        if op == 'STOP':
            return
        if op[0] == 's':
            dma_start(op)
        elif op[0] == 'x':
            x_copy(int(op[1:])).wait()
        elif op[0] == 'n':
            do_ln(int(op[1:]))
            nln = max(nln, int(op[1:]) + 1)
        elif op[0] == 'w':
            w_copy(int(op[1:])).wait()
        elif op[0] == 'p':
            prep(int(op[1:]))
        elif op == 'A':
            prep_a()
        elif op == 'q':
            qproj(tile(0), False)
        elif op == 'K':
            assert nln * 512 >= (CORDP[jk] + 1) * CK
            mpart = p1_chunk(tile(0), CORDP[jk], jk, False)
            jk += 1
        elif op[0] == 'H':
            l1(tile(int(op[1:])))
        elif op == 'L0':
            l2(tile(0))
        elif op == 'Zg':
            anchor(g_buf)
        elif op == 'Zx':
            anchor_x()
        else:
            raise ValueError(op)
    assert jk == NC
    p1_fin(mpart)
    if STOP == 'pro':
        return

    DEF2 = ' '.join(o for o in ORDER if o not in ('N', 'Ns', 'Zx'))
    ORDER2 = DEF2.split()

    def body(order, s, c):
        if 'N' in order:
            @pl.when(s == 1)
            def _():
                x_copy(NU + 1).wait()

        w = jnp.maximum(s - 1, 0)
        fb = w * TQ

        def dma():
            @pl.when(s > 0)
            def _():
                out_copy(fb, LAG, TQ - LAG).start()

            @pl.when(jnp.logical_and(s > 1, s != NT + 1))
            def _():
                out_copy(fb, 0, LAG).start()

        step(order, [(tile(w), 0, TQ, 0)], [(tile(s), 0, TQ, 0)], tile(s), tile(s + 1), tile(s + 3), s, dma)
        return c
    lax.fori_loop(0, NU, functools.partial(body, ORDER), 0)
    lax.fori_loop(NU, NITER, functools.partial(body, ORDER2), 0)

    z = zoff[0]
    t9 = tile(NT - 1)

    tl = tile(NS - 1)
    Y2 = TQ + 3 * LAG

    def body2(s, c):
        step(ORDERP, [(tile(s - 1), 0, TQ, 0)], [(tile(s), 0, TQ, 0), (t9, TQ, LAG, TQ + LAG)],
             tile(s), tile(s + 1), None, None)
        out_copy((s - 1) * TQ, 0, TQ).start()
        return c
    lax.fori_loop(NS - 3, NS - 1, body2, 0)

    RA = 288

    cnt = {'A': 0, 'B': 0}

    def last_block(ops):
        dyn = (lambda t: tile(z + t)) if '1' == '1' else tile
        tl = dyn(NS - 1)
        for op in ops:
            if op == 'A':
                p2_chunk(tl, cnt['A'], cnt['A'], 0, RA)
                cnt['A'] += 1
            elif op == 'B':
                p2_chunk(tl, cnt['B'], cnt['B'], RA, TQ - RA)
                cnt['B'] += 1
            elif op == 'Z':
                anchor(m_buf)
            elif op == 'Ze':
                last[0] = last_e[0]
                anchor(m_buf)
            elif op == 'Zl':
                anchor_l()
            elif op == 'Zm':
                anchor_m()
            elif op == 'S':
                saved = last[0]
            elif op == 'R':
                last[0] = saved
            elif op == 'Mb':
                merge_b([(dyn(NS - 2), 0, TQ, 0), (t9, TQ, LAG, TQ + LAG)])
                out_copy(0, (NS - 2) * TQ, TQ).start()
                out_copy(0, NT * TQ, LAG).start()
            elif op == 'Mc':
                merge_a([(tl, 0, TQ + LAG, Y2)])
            elif op == 'Ga':
                p2_fin(tl, 0, RA)
            elif op == 'Gb':
                p2_fin(tl, RA, TQ - RA)
            elif op == 'M1':
                merge_b([(tl, 0, RA, Y2)])
                out_copy(0, (NS - 1) * TQ, RA).start()
            elif op == 'M2':
                merge_b([(tl, RA, TQ + LAG - RA, Y2 + RA)])
                out_copy(0, (NS - 1) * TQ + RA, TQ + LAG - RA).start()
            else:
                raise ValueError(op)

    for bi, ops in enumerate(' '.join(ORDERL).split('|')):
        pl.when(z < 1 + bi)(functools.partial(last_block, ops.split()))
    assert cnt['A'] == NC and cnt['B'] == NC

    nrows = (NITER - 1) * (TQ - LAG) + sum(LAG for s in range(2, NITER) if s != NT + 1) + 4 * TQ + 2 * LAG
    out_copy(0, LAG, nrows).wait()


@jax.jit
def pallas_standalone__conformer_family_e_branchformer__speech_kernel(
    x, w_qkv, w_att_out, w_mlp_in, dw_csgu, w_mlp_out, dw_merge, w_merge):
    B, T, D = x.shape
    K = dw_csgu.shape[0]
    TQ = 400
    TP = 4096
    CK = 256
    G = D // 128
    NT = T // TQ
    RB = (B * NT + 1) * SLOT
    out = pl.pallas_call(
        functools.partial(kernel, B=B, T=T, D=D, K=K, TQ=TQ, TP=TP, CK=CK),
        in_specs=[pl.BlockSpec(memory_space=pl.ANY)] * 8,
        out_specs=pl.BlockSpec(memory_space=pl.ANY),
        out_shape=jax.ShapeDtypeStruct((B * T, D), x.dtype),
        scratch_shapes=[
            pltpu.VMEM((B * T + 32 + TP - T, D), BF16),
            pltpu.VMEM((B * T + 32, D), BF16),
            pltpu.VMEM((B * TP // 2, D), U32),
            pltpu.VMEM((D // 2, D), U32),
            pltpu.VMEM((D // 2, D), U32),
            pltpu.VMEM((D // 2, 2 * D), U32),
            pltpu.VMEM((D // 2, D), U32),
            pltpu.VMEM((D, D), U32),
            pltpu.VMEM((3 * G, 48, 8, 128), F32),
            pltpu.VMEM((2 * G, RB, 128), F32),
            pltpu.VMEM((4 * G, RB, 128), F32),
            pltpu.VMEM((B * T, D), F32),
            pltpu.VMEM((TQ, TP), F32),
            pltpu.VMEM((TQ + 16, 128), F32),
            pltpu.VMEM((256, D), U32),
            pltpu.VMEM((128, 640), U32),
            pltpu.VMEM((B * 16 * 64, 640), U32),
            pltpu.VMEM((TQ + 16, 128), F32),
            pltpu.VMEM((TQ + 16, 128), F32),
            pltpu.VMEM((TQ, D), F32),
            pltpu.VMEM((8, 224, 128), F32),
            pltpu.VMEM((2 * TQ + 4 * LAG, D), F32),
            pltpu.VMEM(w_qkv.shape, BF16),
            pltpu.VMEM(w_att_out.shape, BF16),
            pltpu.VMEM(w_mlp_in.shape, BF16),
            pltpu.VMEM(dw_csgu.shape, BF16),
            pltpu.VMEM(w_mlp_out.shape, BF16),
            pltpu.VMEM(dw_merge.shape, BF16),
            pltpu.VMEM(w_merge.shape, BF16),
            pltpu.SMEM((1,), jnp.int32),
            pltpu.SemaphoreType.DMA((max(GRP.values()) + 1,)),
            pltpu.SemaphoreType.DMA,
        ],
        compiler_params=pltpu.CompilerParams(vmem_limit_bytes=120 * 1024 * 1024, disable_bounds_checks=True),
    )(x.reshape(B * T, D), w_qkv, w_att_out, w_mlp_in, dw_csgu, w_mlp_out, dw_merge, w_merge)
    return out.reshape(B, T, D)
```

```python
import functools
NITER = 18 - 1
SKIP = ''
STOP = ''
ONLY = 'P12BL'
CV = 10
SMM = 'q'
CQ = 4
MPV = 2
VSEQ = [int(c) for c in '3415726']
STR = 1
RSQ = 1
REM = 2
import jax
import jax.numpy as jnp
from jax import lax
import jax.experimental.pallas as pl
import jax.experimental.pallas.tpu as pltpu

F32 = jnp.float32
BF16 = jnp.bfloat16
U32 = jnp.uint32
LOG2E = 1.4426950408889634
NT_DIMS = (((1,), (1,)), ((), ()))
SLOT = 448
LAG = 16

PRO0 = 'sx0 sw0 | x0 sx1 sw1 n0 w0 sx2 sx3 A q x1 w1 sx4 sx5 sw3 sw4 p1 n1 H0 KK0 K2 x2 x3 x4 sx6 sx7 sw2 sw5 sw6 sw7 sx8 n2 H1 K3 Zx n3 KK4 Zx n4 H2 KK6 x5 x6 x7 w3 w4 w2 w5 w6 w7 x8 sx9 p3 p4 KK8 Zg n5 n6 n7 p5 p6 KK10 K12 K15 K13 K14 L0 p2'.split()
GRP = {}
_g, _prev = -1, False
for _op in PRO0:
    _is_wait = _op[0] in 'xw'
    if _is_wait:
        if not _prev:
            _g += 1
        GRP[_op] = _g
    _prev = _is_wait
GRP['x9'] = _g + 1


def _pk(x):
    return pltpu.bitcast(x, U32)


def _upk(x):
    return pltpu.bitcast(x, BF16)


def _ln(x, eps=1e-5):
    m = jnp.mean(x, axis=-1, keepdims=True)
    xc = x - m
    v = jnp.mean(xc * xc, axis=-1, keepdims=True)
    if RSQ == 0:
        return xc * lax.rsqrt(v + eps)
    return xc * jnp.exp2(jnp.log(v + eps) * (-0.5 * LOG2E))


def _gelu(x):
    c = 0.7978845608028654
    hx = 0.5 * x
    return hx + hx * jnp.tanh(x * (c + (c * 0.044715) * (x * x)))


def _ds(base, off, n, align):
    if isinstance(base, int):
        return pl.ds(base + off, n)
    a = align
    while off % a:
        a //= 2
    return pl.ds(pl.multiple_of(base + off, a), n) if a > 1 else pl.ds(base + off, n)


def _conv(buf_ref, g, w_ref, wg, base, off, nrows, K):
    outs = []
    nv = nrows // 8
    v0 = 0
    while v0 < nv:
        V = min(CV, nv - v0)
        acc = None
        for p in range(8):
            taps = list(range(p, K, 8))
            nq = V + len(taps) - 1
            slab = buf_ref[g, _ds(base, off + 8 * v0 + p - K // 2, 8 * nq, 32), :].reshape(nq, 8, 128)
            for qi, i in enumerate(taps):
                term = slab[qi:qi + V] * w_ref[wg, i][None]
                acc = term if acc is None else acc + term
        outs.append(acc.reshape(8 * V, 128))
        v0 += V
    return jnp.concatenate(outs, axis=0) if len(outs) > 1 else outs[0]


def _conv2(buf_ref, g, ge, w_ref, wg, base, off, nrows, K):
    nq = nrows // 32
    outs = []
    q0 = 0
    while q0 < nq:
        Q = min(CQ, nq - q0)
        am = a0 = a1 = None
        for i in [p + 8 * h for p in range(8) for h in range(2)]:
            r = off + 32 * q0 + i - K // 2 + 16
            xs = buf_ref[g, _ds(base, r, 32 * Q - 16, 32), :]
            xs = jnp.concatenate([xs[32 * k:32 * k + 16] for k in range(Q)], axis=0).reshape(2 * Q, 8, 128)
            t = xs * w_ref[wg, 32 + i][None]
            am = t if am is None else am + t
            if i + 16 < K:
                es = buf_ref[ge, _ds(base, r, 32 * Q, 32), :]
                e2 = jnp.concatenate([es[32 * k + 16:32 * k + 32] for k in range(Q)], axis=0).reshape(2 * Q, 8, 128)
                t = e2 * w_ref[wg, i + 16][None]
                a1 = t if a1 is None else a1 + t
            else:
                es = buf_ref[ge, _ds(base, r, 32 * Q - 16, 32), :]
            e1 = jnp.concatenate([es[32 * k:32 * k + 16] for k in range(Q)], axis=0).reshape(2 * Q, 8, 128)
            t = e1 * w_ref[wg, i][None]
            a0 = t if a0 is None else a0 + t
        y0 = (am - a0).reshape(16 * Q, 128)
        y1 = (am + a1).reshape(16 * Q, 128)
        for k in range(Q):
            outs += [y0[16 * k:16 * k + 16], y1[16 * k:16 * k + 16]]
        q0 += Q
    if nrows % 32:
        outs.append(_conv(buf_ref, g, w_ref, wg, base, off + 32 * nq, nrows - 32 * nq, K))
    return jnp.concatenate(outs, axis=0) if len(outs) > 1 else outs[0]


class Tile:
    def __init__(self, t, NT, NS, TQ, TP, T):
        if isinstance(t, int):
            b = t // NT
            first, last = t % NT == 0, t % NT == NT - 1
            self.prev = (NS if first else t - 1) * SLOT
            self.next = (NS if last else t + 1) * SLOT
        else:
            b = (t >= NT).astype(jnp.int32)
            first = jnp.logical_or(t == 0, t == NT)
            last = jnp.logical_or(t == NT - 1, t == NS - 1)
            self.prev = jnp.where(first, NS, t - 1) * SLOT
            self.next = jnp.where(last, NS, t + 1) * SLOT
        self.cb = t * SLOT
        self.fb = t * TQ
        self.ab = t * (TQ // 2) + b * ((TP - T) // 2)
        self.kb = b * (TP // 2)
        self.cbk = b * (16 * 64)


def kernel(x_hbm, wqkv_hbm, wao_hbm, wmi_hbm, dwc_hbm, wmo_hbm, dwm_hbm, wm_hbm, o_hbm,
           x_buf, o_buf, xa_ref, wa_p, wvo_p, wmi_p, wmo_p, wm_p, ws_ref, dw_f, g_buf, m_buf, u_ref,
           s_ref, mx_ref, q_ref, qc_ref, kc_ref, mp_ref, lp_ref, acc_ref, acc7_ref, y_ref,
           wqkv_ref, wao_ref, wmi_ref, dwc_ref, wmo_ref, dwm_ref, wm_ref,
           zoff, sem_in, sem_out,
           *, B, T, D, K, TQ, TP, CK):
    NT = T // TQ
    NS = B * NT
    G = D // 128
    NC = TP // CK
    LT = CK // 128
    assert B == 2
    last = [None]
    last_e = [None]
    JUNK = NS * SLOT + 64

    def tile(t):
        return Tile(t, NT, NS, TQ, TP, T)

    NU = TP // 512

    def x_copy(u):
        r0 = u * 512 if u < NU else (T if u == NU else T + 512)
        n = min(512, T - r0) if u < NU else (512 if u == NU else T - 512)
        return pltpu.make_async_copy(x_hbm.at[pl.ds(r0, n), :], x_buf.at[pl.ds(LAG + r0, n), :], sem_in.at[GRP['x%d' % u]])

    w_pairs = [(wqkv_hbm.at[:, 0:2 * D], wqkv_ref.at[:, 0:2 * D]), (wmi_hbm, wmi_ref), (wao_hbm, wao_ref), (dwc_hbm, dwc_ref),
               (wmo_hbm, wmo_ref), (dwm_hbm, dwm_ref), (wm_hbm, wm_ref), (wqkv_hbm.at[:, 2 * D:3 * D], wqkv_ref.at[:, 2 * D:3 * D])]

    def w_copy(k):
        return pltpu.make_async_copy(w_pairs[k][0], w_pairs[k][1], sem_in.at[GRP['w%d' % k]])

    def dma_start(op):
        if STOP == 'pro' and op == 'sx9':
            return
        if op[1] == 'x':
            x_copy(int(op[2:])).start()
        elif op == 'swr':
            for k in range(2, len(w_pairs)):
                w_copy(k).start()
        else:
            w_copy(int(op[2:])).start()

    PRO = list(PRO0)
    for op in PRO[:PRO.index('|')]:
        dma_start(op)
    PRO = PRO[PRO.index('|') + 1:]

    zoff[0] = 0
    z16 = jnp.zeros((16, 128), F32)
    for b in range(B):
        for gi in range(G):
            g_buf[gi, b * NT * SLOT:b * NT * SLOT + 16, :] = z16
            g_buf[gi, ((b + 1) * NT - 1) * SLOT + 416:((b + 1) * NT - 1) * SLOT + 432, :] = z16
        for gi in range(2 * G):
            m_buf[gi, b * NT * SLOT:b * NT * SLOT + 16, :] = z16
            m_buf[gi, b * NT * SLOT + 16:b * NT * SLOT + 32, :] = z16
            m_buf[2 * G + gi, b * NT * SLOT + 16:b * NT * SLOT + 32, :] = z16
            m_buf[gi, ((b + 1) * NT - 1) * SLOT + 432:((b + 1) * NT - 1) * SLOT + 448, :] = z16
    x_buf[0:LAG, :] = jnp.zeros((LAG, D), BF16)
    x_buf[LAG + B * T:LAG + B * T + TP - T, :] = jnp.zeros((TP - T, D), BF16)
    q_ref[TQ // 2:, :] = jnp.zeros((q_ref.shape[0] - TQ // 2, D), U32)

    def wcomb(unit, w):
        b11, b12, b21, b22 = w[0:128, 0:128], w[0:128, 128:256], w[128:256, 0:128], w[128:256, 128:256]
        ws_ref[unit] = _pk(jnp.concatenate(
            [b11 + b22, b11, b12 - b22, b21 - b11, b22, b11 + b12, b21 + b22], axis=1).astype(BF16))

    def smm(lhs, units):
        n = lhs.shape[0]
        r1 = (n // 2 + 15) // 16 * 16
        r2 = n - r1
        cat0 = lambda u, v: jnp.concatenate([u, v], axis=0) if v.shape[0] else u
        a11, a12, a21, a22 = lhs[0:r1, 0:128], lhs[0:r1, 128:256], lhs[r1:n, 0:128], lhs[r1:n, 128:256]
        p1 = jnp.concatenate([cat0(a11[0:r2] + a22, a11[r2:]), a11, a11 + a12, cat0(a12[0:r2] - a22, a12[r2:])],
                             axis=1).astype(BF16)
        p2 = jnp.concatenate([a21 + a22, a22, a21 - a11[0:r2]], axis=1).astype(BF16)
        Lk = {1: p1[:, 0:128], 3: p1[:, 128:256], 5: p1[:, 256:384], 7: p1[:, 384:512],
              2: p2[:, 0:128], 4: p2[:, 128:256], 6: p2[:, 256:384]}

        def job(u, k, lo=0, hi=None):
            l = Lk[k] if hi is None and lo == 0 else Lk[k][lo:hi]
            return jnp.dot(l, _upk(ws_ref[u, :, (k - 1) * 128:k * 128]), preferred_element_type=F32)
        m = {}
        if len(units) == 1:
            (a,) = units
            tot = (4 * r1 + 3 * r2) // 4
            s1 = (tot - r1) // 16 * 16
            s2 = min((tot - r2 + 15) // 16 * 16, r2)
            for k in (3, 5, 2, 4):
                m[(a, k)] = job(a, k)
            m6a = job(a, 6, 0, s2)
            m1b = job(a, 1, s1, r1)
            m1a = job(a, 1, 0, s1)
            m7a = job(a, 7, 0, s1)
            m7b = job(a, 7, s1, r1)
            m[(a, 6)] = cat0(m6a, job(a, 6, s2, r2)) if s2 < r2 else m6a
            m[(a, 1)] = cat0(m1a, m1b)
            m[(a, 7)] = cat0(m7a, m7b)
        else:
            a, b = units
            hs = (r1 - (r1 - r2)) // 2 // 16 * 16
            for (u, k) in [(a, 3), (a, 5), (a, 2), (a, 4), (b, 2), (b, 4), (b, 3), (b, 5), (a, 1), (a, 7), (a, 6), (b, 6)]:
                m[(u, k)] = job(u, k)
            m11, m71, m12, m72 = job(b, 1, 0, hs), job(b, 7, 0, hs), job(b, 1, hs, r1), job(b, 7, hs, r1)
            m[(b, 1)] = cat0(m11, m12)
            m[(b, 7)] = cat0(m71, m72)
        last[0] = m[(units[0], 3)][0:16]
        outs = []
        for u in units:
            m1, m2, m3, m4, m5, m6, m7 = (m[(u, k)] for k in range(1, 8))
            c12 = m3 + m5
            c21 = m2 + m4
            c11 = cat0(m4 - m5[0:r2], -m5[r2:]) + (m1 + m7)
            c22 = ((m3[0:r2] - m2) + m6) + m1[0:r2]
            outs.append(jnp.concatenate([jnp.concatenate([c11, c12], axis=1), jnp.concatenate([c21, c22], axis=1)], axis=0))
        return outs

    def prep_a():
        a = lax.dot_general(wqkv_ref[:, 0:D], wqkv_ref[:, D:2 * D], NT_DIMS, preferred_element_type=F32)
        a = a * (D ** -0.5 * LOG2E)
        wa_p[...] = _pk(a.astype(BF16))
        if 'q' in SMM:
            wcomb(0, a)

    def prep(k):
        if k == 1:
            wmi_p[...] = _pk(wmi_ref[...])
            if 'H' in SMM:
                wcomb(1, wmi_ref[:, 0:D].astype(F32))
                wcomb(2, wmi_ref[:, D:2 * D].astype(F32))
        elif k == 2:
            wvo = jnp.dot(wqkv_ref[:, 2 * D:3 * D], wao_ref[...], preferred_element_type=F32)
            wvo_p[...] = _pk(wvo.astype(BF16))
            if 'G' in SMM:
                wcomb(6, wvo)
        elif k == 4:
            wmo_p[...] = _pk(wmo_ref[...])
            if 'L' in SMM:
                wcomb(3, wmo_ref[...].astype(F32))
        elif k == 6:
            wm_p[...] = _pk(wm_ref[...])
            if 'M' in SMM:
                wcomb(4, wm_ref[0:D, :].astype(F32))
                wcomb(5, wm_ref[D:2 * D, :].astype(F32))
        elif k in (3, 5):
            dw = (dwc_ref if k == 3 else dwm_ref)[...].astype(F32)
            g0 = 2 * G if k == 3 else 0
            if k == 5:
                row = lax.broadcasted_iota(jnp.int32, dw.shape, 0)
                dw = jnp.where(row == K // 2, dw + 1.0, dw)
            for gi in range(dw.shape[1] // 128):
                for i in range(K):
                    dw_f[g0 + gi, i] = jnp.broadcast_to(dw[i:i + 1, gi * 128:(gi + 1) * 128], (8, 128))
                for i in range(16):
                    v = dw_f[g0 + gi, i]
                    dw_f[g0 + gi, 32 + i] = v + dw_f[g0 + gi, i + 16] if i + 16 < K else v

    def ln_unit(base, off, n):
        xk = _ln(x_buf[_ds(base, off, n, 16), :].astype(F32))
        if n < 512:
            xk = jnp.concatenate([xk, jnp.zeros((512 - n, D), F32)], axis=0)
        vs = []
        for c in range(2):
            r = c * 256
            alo, ahi = xk[r:r + 128, 0:128], xk[r:r + 128, 128:256]
            blo, bhi = xk[r + 128:r + 256, 0:128], xk[r + 128:r + 256, 128:256]
            vs.append(jnp.concatenate([alo + bhi, ahi - bhi, blo - alo, alo + ahi, blo + bhi], axis=1))
        return _pk(xk.astype(BF16)), _pk(jnp.concatenate(vs, axis=0).astype(BF16))

    def xq_of(t):
        return _upk(xa_ref[_ds(t.ab, 0, TQ // 2, 8), :])

    def xa_chunk(t, j):
        return _upk(xa_ref[_ds(t.kb, j * CK // 2, CK // 2, 16), :])

    R1 = 208
    R2 = TQ - R1

    def qproj(t, combos=True, fast=True):
        if 'q' in SMM and fast:
            (qf,) = smm(xq_of(t).astype(F32), [0])
        else:
            qf = jnp.dot(xq_of(t), _upk(wa_p[...]), preferred_element_type=F32)
            last[0] = qf[0:16, 0:128]
        q_ref[0:TQ // 2, :] = _pk(qf.astype(BF16))
        if STR and combos:
            a11, a12 = qf[0:R1, 0:128], qf[0:R1, 128:256]
            a21, a22 = qf[R1:TQ, 0:128], qf[R1:TQ, 128:256]
            cat = lambda u, v: jnp.concatenate([u, v], axis=0)
            qc_ref[0:R1 // 2, 0:384] = _pk(jnp.concatenate(
                [cat(a11[0:R2] + a22, a11[R2:]), a12 - a11, cat(a12[0:R2] + a22, a12[R2:])], axis=1).astype(BF16))
            qc_ref[0:R2 // 2, 384:640] = _pk(jnp.concatenate([a21 - a22, a11[0:R2] + a21], axis=1).astype(BF16))

    def l1(t, fast=True):
        if 'H' in SMM and fast:
            hp = jnp.concatenate(smm(xq_of(t).astype(F32), [2, 1])[::-1], axis=1)
        else:
            hp = jnp.dot(xq_of(t), _upk(wmi_p[...]), preferred_element_type=F32)
            last[0] = hp[0:16, 0:128]
        h = _gelu(hp)
        u_ref[_ds(t.fb, 0, TQ, 16), :] = h[:, :D]
        g = _ln(h[:, D:])
        halo = jnp.concatenate([g_buf[gi, _ds(t.cb, 0, 16, 32), :] for gi in range(G)], axis=1)
        e = jnp.concatenate([g[0:16] - halo, g[16:] - g[:TQ - 16], -g[TQ - 16:]], axis=0)
        for gi in range(G):
            g_buf[gi, _ds(t.prev, 16 + TQ, 16, 32), :] = g[0:16, gi * 128:(gi + 1) * 128]
            g_buf[G + gi, _ds(t.prev, 16 + TQ, 16, 32), :] = e[0:16, gi * 128:(gi + 1) * 128]
        for gi in range(G):
            g_buf[gi, _ds(t.cb, 16, TQ, 32), :] = g[:, gi * 128:(gi + 1) * 128]
            g_buf[G + gi, _ds(t.cb, 16, TQ + 16, 32), :] = e[:, gi * 128:(gi + 1) * 128]
        for gi in range(G):
            g_buf[gi, _ds(t.next, 0, 16, 32), :] = g[TQ - 16:TQ, gi * 128:(gi + 1) * 128]

    def m_store(t, g0, v, r0=0):
        n = v.shape[0]
        halo = jnp.concatenate([m_buf[g0 + gi, _ds(t.cb, 16 + r0, 16, 32), :] for gi in range(G)], axis=1)
        parts = [v[0:16] - halo, v[16:] - v[:n - 16]]
        if r0 + n == TQ:
            parts.append(-v[n - 16:])
        e = jnp.concatenate(parts, axis=0)
        for gi in range(G):
            m_buf[g0 + gi, _ds(t.cb, 32 + r0, n, 32), :] = v[:, gi * 128:(gi + 1) * 128]
            m_buf[2 * G + g0 + gi, _ds(t.cb, 32 + r0, e.shape[0], 32), :] = e[:, gi * 128:(gi + 1) * 128]
        if n == TQ:
            for gi in range(G):
                m_buf[g0 + gi, _ds(t.next, 0, 32, 32), :] = v[TQ - 32:TQ, gi * 128:(gi + 1) * 128]
                m_buf[2 * G + g0 + gi, _ds(t.next, 16, 16, 32), :] = e[TQ - 16:TQ, gi * 128:(gi + 1) * 128]

    def l2(t, fast=True):
        gc = jnp.concatenate([_conv2(g_buf, gi, G + gi, dw_f, 2 * G + gi, t.cb, 16, TQ, K) for gi in range(G)], axis=-1)
        u = u_ref[_ds(t.fb, 0, TQ, 16), :]
        if 'L' in SMM and fast:
            (loc,) = smm(u * gc, [3])
        else:
            loc = jnp.dot((u * gc).astype(BF16), _upk(wmo_p[...]), preferred_element_type=F32)
        m_store(t, G, loc)

    def merge_half(half, pieces):
        lhs = []
        for (t, off, nrows, yo) in pieces:
            r = 32 - LAG + off
            ms = [_conv2(m_buf, gi, 2 * G + gi, dw_f, gi, t.cb, r, nrows, K)
                  for gi in range(half * G, (half + 1) * G)]
            lhs.append(jnp.concatenate(ms, axis=-1))
        lhs = lhs[0] if len(lhs) == 1 else jnp.concatenate(lhs, axis=0)
        if 'M' in SMM and lhs.shape[0] >= TQ:
            return smm(lhs, [4 + half])[0]
        return jnp.dot(lhs.astype(BF16), _upk(wm_p[half * D // 2:(half + 1) * D // 2, :]), preferred_element_type=F32)

    def merge_a(pieces):
        y = merge_half(1, pieces)
        r = 0
        for (t, off, nrows, yo) in pieces:
            y_ref[yo:yo + nrows, :] = x_buf[_ds(t.fb, off, nrows, 16), :].astype(F32) + y[r:r + nrows]
            r += nrows

    def merge_b(pieces):
        y = merge_half(0, pieces)
        r = 0
        for (t, off, nrows, yo) in pieces:
            o_buf[_ds(t.fb, off, nrows, 16), :] = (y_ref[yo:yo + nrows, :] + y[r:r + nrows]).astype(BF16)
            r += nrows

    def p1_pair(t, js, pos):
        nt = lambda a, b: lax.dot_general(_upk(a), _upk(b), NT_DIMS, preferred_element_type=F32)
        kc = lambda j, i: kc_ref[_ds(t.cbk, j * 64, 64, 32), i * 128:(i + 1) * 128]
        b11 = lambda j: xa_ref[_ds(t.kb, j * 128, 64, 16), 0:128]
        b22 = lambda j: xa_ref[_ds(t.kb, j * 128 + 64, 64, 16), 128:256]
        h1, h2, hs = R1 // 2, R2 // 2, 48
        f = {
            1: lambda j: nt(qc_ref[0:h1, 0:128], kc(j, 0)),
            11: lambda j: nt(qc_ref[0:hs, 0:128], kc(j, 0)),
            12: lambda j: nt(qc_ref[hs:h1, 0:128], kc(j, 0)),
            2: lambda j: nt(q_ref[0:h1, 0:128], kc(j, 4)),
            3: lambda j: nt(qc_ref[0:h2, 384:512], b11(j)),
            4: lambda j: nt(qc_ref[0:h1, 128:256], b22(j)),
            5: lambda j: nt(q_ref[h1:TQ // 2, 128:256], kc(j, 3)),
            6: lambda j: nt(qc_ref[0:h2, 512:640], kc(j, 2)),
            7: lambda j: nt(qc_ref[0:h1, 256:384], kc(j, 1)),
            71: lambda j: nt(qc_ref[0:hs, 256:384], kc(j, 1)),
            72: lambda j: nt(qc_ref[hs:h1, 256:384], kc(j, 1)),
        }
        a, b = js
        cat0 = lambda u, v: jnp.concatenate([u, v], axis=0)

        def mx_upd(ml, final=False):
            if final:
                return jnp.maximum(mp_ref[0:TQ], ml)
            mp_ref[0:TQ] = jnp.maximum(mp_ref[0:TQ], ml) if pos > 0 else ml

        assert pos > 0 or MPV == 2
        for j, order in ((a, (2, 4, 3, 5)), (b, (3, 5, 2, 4))):
            m = {k: f[k](j) for k in order}
            if j == a:
                last[0] = m[2][0:16]
            c0 = j * CK
            c12 = m[2] + m[4]
            c21 = m[3] + m[5]
            s_ref[0:R1, c0 + 128:c0 + 256] = c12
            s_ref[R1:TQ, c0:c0 + 128] = c21
            s_ref[0:R1, c0:c0 + 128] = cat0(m[4][0:R2] - m[5], m[4][R2:])
            s_ref[R1:TQ, c0 + 128:c0 + 256] = m[3] - m[2][0:R2]
            if MPV == 0:
                mx_upd(cat0(c12, c21))
        reload = lambda j: cat0(s_ref[0:R1, j * CK + 128:j * CK + 256], s_ref[R1:TQ, j * CK:j * CK + 128])
        reload2 = lambda j: cat0(s_ref[0:R1, j * CK:j * CK + 128], s_ref[R1:TQ, j * CK + 128:j * CK + 256])
        m1, m7, m6, m6b = f[1](a), f[7](a), f[6](a), f[6](b)
        c0 = a * CK
        c11 = s_ref[0:R1, c0:c0 + 128] + (m1 + m7)
        c22 = s_ref[R1:TQ, c0 + 128:c0 + 256] + (m1[0:R2] + m6)
        s_ref[0:R1, c0:c0 + 128] = c11
        s_ref[R1:TQ, c0 + 128:c0 + 256] = c22
        if MPV == 0:
            mx_upd(cat0(c11, c22))
        elif MPV == 1:
            mx_upd(jnp.maximum(cat0(c11, c22), reload(a)))
        c0 = b * CK
        s_ref[R1:TQ, c0 + 128:c0 + 256] += m6b
        m11, m71, m12, m72 = f[11](b), f[71](b), f[12](b), f[72](b)
        m1, m7 = cat0(m11, m12), cat0(m71, m72)
        c11 = s_ref[0:R1, c0:c0 + 128] + (m1 + m7)
        c22 = s_ref[R1:TQ, c0 + 128:c0 + 256] + m1[0:R2]
        s_ref[0:R1, c0:c0 + 128] = c11
        s_ref[R1:TQ, c0 + 128:c0 + 256] = c22
        ml = cat0(c11, c22)
        if MPV >= 1:
            ml = jnp.maximum(ml, reload(b))
        if MPV == 2:
            ml = jnp.maximum(ml, jnp.maximum(reload(a), reload2(a)))
        return mx_upd(ml, pos >= NC - 2)

    def p1_single(t, j, pos):
        nt = lambda a, b: lax.dot_general(_upk(a), _upk(b), NT_DIMS, preferred_element_type=F32)
        kc = lambda i: kc_ref[_ds(t.cbk, j * 64, 64, 32), i * 128:(i + 1) * 128]
        b11 = xa_ref[_ds(t.kb, j * 128, 64, 16), 0:128]
        b22 = xa_ref[_ds(t.kb, j * 128 + 64, 64, 16), 128:256]
        cat0 = lambda u, v: jnp.concatenate([u, v], axis=0)
        h1, h2, s1, s2 = R1 // 2, R2 // 2, 72, 80
        m2 = nt(q_ref[0:h1, 0:128], kc(4))
        m4 = nt(qc_ref[0:h1, 128:256], b22)
        m3 = nt(qc_ref[0:h2, 384:512], b11)
        m5 = nt(q_ref[h1:TQ // 2, 128:256], kc(3))
        last[0] = m2[0:16]
        c0 = j * CK
        s_ref[0:R1, c0 + 128:c0 + 256] = m2 + m4
        s_ref[R1:TQ, c0:c0 + 128] = m3 + m5
        s_ref[0:R1, c0:c0 + 128] = cat0(m4[0:R2] - m5, m4[R2:])
        s_ref[R1:TQ, c0 + 128:c0 + 256] = m3 - m2[0:R2]
        m6a = nt(qc_ref[0:s2, 512:640], kc(2))
        m1b = nt(qc_ref[s1:h1, 0:128], kc(0))
        m1a = nt(qc_ref[0:s1, 0:128], kc(0))
        m7a = nt(qc_ref[0:s1, 256:384], kc(1))
        m7b = nt(qc_ref[s1:h1, 256:384], kc(1))
        m6b = nt(qc_ref[s2:h2, 512:640], kc(2))
        m1, m7, m6 = cat0(m1a, m1b), cat0(m7a, m7b), cat0(m6a, m6b)
        c11 = s_ref[0:R1, c0:c0 + 128] + (m1 + m7)
        c22 = s_ref[R1:TQ, c0 + 128:c0 + 256] + (m1[0:R2] + m6)
        s_ref[0:R1, c0:c0 + 128] = c11
        s_ref[R1:TQ, c0 + 128:c0 + 256] = c22
        ml = jnp.maximum(cat0(c11, c22), cat0(s_ref[0:R1, c0 + 128:c0 + 256], s_ref[R1:TQ, c0:c0 + 128]))
        assert 0 < pos
        if pos == NC - 1:
            return jnp.maximum(mp_ref[0:TQ], ml)
        mp_ref[0:TQ] = jnp.maximum(mp_ref[0:TQ], ml)

    def p1_chunk(t, j, pos, strassen=True):
        q = _upk(q_ref[0:TQ // 2, :])
        if (j + 1) * CK <= T or REM == 0:
            sj = lax.dot_general(q, xa_chunk(t, j), NT_DIMS, preferred_element_type=F32)
            sts = [sj[:, lt * 128:(lt + 1) * 128] for lt in range(LT)]
            if (j + 1) * CK > T:
                col = lax.broadcasted_iota(jnp.int32, (TQ, 128), 1)
                sts[-1] = jnp.where(col < T % 128, sts[-1], -jnp.inf)
        else:
            nfull = (T - j * CK) // 128
            nrem = T - j * CK - nfull * 128
            assert nfull + 1 == LT and nrem % 16 == 0
            kf = _upk(xa_ref[_ds(t.kb, j * CK // 2, nfull * 64, 16), :])
            if REM == 1:
                sj = lax.dot_general(q, kf, NT_DIMS, preferred_element_type=F32)
            else:
                sj = jnp.concatenate([lax.dot_general(q[0:208], kf, NT_DIMS, preferred_element_type=F32),
                                      lax.dot_general(q[208:TQ], kf, NT_DIMS, preferred_element_type=F32)], axis=0)
            sts = [sj[:, lt * 128:(lt + 1) * 128] for lt in range(nfull)]
            kr = _upk(xa_ref[_ds(t.kb, j * CK // 2 + nfull * 64, nrem // 2, 16), :])
            st = lax.dot_general(kr, _upk(q_ref[...]), NT_DIMS, preferred_element_type=F32)
            st = jnp.concatenate([st, jnp.full((128 - nrem, st.shape[1]), -jnp.inf, F32)], axis=0)
            sts.append(st.T[0:TQ])
        last[0] = sj[0:16, 0:128]
        mloc = None
        for lt in range(LT):
            c0 = j * CK + lt * 128
            s_ref[:, c0:c0 + 128] = sts[lt]
            mloc = sts[lt] if mloc is None else jnp.maximum(mloc, sts[lt])
        if pos == 0:
            mp_ref[0:TQ] = mloc
        elif pos < NC - 1:
            mp_ref[0:TQ] = jnp.maximum(mp_ref[0:TQ], mloc)
        else:
            return jnp.maximum(mp_ref[0:TQ], mloc)

    def p1_fin(mpart, scaled=True):
        m = jnp.max(mpart, axis=-1, keepdims=True)
        if scaled:
            lam = jnp.sum(jnp.exp2(mpart - m), axis=-1, keepdims=True)
            m = m + jnp.log(lam) * LOG2E
        mx_ref[0:TQ] = jnp.broadcast_to(m, (TQ, 128))

    def p2_group(t, js, first, r0=0, r1=R1, r2=R2):
        cat0 = lambda u, v: jnp.concatenate([u, v], axis=0) if v.shape[0] else u
        ra, rb, rc = r0, r0 + r1, r0 + r1 + r2
        L = {k: [] for k in range(1, 8)}
        l1 = l2 = None
        for j in js:
            c0 = j * CK
            a11 = jnp.exp2(s_ref[ra:rb, c0:c0 + 128] - mx_ref[ra:rb])
            a12 = jnp.exp2(s_ref[ra:rb, c0 + 128:c0 + 256] - mx_ref[ra:rb])
            a21 = jnp.exp2(s_ref[rb:rc, c0:c0 + 128] - mx_ref[rb:rc])
            a22 = jnp.exp2(s_ref[rb:rc, c0 + 128:c0 + 256] - mx_ref[rb:rc])
            s1 = a11 + a12
            s2 = a21 + a22
            l1 = s1 if l1 is None else l1 + s1
            l2 = s2 if l2 is None else l2 + s2
            L[1].append(cat0(a11[0:r2] + a22, a11[r2:]))
            L[2].append(s2)
            L[3].append(a11)
            L[4].append(a22)
            L[5].append(s1)
            L[6].append(a21 - a11[0:r2])
            L[7].append(cat0(a12[0:r2] - a22, a12[r2:]))
        kc = lambda j, i: kc_ref[_ds(t.cbk, j * 64, 64, 32), i * 128:(i + 1) * 128]
        W = {
            1: lambda j: kc(j, 0),
            2: lambda j: xa_ref[_ds(t.kb, j * 128, 64, 16), 0:128],
            3: lambda j: kc(j, 1),
            4: lambda j: kc(j, 2),
            5: lambda j: xa_ref[_ds(t.kb, j * 128 + 64, 64, 16), 128:256],
            6: lambda j: kc(j, 3),
            7: lambda j: kc(j, 4),
        }
        for i, k in enumerate(VSEQ):
            lhs = jnp.concatenate(L[k], axis=1).astype(BF16)
            rhs = _upk(jnp.concatenate([W[k](j) for j in js], axis=0))
            mk = jnp.dot(lhs, rhs, preferred_element_type=F32)
            last[0] = mk[0:16]
            if i == 0:
                last_e[0] = mk[0:16]
            n = mk.shape[0]
            if first:
                acc7_ref[k, 0:n] = mk
            else:
                acc7_ref[k, 0:n] += mk
        lloc = cat0(l1, l2)
        if first:
            lp_ref[ra:rc] = lloc
        else:
            lp_ref[ra:rc] += lloc

    def p2_fin7(t, r0=0, r1=R1, r2=R2):
        cat0 = lambda u, v: jnp.concatenate([u, v], axis=0) if v.shape[0] else u
        l = jnp.sum(lp_ref[r0:r0 + r1 + r2], axis=-1, keepdims=True)
        m1, m3, m5, m7 = (acc7_ref[k, 0:r1] for k in (1, 3, 5, 7))
        m2, m4, m6 = (acc7_ref[k, 0:r2] for k in (2, 4, 6))
        c11 = m1 + (m7 - m5)
        c11 = cat0(c11[0:r2] + m4, c11[r2:])
        c12 = m3 + m5
        c21 = m2 + m4
        c22 = (m1[0:r2] - m2) + (m3[0:r2] + m6)
        acc = jnp.concatenate([jnp.concatenate([c11, c12], axis=1), jnp.concatenate([c21, c22], axis=1)], axis=0)
        o = acc * (1.0 / l)
        glob = jnp.dot(o.astype(BF16), _upk(wvo_p[...]), preferred_element_type=F32)
        m_store(t, 0, glob, r0)

    def p2_chunk(t, j, pos, r0=0, n=TQ):
        ps = []
        lloc = None
        for lt in range(LT):
            c0 = j * CK + lt * 128
            p = jnp.exp2(s_ref[r0:r0 + n, c0:c0 + 128] - mx_ref[r0:r0 + n])
            lloc = p if lloc is None else lloc + p
            ps.append(p)
        pv = jnp.dot(jnp.concatenate(ps, axis=-1).astype(BF16), xa_chunk(t, j), preferred_element_type=F32)
        last[0] = pv[0:16, 0:128]
        last_e[0] = lloc[0:16]
        if pos == 0:
            lp_ref[r0:r0 + n] = lloc
            acc_ref[r0:r0 + n] = pv
        else:
            lp_ref[r0:r0 + n] += lloc
            acc_ref[r0:r0 + n] += pv

    def p2_fin(t, r0=0, n=TQ):
        l = jnp.sum(lp_ref[r0:r0 + n], axis=-1, keepdims=True)
        o = (acc_ref[r0:r0 + n] * (1.0 / l)).astype(BF16)
        glob = jnp.dot(o, _upk(wvo_p[...]), preferred_element_type=F32)
        m_store(t, 0, glob, r0)

    def anchor(buf):
        zrow = pl.multiple_of(zoff[0], 8)
        buf[0, pl.ds(zrow + JUNK, 8), :] = last[0][0:8]

    def anchor_l():
        zrow = pl.multiple_of(zoff[0], 8)
        lp_ref[pl.ds(zrow + TQ, 8), :] = last[0][0:8]

    def anchor_m():
        zrow = pl.multiple_of(zoff[0], 8)
        mx_ref[pl.ds(zrow + TQ, 8), :] = last[0][0:8]

    def anchor_x():
        zrow = pl.multiple_of(zoff[0], 16)
        x_buf[pl.ds(zrow + B * T + LAG + TP - T, 16), 0:128] = last[0].astype(BF16)

    def out_copy(base, off, n):
        return pltpu.make_async_copy(o_buf.at[_ds(base, off, n, 16), :], o_hbm.at[_ds(base, off - LAG, n, 16), :], sem_out)

    DEF = 'q Z Zg W W Mb K Ks D W Ma W Zl L H KK KK Zx n KK Zx n KK Zx n KK Zx n KK KK Ns G7'
    ORDER = DEF.split()
    ORDERP = 'q Z Zg W W Mb K Ks W Ma W Zl L KK KK KK KK KK KK KK G7'.split()
    ORDERL = 'WA E Z WA WA Mb WA Zl Mc G7a | B Z S B B R Zm B S B B R Zm B B B B B B B B B B Zl M1 Gb M2'.split()

    RPOS = 3
    CORD = list(range(NC - 1))
    CORD.insert(RPOS, NC - 1)
    CORDP = list(range(NC - 1))
    CORDP.insert(NC - 3, NC - 1)

    def step(order, pb, pa, t0, tp, th, tn, dma=None, pc=None, cc=None):
        CORD = []
        nxt = 0
        for op in order:
            if op == 'KK':
                CORD += [nxt, nxt + 1]
                nxt += 2
            elif op in ('Ks', 'K1'):
                CORD.append(NC - 2)
            elif op == 'K':
                CORD.append(NC - 1)
        assert order.count('V') + 4 * order.count('W') == NC and sorted(CORD) == list(range(NC))
        mpart = None
        jv = jk = 0
        nq = []
        for op in order:
            if op in SKIP.split(','):
                continue
            if op == 'q':
                qproj(tp)
            elif op == 'V':
                p2_chunk(t0, CORD[jv], jv)
                jv += 1
            elif op == 'W':
                p2_group(t0, CORD[jv:jv + 4], jv == 0)
                jv += 4
            elif op == 'G7':
                p2_fin7(t0)
            elif op == 'K':
                assert jk < jv
                mpart = p1_chunk(tp, CORD[jk], jk)
                jk += 1
            elif op == 'KK':
                assert jk + 1 < jv and CORD[jk] < NC - 1 and CORD[jk + 1] < NC - 1
                mpart = p1_pair(tp, (CORD[jk], CORD[jk + 1]), jk)
                jk += 2
            elif op == 'K1':
                assert jk < jv
                mpart = p1_single(tp, CORD[jk], jk)
                jk += 1
            elif op == 'Ks':
                assert jk < jv
                mpart = p1_chunk(tp, CORD[jk], jk, False)
                jk += 1
            elif op == 'Z':
                anchor(m_buf)
            elif op == 'Zg':
                anchor(g_buf)
            elif op == 'Zx':
                anchor_x()
            elif op == 'Zl':
                anchor_l()
            elif op == 'Ma':
                merge_a(pa)
            elif op == 'Mc':
                merge_a(pc)
            elif op == 'Mb':
                merge_b(pb)
            elif op == 'H':
                l1(th)
            elif op == 'L':
                l2(tp)
            elif op == 'N':
                xa_n, kc_n = ln_unit(tn * 512, LAG + T, 512)
            elif op == 'n':
                r = (len(nq) // 2) * 256 + (len(nq) % 2) * 64
                xa_, xb_ = (_ln(x_buf[_ds(tn * 512, LAG + T + r + o, 64, 16), :].astype(F32)) for o in (0, 128))
                alo, ahi, blo, bhi = xa_[:, 0:128], xa_[:, 128:256], xb_[:, 0:128], xb_[:, 128:256]
                v = jnp.concatenate([xa_, xb_, alo + bhi, ahi - bhi, blo - alo, alo + ahi, blo + bhi], axis=1)
                nq.append((r, _pk(v.astype(BF16))))
            elif op == 'Ns' and nq:
                assert len(nq) == 4
                for r, v in nq:
                    xa_ref[_ds(tn * 256, TP // 2 + r // 2, 32, 256), :] = v[:, 0:256]
                    xa_ref[_ds(tn * 256, TP // 2 + r // 2 + 64, 32, 256), :] = v[:, 256:512]
                    kc_ref[_ds(tn * 128, 16 * 64 + (r // 256) * 64 + (r % 256) // 2, 32, 128), :] = v[:, 512:1152]
            elif op == 'Ns':
                xa_ref[_ds(tn * 256, TP // 2, 256, 256), :] = xa_n
                kc_ref[_ds(tn * 128, 16 * 64, 128, 128), :] = kc_n
            elif op == 'G':
                p2_fin(t0)
            elif op == 'D':
                dma()

            else:
                raise ValueError(op)
        if tp is not None:
            p1_fin(mpart)

    def do_ln(u):
        xa_ref[u * 256:(u + 1) * 256, :], kc_ref[u * 128:(u + 1) * 128, :] = ln_unit(0, LAG + u * 512, min(512, T - u * 512))

    jk = 0
    nln = 0
    done = []
    for op in PRO:
        if 'P' not in ONLY and op[0] not in 'xws':
            continue
        if op == 'STOP':
            return
        if op[0] == 's':
            dma_start(op)
        elif op[0] == 'x':
            x_copy(int(op[1:])).wait()
        elif op[0] == 'n':
            do_ln(int(op[1:]))
            nln = max(nln, int(op[1:]) + 1)
        elif op[0] == 'w':
            w_copy(int(op[1:])).wait()
        elif op[0] == 'p':
            prep(int(op[1:]))
        elif op == 'A':
            prep_a()
        elif op == 'q':
            qproj(tile(0), any(o.startswith('KK') for o in PRO), False)
        elif op.startswith('KK'):
            j = int(op[2:])
            assert nln * 512 >= (j + 2) * CK
            mpart = p1_pair(tile(0), (j, j + 1), jk)
            done += [j, j + 1]
            jk += 2
        elif op[0] == 'K':
            j = int(op[1:])
            assert nln * 512 >= (j + 1) * CK
            mpart = p1_chunk(tile(0), j, jk, False)
            done.append(j)
            jk += 1
        elif op[0] == 'H':
            l1(tile(int(op[1:])), False)
        elif op == 'L0':
            l2(tile(0), False)
        elif op == 'Zg':
            anchor(g_buf)
        elif op == 'Zx':
            anchor_x()
        else:
            raise ValueError(op)
    if 'P' in ONLY:
        assert sorted(done) == list(range(NC))
        p1_fin(mpart)
    if STOP == 'pro':
        return

    DEF2 = ' '.join(o for o in ORDER if o not in ('N', 'n', 'Ns', 'Zx'))
    ORDER2 = DEF2.split()

    def body(order, s, c):
        if 'Ns' in order:
            @pl.when(s == 1)
            def _():
                x_copy(NU + 1).wait()

        w = jnp.maximum(s - 1, 0)
        fb = w * TQ

        def dma():
            @pl.when(s > 0)
            def _():
                out_copy(fb, LAG, TQ - LAG).start()

            @pl.when(jnp.logical_and(s > 1, s != NT + 1))
            def _():
                out_copy(fb, 0, LAG).start()

        step(order, [(tile(w), 0, TQ, 0)], [(tile(s), 0, TQ, 0)], tile(s), tile(s + 1), tile(s + 3), s, dma)
        return c
    if '1' in ONLY:
        lax.fori_loop(0, NU, functools.partial(body, ORDER), 0)
    if '2' in ONLY:
        lax.fori_loop(NU, NITER, functools.partial(body, ORDER2), 0)

    z = zoff[0]
    t9 = tile(NT - 1)

    tl = tile(NS - 1)
    Y2 = TQ + 3 * LAG

    def body2(s, c):
        step(ORDERP, [(tile(s - 1), 0, TQ, 0)], [(tile(s), 0, TQ, 0), (t9, TQ, LAG, TQ + LAG)],
             tile(s), tile(s + 1), None, None)
        out_copy((s - 1) * TQ, 0, TQ).start()
        return c
    if 'B' in ONLY:
        lax.fori_loop(NS - 3, NS - 1, body2, 0)

    RA = 288

    cnt = {'A': 0, 'B': 0}
    RB1 = ((TQ - RA) // 2 + 15) // 16 * 16

    def last_block(ops):
        dyn = (lambda t: tile(z + t)) if '1' == '1' else tile
        tl = dyn(NS - 1)
        for op in ops:
            if op == 'A':
                p2_chunk(tl, cnt['A'], cnt['A'], 0, RA)
                cnt['A'] += 1
            elif op == 'B':
                p2_chunk(tl, cnt['B'], cnt['B'], RA, TQ - RA)
                cnt['B'] += 1
            elif op == 'WA':
                p2_group(tl, list(range(cnt['A'], cnt['A'] + 4)), cnt['A'] == 0, 0, RA // 2, RA // 2)
                cnt['A'] += 4
            elif op == 'WB':
                p2_group(tl, list(range(cnt['B'], cnt['B'] + 4)), cnt['B'] == 0, RA, RB1, TQ - RA - RB1)
                cnt['B'] += 4
            elif op == 'G7a':
                p2_fin7(tl, 0, RA // 2, RA // 2)
            elif op == 'G7b':
                p2_fin7(tl, RA, RB1, TQ - RA - RB1)
            elif op == 'E':
                last[0] = last_e[0]
            elif op == 'Z':
                anchor(m_buf)
            elif op == 'Ze':
                last[0] = last_e[0]
                anchor(m_buf)
            elif op == 'Zl':
                anchor_l()
            elif op == 'Zm':
                anchor_m()
            elif op == 'S':
                saved = last[0]
            elif op == 'R':
                last[0] = saved
            elif op == 'Mb':
                merge_b([(dyn(NS - 2), 0, TQ, 0), (t9, TQ, LAG, TQ + LAG)])
                out_copy(0, (NS - 2) * TQ, TQ).start()
                out_copy(0, NT * TQ, LAG).start()
            elif op == 'Mc':
                merge_a([(tl, 0, TQ + LAG, Y2)])
            elif op == 'Ga':
                p2_fin(tl, 0, RA)
            elif op == 'Gb':
                p2_fin(tl, RA, TQ - RA)
            elif op == 'M1':
                merge_b([(tl, 0, RA, Y2)])
                out_copy(0, (NS - 1) * TQ, RA).start()
            elif op == 'M2':
                merge_b([(tl, RA, TQ + LAG - RA, Y2 + RA)])
                out_copy(0, (NS - 1) * TQ + RA, TQ + LAG - RA).start()
            else:
                raise ValueError(op)

    if 'L' not in ONLY:
        return
    for bi, ops in enumerate(' '.join(ORDERL).split('|')):
        pl.when(z < 1 + bi)(functools.partial(last_block, ops.split()))
    assert cnt['A'] == NC and cnt['B'] == NC

    nrows = (NITER - 1) * (TQ - LAG) + sum(LAG for s in range(2, NITER) if s != NT + 1) + 4 * TQ + 2 * LAG
    out_copy(0, LAG, nrows).wait()


@jax.jit
def pallas_standalone__conformer_family_e_branchformer__speech_kernel(
    x, w_qkv, w_att_out, w_mlp_in, dw_csgu, w_mlp_out, dw_merge, w_merge):
    B, T, D = x.shape
    K = dw_csgu.shape[0]
    TQ = 400
    TP = 4096
    CK = 256
    G = D // 128
    NT = T // TQ
    RB = (B * NT + 1) * SLOT
    out = pl.pallas_call(
        functools.partial(kernel, B=B, T=T, D=D, K=K, TQ=TQ, TP=TP, CK=CK),
        in_specs=[pl.BlockSpec(memory_space=pl.ANY)] * 8,
        out_specs=pl.BlockSpec(memory_space=pl.ANY),
        out_shape=jax.ShapeDtypeStruct((B * T, D), x.dtype),
        scratch_shapes=[
            pltpu.VMEM((B * T + 32 + TP - T, D), BF16),
            pltpu.VMEM((B * T + 32, D), BF16),
            pltpu.VMEM((B * TP // 2, D), U32),
            pltpu.VMEM((D // 2, D), U32),
            pltpu.VMEM((D // 2, D), U32),
            pltpu.VMEM((D // 2, 2 * D), U32),
            pltpu.VMEM((D // 2, D), U32),
            pltpu.VMEM((D, D), U32),
            pltpu.VMEM((8, 64, 896), U32),
            pltpu.VMEM((3 * G, 48, 8, 128), F32),
            pltpu.VMEM((2 * G, RB, 128), F32),
            pltpu.VMEM((4 * G, RB, 128), F32),
            pltpu.VMEM((B * T, D), F32),
            pltpu.VMEM((TQ, TP), F32),
            pltpu.VMEM((TQ + 16, 128), F32),
            pltpu.VMEM((256, D), U32),
            pltpu.VMEM((128, 640), U32),
            pltpu.VMEM((B * 16 * 64, 640), U32),
            pltpu.VMEM((TQ + 16, 128), F32),
            pltpu.VMEM((TQ + 16, 128), F32),
            pltpu.VMEM((TQ, D), F32),
            pltpu.VMEM((8, 224, 128), F32),
            pltpu.VMEM((2 * TQ + 4 * LAG, D), F32),
            pltpu.VMEM(w_qkv.shape, BF16),
            pltpu.VMEM(w_att_out.shape, BF16),
            pltpu.VMEM(w_mlp_in.shape, BF16),
            pltpu.VMEM(dw_csgu.shape, BF16),
            pltpu.VMEM(w_mlp_out.shape, BF16),
            pltpu.VMEM(dw_merge.shape, BF16),
            pltpu.VMEM(w_merge.shape, BF16),
            pltpu.SMEM((1,), jnp.int32),
            pltpu.SemaphoreType.DMA((max(GRP.values()) + 1,)),
            pltpu.SemaphoreType.DMA,
        ],
        compiler_params=pltpu.CompilerParams(vmem_limit_bytes=120 * 1024 * 1024, disable_bounds_checks=True),
    )(x.reshape(B * T, D), w_qkv, w_att_out, w_mlp_in, dw_csgu, w_mlp_out, dw_merge, w_merge)
    return out.reshape(B, T, D)
```

```python
import functools

import jax
import jax.numpy as jnp
from jax import lax
import jax.experimental.pallas as pl
import jax.experimental.pallas.tpu as pltpu

F32 = jnp.float32
BF16 = jnp.bfloat16
U32 = jnp.uint32
LOG2E = 1.4426950408889634
NT_DIMS = (((1,), (1,)), ((), ()))

TQ = 400
CK = 256
SLOT = 448
LAG = 16
R1 = 208
R2 = TQ - R1
RA = 288
VSEQ = (3, 4, 1, 5, 7, 2, 6)

PROLOGUE = (
    'sx0 sw0 | x0 sx1 sw1 n0 w0 sx2 sx3 A q x1 w1 sx4 sx5 sw3 sw4 p1 n1 H0 KK0 K2 '
    'x2 x3 x4 sx6 sx7 sw2 sw5 sw6 sw7 sx8 n2 H1 K3 Zx n3 KK4 Zx n4 H2 KK6 '
    'x5 x6 x7 w3 w4 w2 w5 w6 w7 x8 sx9 p3 p4 KK8 Zg n5 n6 n7 p5 p6 KK10 K12 K15 K13 K14 L0 p2').split()
STEP_A1 = 'q Z Zg W W Mb K Ks D W Ma W Zl L H KK KK Zx n KK Zx n KK Zx n KK Zx n KK KK Ns G'.split()
STEP_A2 = 'q Z Zg W W Mb K Ks D W Ma W Zl L H KK KK KK KK KK KK KK G'.split()
STEP_B = 'q Z Zg W W Mb K Ks W Ma W Zl L KK KK KK KK KK KK KK G'.split()
LAST_A = 'WA E Z WA WA Mb WA Zl Mc Ga'.split()
LAST_B = 'B Z S B B R Zm B S B B R Zm B B B B B B B B B B Zl M1 Gb M2'.split()


def _sem_groups():
    grp, g, prev = {}, -1, False
    for op in PROLOGUE:
        is_wait = op[0] in 'xw'
        if is_wait:
            g += 0 if prev else 1
            grp[op] = g
        prev = is_wait
    grp['x9'] = g + 1
    return grp


GRP = _sem_groups()


def _pk(x):
    return pltpu.bitcast(x, U32)


def _upk(x):
    return pltpu.bitcast(x, BF16)


def _cat0(u, v):
    return jnp.concatenate([u, v], axis=0) if v.shape[0] else u


def _ln(x, eps=1e-5):
    m = jnp.mean(x, axis=-1, keepdims=True)
    xc = x - m
    v = jnp.mean(xc * xc, axis=-1, keepdims=True)
    return xc * jnp.exp2(jnp.log(v + eps) * (-0.5 * LOG2E))


def _gelu(x):
    c = 0.7978845608028654
    hx = 0.5 * x
    return hx + hx * jnp.tanh(x * (c + (c * 0.044715) * (x * x)))


def _ds(base, off, n, align):
    if isinstance(base, int):
        return pl.ds(base + off, n)
    a = align
    while off % a:
        a //= 2
    return pl.ds(pl.multiple_of(base + off, a), n) if a > 1 else pl.ds(base + off, n)


def _conv_direct(buf_ref, g, w_ref, wg, base, off, nrows, K):
    V = nrows // 8
    acc = None
    for p in range(8):
        taps = list(range(p, K, 8))
        nq = V + len(taps) - 1
        slab = buf_ref[g, _ds(base, off + p - K // 2, 8 * nq, 32), :].reshape(nq, 8, 128)
        for qi, i in enumerate(taps):
            term = slab[qi:qi + V] * w_ref[wg, i][None]
            acc = term if acc is None else acc + term
    return acc.reshape(8 * V, 128)


def _conv(buf_ref, g, ge, w_ref, wg, base, off, nrows, K):
    nq = nrows // 32
    outs = []
    q0 = 0
    while q0 < nq:
        Q = min(4, nq - q0)
        am = a0 = a1 = None
        for i in [p + 8 * h for p in range(8) for h in range(2)]:
            r = off + 32 * q0 + i - K // 2 + 16
            xs = buf_ref[g, _ds(base, r, 32 * Q - 16, 32), :]
            xs = jnp.concatenate([xs[32 * k:32 * k + 16] for k in range(Q)], axis=0).reshape(2 * Q, 8, 128)
            t = xs * w_ref[wg, 32 + i][None]
            am = t if am is None else am + t
            if i + 16 < K:
                es = buf_ref[ge, _ds(base, r, 32 * Q, 32), :]
                e2 = jnp.concatenate([es[32 * k + 16:32 * k + 32] for k in range(Q)], axis=0).reshape(2 * Q, 8, 128)
                t = e2 * w_ref[wg, i + 16][None]
                a1 = t if a1 is None else a1 + t
            else:
                es = buf_ref[ge, _ds(base, r, 32 * Q - 16, 32), :]
            e1 = jnp.concatenate([es[32 * k:32 * k + 16] for k in range(Q)], axis=0).reshape(2 * Q, 8, 128)
            t = e1 * w_ref[wg, i][None]
            a0 = t if a0 is None else a0 + t
        y0 = (am - a0).reshape(16 * Q, 128)
        y1 = (am + a1).reshape(16 * Q, 128)
        for k in range(Q):
            outs += [y0[16 * k:16 * k + 16], y1[16 * k:16 * k + 16]]
        q0 += Q
    if nrows % 32:
        outs.append(_conv_direct(buf_ref, g, w_ref, wg, base, off + 32 * nq, nrows - 32 * nq, K))
    return jnp.concatenate(outs, axis=0) if len(outs) > 1 else outs[0]


def _key_combos(alo, ahi, blo, bhi):
    return [alo + bhi, ahi - bhi, blo - alo, alo + ahi, blo + bhi]


class _Tile:
    def __init__(self, t, NT, NS, TP, T):
        if isinstance(t, int):
            b = t // NT
            self.prev = (NS if t % NT == 0 else t - 1) * SLOT
            self.next = (NS if t % NT == NT - 1 else t + 1) * SLOT
        else:
            b = (t >= NT).astype(jnp.int32)
            first = jnp.logical_or(t == 0, t == NT)
            last = jnp.logical_or(t == NT - 1, t == NS - 1)
            self.prev = jnp.where(first, NS, t - 1) * SLOT
            self.next = jnp.where(last, NS, t + 1) * SLOT
        self.cb = t * SLOT
        self.fb = t * TQ
        self.ab = t * (TQ // 2) + b * ((TP - T) // 2)
        self.kb = b * (TP // 2)
        self.cbk = b * (TP // 4)


def _kernel(x_hbm, wqkv_hbm, wao_hbm, wmi_hbm, dwc_hbm, wmo_hbm, dwm_hbm, wm_hbm, o_hbm,
            x_buf, o_buf, xa_ref, wa_p, wvo_p, wmi_p, wmo_p, wm_p, ws_ref, dw_f, g_buf, m_buf, u_ref,
            s_ref, mx_ref, q_ref, qc_ref, kc_ref, mp_ref, lp_ref, acc_ref, acc7_ref, y_ref,
            wqkv_ref, wao_ref, wmi_ref, dwc_ref, wmo_ref, dwm_ref, wm_ref,
            zoff, sem_in, sem_out,
            *, B, T, D, K, TP):
    NT = T // TQ
    NS = B * NT
    G = D // 128
    NC = TP // CK
    NU = TP // 512
    assert B == 2 and D == 256 and K == 31 and T % TQ == 0 and NC == 16
    last = [None]
    first_w = [None]

    def tile(t):
        return _Tile(t, NT, NS, TP, T)

    def x_copy(u):
        r0 = u * 512 if u < NU else (T if u == NU else T + 512)
        n = min(512, T - r0) if u < NU else (512 if u == NU else T - 512)
        return pltpu.make_async_copy(x_hbm.at[pl.ds(r0, n), :], x_buf.at[pl.ds(LAG + r0, n), :],
                                     sem_in.at[GRP['x%d' % u]])

    w_pairs = [(wqkv_hbm.at[:, 0:2 * D], wqkv_ref.at[:, 0:2 * D]), (wmi_hbm, wmi_ref), (wao_hbm, wao_ref),
               (dwc_hbm, dwc_ref), (wmo_hbm, wmo_ref), (dwm_hbm, dwm_ref), (wm_hbm, wm_ref),
               (wqkv_hbm.at[:, 2 * D:3 * D], wqkv_ref.at[:, 2 * D:3 * D])]

    def w_copy(k):
        return pltpu.make_async_copy(w_pairs[k][0], w_pairs[k][1], sem_in.at[GRP['w%d' % k]])

    def dma_start(op):
        (x_copy if op[1] == 'x' else w_copy)(int(op[2:])).start()

    def out_copy(base, off, n):
        return pltpu.make_async_copy(o_buf.at[_ds(base, off, n, 16), :], o_hbm.at[_ds(base, off - LAG, n, 16), :],
                                     sem_out)

    split = PROLOGUE.index('|')
    for op in PROLOGUE[:split]:
        dma_start(op)

    zoff[0] = 0
    z16 = jnp.zeros((16, 128), F32)
    for b in range(B):
        lo, hi = b * NT * SLOT, ((b + 1) * NT - 1) * SLOT
        for gi in range(G):
            g_buf[gi, lo:lo + 16, :] = z16
            g_buf[gi, hi + 416:hi + 432, :] = z16
        for gi in range(2 * G):
            m_buf[gi, lo:lo + 16, :] = z16
            m_buf[gi, lo + 16:lo + 32, :] = z16
            m_buf[2 * G + gi, lo + 16:lo + 32, :] = z16
            m_buf[gi, hi + 432:hi + 448, :] = z16
    x_buf[0:LAG, :] = jnp.zeros((LAG, D), BF16)
    x_buf[LAG + B * T:LAG + B * T + TP - T, :] = jnp.zeros((TP - T, D), BF16)
    q_ref[TQ // 2:, :] = jnp.zeros((q_ref.shape[0] - TQ // 2, D), U32)

    def prep_a():
        a = lax.dot_general(wqkv_ref[:, 0:D], wqkv_ref[:, D:2 * D], NT_DIMS, preferred_element_type=F32)
        a = a * (D ** -0.5 * LOG2E)
        wa_p[...] = _pk(a.astype(BF16))
        b11, b12, b21, b22 = a[0:128, 0:128], a[0:128, 128:256], a[128:256, 0:128], a[128:256, 128:256]
        ws_ref[...] = _pk(jnp.concatenate(
            [b11 + b22, b11, b12 - b22, b21 - b11, b22, b11 + b12, b21 + b22], axis=1).astype(BF16))

    def prep(k):
        if k == 1:
            wmi_p[...] = _pk(wmi_ref[...])
        elif k == 2:
            wvo = jnp.dot(wqkv_ref[:, 2 * D:3 * D], wao_ref[...], preferred_element_type=F32)
            wvo_p[...] = _pk(wvo.astype(BF16))
        elif k == 4:
            wmo_p[...] = _pk(wmo_ref[...])
        elif k == 6:
            wm_p[...] = _pk(wm_ref[...])
        else:
            dw = (dwc_ref if k == 3 else dwm_ref)[...].astype(F32)
            g0 = 2 * G if k == 3 else 0
            if k == 5:
                row = lax.broadcasted_iota(jnp.int32, dw.shape, 0)
                dw = jnp.where(row == K // 2, dw + 1.0, dw)
            for gi in range(dw.shape[1] // 128):
                for i in range(K):
                    dw_f[g0 + gi, i] = jnp.broadcast_to(dw[i:i + 1, gi * 128:(gi + 1) * 128], (8, 128))
                for i in range(16):
                    v = dw_f[g0 + gi, i]
                    dw_f[g0 + gi, 32 + i] = v + dw_f[g0 + gi, i + 16] if i + 16 < K else v

    def ln_unit(u):
        n = min(512, T - u * 512)
        xk = _ln(x_buf[pl.ds(LAG + u * 512, n), :].astype(F32))
        if n < 512:
            xk = jnp.concatenate([xk, jnp.zeros((512 - n, D), F32)], axis=0)
        vs = []
        for r in (0, 256):
            vs.append(jnp.concatenate(_key_combos(xk[r:r + 128, 0:128], xk[r:r + 128, 128:256],
                                                  xk[r + 128:r + 256, 0:128], xk[r + 128:r + 256, 128:256]), axis=1))
        xa_p, kc_p = _pk(xk.astype(BF16)), _pk(jnp.concatenate(vs, axis=0).astype(BF16))
        xa_ref[u * 256:(u + 1) * 256, :] = xa_p
        kc_ref[u * 128:(u + 1) * 128, :] = kc_p

    def xq_of(t):
        return _upk(xa_ref[_ds(t.ab, 0, TQ // 2, 8), :])

    def xa_chunk(t, j):
        return _upk(xa_ref[_ds(t.kb, j * CK // 2, CK // 2, 16), :])

    def kc(t, j, i):
        return kc_ref[_ds(t.cbk, j * 64, 64, 32), i * 128:(i + 1) * 128]

    def k_alo(t, j):
        return xa_ref[_ds(t.kb, j * 128, 64, 16), 0:128]

    def k_bhi(t, j):
        return xa_ref[_ds(t.kb, j * 128 + 64, 64, 16), 128:256]

    def q_strassen(lhs):
        a11, a12, a21, a22 = lhs[0:R1, 0:128], lhs[0:R1, 128:256], lhs[R1:TQ, 0:128], lhs[R1:TQ, 128:256]
        p1 = jnp.concatenate([_cat0(a11[0:R2] + a22, a11[R2:]), a11, a11 + a12, _cat0(a12[0:R2] - a22, a12[R2:])],
                             axis=1).astype(BF16)
        p2 = jnp.concatenate([a21 + a22, a22, a21 - a11[0:R2]], axis=1).astype(BF16)
        lk = {1: p1[:, 0:128], 3: p1[:, 128:256], 5: p1[:, 256:384], 7: p1[:, 384:512],
              2: p2[:, 0:128], 4: p2[:, 128:256], 6: p2[:, 256:384]}

        def job(k, lo=None, hi=None):
            l = lk[k] if lo is None else lk[k][lo:hi]
            return jnp.dot(l, _upk(ws_ref[:, (k - 1) * 128:k * 128]), preferred_element_type=F32)
        s1, s2 = 144, 160
        m3, m5, m2, m4 = job(3), job(5), job(2), job(4)
        m6a = job(6, 0, s2)
        m1b = job(1, s1, R1)
        m1a = job(1, 0, s1)
        m7a = job(7, 0, s1)
        m7b = job(7, s1, R1)
        m6 = _cat0(m6a, job(6, s2, R2))
        m1, m7 = _cat0(m1a, m1b), _cat0(m7a, m7b)
        last[0] = m3[0:16]
        c12 = m3 + m5
        c21 = m2 + m4
        c11 = _cat0(m4 - m5[0:R2], -m5[R2:]) + (m1 + m7)
        c22 = ((m3[0:R2] - m2) + m6) + m1[0:R2]
        return jnp.concatenate([jnp.concatenate([c11, c12], axis=1), jnp.concatenate([c21, c22], axis=1)], axis=0)

    def qproj(t, fast=True):
        if fast:
            qf = q_strassen(xq_of(t).astype(F32))
        else:
            qf = jnp.dot(xq_of(t), _upk(wa_p[...]), preferred_element_type=F32)
            last[0] = qf[0:16, 0:128]
        q_ref[0:TQ // 2, :] = _pk(qf.astype(BF16))
        a11, a12 = qf[0:R1, 0:128], qf[0:R1, 128:256]
        a21, a22 = qf[R1:TQ, 0:128], qf[R1:TQ, 128:256]
        qc_ref[0:R1 // 2, 0:384] = _pk(jnp.concatenate(
            [_cat0(a11[0:R2] + a22, a11[R2:]), a12 - a11, _cat0(a12[0:R2] + a22, a12[R2:])], axis=1).astype(BF16))
        qc_ref[0:R2 // 2, 384:640] = _pk(jnp.concatenate([a21 - a22, a11[0:R2] + a21], axis=1).astype(BF16))

    def mlp_in(t):
        hp = jnp.dot(xq_of(t), _upk(wmi_p[...]), preferred_element_type=F32)
        last[0] = hp[0:16, 0:128]
        h = _gelu(hp)
        u_ref[_ds(t.fb, 0, TQ, 16), :] = h[:, :D]
        g = _ln(h[:, D:])
        halo = jnp.concatenate([g_buf[gi, _ds(t.cb, 0, 16, 32), :] for gi in range(G)], axis=1)
        e = jnp.concatenate([g[0:16] - halo, g[16:] - g[:TQ - 16]], axis=0)
        for gi in range(G):
            g_buf[gi, _ds(t.prev, 16 + TQ, 16, 32), :] = g[0:16, gi * 128:(gi + 1) * 128]
        for gi in range(G):
            g_buf[gi, _ds(t.cb, 16, TQ, 32), :] = g[:, gi * 128:(gi + 1) * 128]
            g_buf[G + gi, _ds(t.cb, 16, TQ, 32), :] = e[:, gi * 128:(gi + 1) * 128]
        for gi in range(G):
            g_buf[gi, _ds(t.next, 0, 16, 32), :] = g[TQ - 16:TQ, gi * 128:(gi + 1) * 128]

    def m_store(t, g0, v, r0=0):
        n = v.shape[0]
        halo = jnp.concatenate([m_buf[g0 + gi, _ds(t.cb, 16 + r0, 16, 32), :] for gi in range(G)], axis=1)
        parts = [v[0:16] - halo, v[16:] - v[:n - 16]]
        if r0 + n == TQ:
            parts.append(-v[n - 16:])
        e = jnp.concatenate(parts, axis=0)
        for gi in range(G):
            m_buf[g0 + gi, _ds(t.cb, 32 + r0, n, 32), :] = v[:, gi * 128:(gi + 1) * 128]
            m_buf[2 * G + g0 + gi, _ds(t.cb, 32 + r0, e.shape[0], 32), :] = e[:, gi * 128:(gi + 1) * 128]
        if n == TQ:
            for gi in range(G):
                m_buf[g0 + gi, _ds(t.next, 0, 32, 32), :] = v[TQ - 32:TQ, gi * 128:(gi + 1) * 128]
                m_buf[2 * G + g0 + gi, _ds(t.next, 16, 16, 32), :] = e[TQ - 16:TQ, gi * 128:(gi + 1) * 128]

    def mlp_out(t):
        gc = jnp.concatenate([_conv(g_buf, gi, G + gi, dw_f, 2 * G + gi, t.cb, 16, TQ, K) for gi in range(G)], axis=-1)
        u = u_ref[_ds(t.fb, 0, TQ, 16), :]
        loc = jnp.dot((u * gc).astype(BF16), _upk(wmo_p[...]), preferred_element_type=F32)
        m_store(t, G, loc)

    def merge_half(half, pieces):
        lhs = []
        for (t, off, nrows, _) in pieces:
            ms = [_conv(m_buf, gi, 2 * G + gi, dw_f, gi, t.cb, 32 - LAG + off, nrows, K)
                  for gi in range(half * G, (half + 1) * G)]
            lhs.append(jnp.concatenate(ms, axis=-1))
        lhs = lhs[0] if len(lhs) == 1 else jnp.concatenate(lhs, axis=0)
        return jnp.dot(lhs.astype(BF16), _upk(wm_p[half * D // 2:(half + 1) * D // 2, :]),
                       preferred_element_type=F32)

    def merge_loc(pieces):
        y = merge_half(1, pieces)
        r = 0
        for (t, off, nrows, yo) in pieces:
            y_ref[yo:yo + nrows, :] = x_buf[_ds(t.fb, off, nrows, 16), :].astype(F32) + y[r:r + nrows]
            r += nrows

    def merge_glob(pieces):
        y = merge_half(0, pieces)
        r = 0
        for (t, off, nrows, yo) in pieces:
            o_buf[_ds(t.fb, off, nrows, 16), :] = (y_ref[yo:yo + nrows, :] + y[r:r + nrows]).astype(BF16)
            r += nrows

    def max_update(ml, first, final):
        if final:
            return jnp.maximum(mp_ref[0:TQ], ml)
        mp_ref[0:TQ] = ml if first else jnp.maximum(mp_ref[0:TQ], ml)

    def scores_pair(t, a, b, pos):
        def nt(l, w):
            return lax.dot_general(_upk(l), _upk(w), NT_DIMS, preferred_element_type=F32)
        h1, h2, hs = R1 // 2, R2 // 2, 48
        f = {
            1: lambda j: nt(qc_ref[0:h1, 0:128], kc(t, j, 0)),
            11: lambda j: nt(qc_ref[0:hs, 0:128], kc(t, j, 0)),
            12: lambda j: nt(qc_ref[hs:h1, 0:128], kc(t, j, 0)),
            2: lambda j: nt(q_ref[0:h1, 0:128], kc(t, j, 4)),
            3: lambda j: nt(qc_ref[0:h2, 384:512], k_alo(t, j)),
            4: lambda j: nt(qc_ref[0:h1, 128:256], k_bhi(t, j)),
            5: lambda j: nt(q_ref[h1:TQ // 2, 128:256], kc(t, j, 3)),
            6: lambda j: nt(qc_ref[0:h2, 512:640], kc(t, j, 2)),
            7: lambda j: nt(qc_ref[0:h1, 256:384], kc(t, j, 1)),
            71: lambda j: nt(qc_ref[0:hs, 256:384], kc(t, j, 1)),
            72: lambda j: nt(qc_ref[hs:h1, 256:384], kc(t, j, 1)),
        }
        for j, order in ((a, (2, 4, 3, 5)), (b, (3, 5, 2, 4))):
            m = {k: f[k](j) for k in order}
            if j == a:
                last[0] = m[2][0:16]
            c0 = j * CK
            s_ref[0:R1, c0 + 128:c0 + 256] = m[2] + m[4]
            s_ref[R1:TQ, c0:c0 + 128] = m[3] + m[5]
            s_ref[0:R1, c0:c0 + 128] = _cat0(m[4][0:R2] - m[5], m[4][R2:])
            s_ref[R1:TQ, c0 + 128:c0 + 256] = m[3] - m[2][0:R2]

        def off_diag(j):
            return _cat0(s_ref[0:R1, j * CK + 128:j * CK + 256], s_ref[R1:TQ, j * CK:j * CK + 128])

        def diag(j):
            return _cat0(s_ref[0:R1, j * CK:j * CK + 128], s_ref[R1:TQ, j * CK + 128:j * CK + 256])
        m1, m7, m6, m6b = f[1](a), f[7](a), f[6](a), f[6](b)
        c0 = a * CK
        c11 = s_ref[0:R1, c0:c0 + 128] + (m1 + m7)
        c22 = s_ref[R1:TQ, c0 + 128:c0 + 256] + (m1[0:R2] + m6)
        s_ref[0:R1, c0:c0 + 128] = c11
        s_ref[R1:TQ, c0 + 128:c0 + 256] = c22
        c0 = b * CK
        s_ref[R1:TQ, c0 + 128:c0 + 256] += m6b
        m11, m71, m12, m72 = f[11](b), f[71](b), f[12](b), f[72](b)
        m1, m7 = _cat0(m11, m12), _cat0(m71, m72)
        c11 = s_ref[0:R1, c0:c0 + 128] + (m1 + m7)
        c22 = s_ref[R1:TQ, c0 + 128:c0 + 256] + m1[0:R2]
        s_ref[0:R1, c0:c0 + 128] = c11
        s_ref[R1:TQ, c0 + 128:c0 + 256] = c22
        ml = jnp.maximum(_cat0(c11, c22), off_diag(b))
        ml = jnp.maximum(ml, jnp.maximum(off_diag(a), diag(a)))
        return max_update(ml, pos == 0, pos >= NC - 2)

    def scores_chunk(t, j, pos):
        q = _upk(q_ref[0:TQ // 2, :])
        if (j + 1) * CK <= T:
            sj = lax.dot_general(q, xa_chunk(t, j), NT_DIMS, preferred_element_type=F32)
            sts = [sj[:, 0:128], sj[:, 128:256]]
        else:
            nrem = T - j * CK - 128
            assert 0 < nrem < 128 and nrem % 16 == 0
            kf = _upk(xa_ref[_ds(t.kb, j * CK // 2, 64, 16), :])
            sj = jnp.concatenate([lax.dot_general(q[0:R1], kf, NT_DIMS, preferred_element_type=F32),
                                  lax.dot_general(q[R1:TQ], kf, NT_DIMS, preferred_element_type=F32)], axis=0)
            kr = _upk(xa_ref[_ds(t.kb, j * CK // 2 + 64, nrem // 2, 16), :])
            st = lax.dot_general(kr, _upk(q_ref[...]), NT_DIMS, preferred_element_type=F32)
            st = jnp.concatenate([st, jnp.full((128 - nrem, st.shape[1]), -jnp.inf, F32)], axis=0)
            sts = [sj, st.T[0:TQ]]
        last[0] = sj[0:16, 0:128]
        s_ref[:, j * CK:j * CK + 128] = sts[0]
        s_ref[:, j * CK + 128:(j + 1) * CK] = sts[1]
        return max_update(jnp.maximum(sts[0], sts[1]), pos == 0, pos == NC - 1)

    def scores_fin(mpart):
        m = jnp.max(mpart, axis=-1, keepdims=True)
        lam = jnp.sum(jnp.exp2(mpart - m), axis=-1, keepdims=True)
        m = m + jnp.log(lam) * LOG2E
        mx_ref[0:TQ] = jnp.broadcast_to(m, (TQ, 128))

    def pv_group(t, js, first, r0=0, r1=R1, r2=R2):
        ra, rb, rc = r0, r0 + r1, r0 + r1 + r2
        L = {k: [] for k in range(1, 8)}
        l1 = l2 = None
        for j in js:
            c0 = j * CK
            a11 = jnp.exp2(s_ref[ra:rb, c0:c0 + 128] - mx_ref[ra:rb])
            a12 = jnp.exp2(s_ref[ra:rb, c0 + 128:c0 + 256] - mx_ref[ra:rb])
            a21 = jnp.exp2(s_ref[rb:rc, c0:c0 + 128] - mx_ref[rb:rc])
            a22 = jnp.exp2(s_ref[rb:rc, c0 + 128:c0 + 256] - mx_ref[rb:rc])
            s1 = a11 + a12
            s2 = a21 + a22
            l1 = s1 if l1 is None else l1 + s1
            l2 = s2 if l2 is None else l2 + s2
            L[1].append(_cat0(a11[0:r2] + a22, a11[r2:]))
            L[2].append(s2)
            L[3].append(a11)
            L[4].append(a22)
            L[5].append(s1)
            L[6].append(a21 - a11[0:r2])
            L[7].append(_cat0(a12[0:r2] - a22, a12[r2:]))
        W = {1: lambda j: kc(t, j, 0), 2: lambda j: k_alo(t, j), 3: lambda j: kc(t, j, 1), 4: lambda j: kc(t, j, 2),
             5: lambda j: k_bhi(t, j), 6: lambda j: kc(t, j, 3), 7: lambda j: kc(t, j, 4)}
        for i, k in enumerate(VSEQ):
            lhs = jnp.concatenate(L[k], axis=1).astype(BF16)
            rhs = _upk(jnp.concatenate([W[k](j) for j in js], axis=0))
            mk = jnp.dot(lhs, rhs, preferred_element_type=F32)
            last[0] = mk[0:16]
            if i == 0:
                first_w[0] = mk[0:16]
            n = mk.shape[0]
            if first:
                acc7_ref[k, 0:n] = mk
            else:
                acc7_ref[k, 0:n] += mk
        lloc = _cat0(l1, l2)
        if first:
            lp_ref[ra:rc] = lloc
        else:
            lp_ref[ra:rc] += lloc

    def pv_fin(t, r0=0, r1=R1, r2=R2):
        l = jnp.sum(lp_ref[r0:r0 + r1 + r2], axis=-1, keepdims=True)
        m1, m3, m5, m7 = (acc7_ref[k, 0:r1] for k in (1, 3, 5, 7))
        m2, m4, m6 = (acc7_ref[k, 0:r2] for k in (2, 4, 6))
        c11 = m1 + (m7 - m5)
        c11 = _cat0(c11[0:r2] + m4, c11[r2:])
        c12 = m3 + m5
        c21 = m2 + m4
        c22 = (m1[0:r2] - m2) + (m3[0:r2] + m6)
        acc = jnp.concatenate([jnp.concatenate([c11, c12], axis=1), jnp.concatenate([c21, c22], axis=1)], axis=0)
        o = acc * (1.0 / l)
        glob = jnp.dot(o.astype(BF16), _upk(wvo_p[...]), preferred_element_type=F32)
        m_store(t, 0, glob, r0)

    def pv_chunk(t, j, r0, n):
        c0 = j * CK
        pa = jnp.exp2(s_ref[r0:r0 + n, c0:c0 + 128] - mx_ref[r0:r0 + n])
        pb = jnp.exp2(s_ref[r0:r0 + n, c0 + 128:c0 + 256] - mx_ref[r0:r0 + n])
        lloc = pa + pb
        pv = jnp.dot(jnp.concatenate([pa, pb], axis=-1).astype(BF16), xa_chunk(t, j), preferred_element_type=F32)
        last[0] = pv[0:16, 0:128]
        if j == 0:
            lp_ref[r0:r0 + n] = lloc
            acc_ref[r0:r0 + n] = pv
        else:
            lp_ref[r0:r0 + n] += lloc
            acc_ref[r0:r0 + n] += pv

    def pv_chunk_fin(t, r0, n):
        l = jnp.sum(lp_ref[r0:r0 + n], axis=-1, keepdims=True)
        o = (acc_ref[r0:r0 + n] * (1.0 / l)).astype(BF16)
        glob = jnp.dot(o, _upk(wvo_p[...]), preferred_element_type=F32)
        m_store(t, 0, glob, r0)

    def anchor(op):
        if op == 'Zx':
            zrow = pl.multiple_of(zoff[0], 16)
            x_buf[pl.ds(zrow + B * T + LAG + TP - T, 16), 0:128] = last[0].astype(BF16)
            return
        zrow = pl.multiple_of(zoff[0], 8)
        if op in ('Z', 'Zg'):
            (m_buf if op == 'Z' else g_buf)[0, pl.ds(zrow + NS * SLOT + 64, 8), :] = last[0][0:8]
        else:
            (lp_ref if op == 'Zl' else mx_ref)[pl.ds(zrow + TQ, 8), :] = last[0][0:8]

    def step(order, pb, pa, t0, tp, th=None, un=None, dma=None):
        cord, nxt = [], 0
        for op in order:
            if op == 'KK':
                cord += [nxt, nxt + 1]
                nxt += 2
            elif op in ('Ks', 'K'):
                cord.append(NC - 2 if op == 'Ks' else NC - 1)
        assert 4 * order.count('W') == NC and sorted(cord) == list(range(NC))
        mpart = None
        jv = jk = 0
        nq = []
        for op in order:
            if op == 'q':
                qproj(tp)
            elif op == 'W':
                pv_group(t0, cord[jv:jv + 4], jv == 0)
                jv += 4
            elif op == 'G':
                pv_fin(t0)
            elif op in ('K', 'Ks'):
                assert jk < jv
                mpart = scores_chunk(tp, cord[jk], jk)
                jk += 1
            elif op == 'KK':
                assert jk + 1 < jv
                mpart = scores_pair(tp, cord[jk], cord[jk + 1], jk)
                jk += 2
            elif op[0] == 'Z':
                anchor(op)
            elif op == 'Ma':
                merge_loc(pa)
            elif op == 'Mb':
                merge_glob(pb)
            elif op == 'H':
                mlp_in(th)
            elif op == 'L':
                mlp_out(tp)
            elif op == 'n':
                r = (len(nq) // 2) * 256 + (len(nq) % 2) * 64
                xa_, xb_ = (_ln(x_buf[_ds(un * 512, LAG + T + r + o, 64, 16), :].astype(F32)) for o in (0, 128))
                v = jnp.concatenate(
                    [xa_, xb_] + _key_combos(xa_[:, 0:128], xa_[:, 128:256], xb_[:, 0:128], xb_[:, 128:256]), axis=1)
                nq.append((r, _pk(v.astype(BF16))))
            elif op == 'Ns':
                assert len(nq) == 4
                for r, v in nq:
                    xa_ref[_ds(un * 256, TP // 2 + r // 2, 32, 256), :] = v[:, 0:256]
                    xa_ref[_ds(un * 256, TP // 2 + r // 2 + 64, 32, 256), :] = v[:, 256:512]
                    kc_ref[_ds(un * 128, TP // 4 + (r // 256) * 64 + (r % 256) // 2, 32, 128), :] = v[:, 512:1152]
            elif op == 'D':
                dma()
            else:
                raise ValueError(op)
        scores_fin(mpart)

    done, nln = [], 0
    for op in PROLOGUE[split + 1:]:
        if op[0] == 's':
            dma_start(op)
        elif op[0] == 'x':
            x_copy(int(op[1:])).wait()
        elif op[0] == 'w':
            w_copy(int(op[1:])).wait()
        elif op[0] == 'n':
            ln_unit(int(op[1:]))
            nln = int(op[1:]) + 1
        elif op[0] == 'p':
            prep(int(op[1:]))
        elif op == 'A':
            prep_a()
        elif op == 'q':
            qproj(tile(0), False)
        elif op.startswith('KK'):
            j = int(op[2:])
            assert nln * 512 >= (j + 2) * CK
            mpart = scores_pair(tile(0), j, j + 1, len(done))
            done += [j, j + 1]
        elif op[0] == 'K':
            j = int(op[1:])
            assert nln * 512 >= (j + 1) * CK
            mpart = scores_chunk(tile(0), j, len(done))
            done.append(j)
        elif op[0] == 'H':
            assert nln * 512 >= (int(op[1:]) + 1) * TQ
            mlp_in(tile(int(op[1:])))
        elif op == 'L0':
            mlp_out(tile(0))
        elif op[0] == 'Z':
            anchor(op)
        else:
            raise ValueError(op)
    assert sorted(done) == list(range(NC))
    scores_fin(mpart)

    def body_a(order, s, c):
        if 'Ns' in order:
            @pl.when(s == 1)
            def _():
                x_copy(NU + 1).wait()

        w = jnp.maximum(s - 1, 0)
        fb = w * TQ

        def dma():
            @pl.when(s > 0)
            def _():
                out_copy(fb, LAG, TQ - LAG).start()

            @pl.when(jnp.logical_and(s > 1, s != NT + 1))
            def _():
                out_copy(fb, 0, LAG).start()

        step(order, [(tile(w), 0, TQ, 0)], [(tile(s), 0, TQ, 0)], tile(s), tile(s + 1), tile(s + 3), s, dma)
        return c
    lax.fori_loop(0, NU, functools.partial(body_a, STEP_A1), 0)
    lax.fori_loop(NU, NS - 3, functools.partial(body_a, STEP_A2), 0)

    z = zoff[0]
    tail0 = (tile(NT - 1), TQ, LAG, TQ + LAG)
    Y2 = TQ + 3 * LAG

    def body_b(s, c):
        step(STEP_B, [(tile(s - 1), 0, TQ, 0)], [(tile(s), 0, TQ, 0), tail0], tile(s), tile(s + 1))
        out_copy((s - 1) * TQ, 0, TQ).start()
        return c
    lax.fori_loop(NS - 3, NS - 1, body_b, 0)

    def last_block(ops):
        tl = tile(z + (NS - 1))
        j = 0
        saved = None
        for op in ops:
            if op == 'WA':
                pv_group(tl, list(range(j, j + 4)), j == 0, 0, RA // 2, RA // 2)
                j += 4
            elif op == 'B':
                pv_chunk(tl, j, RA, TQ - RA)
                j += 1
            elif op == 'Ga':
                pv_fin(tl, 0, RA // 2, RA // 2)
            elif op == 'Gb':
                pv_chunk_fin(tl, RA, TQ - RA)
            elif op == 'E':
                last[0] = first_w[0]
            elif op == 'S':
                saved = last[0]
            elif op == 'R':
                last[0] = saved
            elif op[0] == 'Z':
                anchor(op)
            elif op == 'Mb':
                merge_glob([(tile(z + (NS - 2)), 0, TQ, 0), tail0])
                out_copy(0, (NS - 2) * TQ, TQ).start()
                out_copy(0, NT * TQ, LAG).start()
            elif op == 'Mc':
                merge_loc([(tl, 0, TQ + LAG, Y2)])
            elif op == 'M1':
                merge_glob([(tl, 0, RA, Y2)])
                out_copy(0, (NS - 1) * TQ, RA).start()
            elif op == 'M2':
                merge_glob([(tl, RA, TQ + LAG - RA, Y2 + RA)])
                out_copy(0, (NS - 1) * TQ + RA, TQ + LAG - RA).start()
            else:
                raise ValueError(op)
        assert j == NC

    pl.when(z < 1)(functools.partial(last_block, LAST_A))
    pl.when(z < 2)(functools.partial(last_block, LAST_B))

    out_copy(0, LAG, B * T).wait()


@jax.jit
def pallas_standalone__conformer_family_e_branchformer__speech_kernel(
    x: jax.Array,
    w_qkv: jax.Array,
    w_att_out: jax.Array,
    w_mlp_in: jax.Array,
    dw_csgu: jax.Array,
    w_mlp_out: jax.Array,
    dw_merge: jax.Array,
    w_merge: jax.Array,
):
    B, T, D = x.shape
    K = dw_csgu.shape[0]
    TP = (T + 511) // 512 * 512
    G = D // 128
    RB = (B * (T // TQ) + 1) * SLOT
    out = pl.pallas_call(
        functools.partial(_kernel, B=B, T=T, D=D, K=K, TP=TP),
        in_specs=[pl.BlockSpec(memory_space=pl.ANY)] * 8,
        out_specs=pl.BlockSpec(memory_space=pl.ANY),
        out_shape=jax.ShapeDtypeStruct((B * T, D), x.dtype),
        scratch_shapes=[
            pltpu.VMEM((B * T + 32 + TP - T, D), BF16),
            pltpu.VMEM((B * T + 32, D), BF16),
            pltpu.VMEM((B * TP // 2, D), U32),
            pltpu.VMEM((D // 2, D), U32),
            pltpu.VMEM((D // 2, D), U32),
            pltpu.VMEM((D // 2, 2 * D), U32),
            pltpu.VMEM((D // 2, D), U32),
            pltpu.VMEM((D, D), U32),
            pltpu.VMEM((64, 896), U32),
            pltpu.VMEM((3 * G, 48, 8, 128), F32),
            pltpu.VMEM((2 * G, RB, 128), F32),
            pltpu.VMEM((4 * G, RB, 128), F32),
            pltpu.VMEM((B * T, D), F32),
            pltpu.VMEM((TQ, TP), F32),
            pltpu.VMEM((TQ + 16, 128), F32),
            pltpu.VMEM((256, D), U32),
            pltpu.VMEM((128, 640), U32),
            pltpu.VMEM((B * TP // 4, 640), U32),
            pltpu.VMEM((TQ + 16, 128), F32),
            pltpu.VMEM((TQ + 16, 128), F32),
            pltpu.VMEM((TQ, D), F32),
            pltpu.VMEM((8, 224, 128), F32),
            pltpu.VMEM((2 * TQ + 4 * LAG, D), F32),
            pltpu.VMEM(w_qkv.shape, BF16),
            pltpu.VMEM(w_att_out.shape, BF16),
            pltpu.VMEM(w_mlp_in.shape, BF16),
            pltpu.VMEM(dw_csgu.shape, BF16),
            pltpu.VMEM(w_mlp_out.shape, BF16),
            pltpu.VMEM(dw_merge.shape, BF16),
            pltpu.VMEM(w_merge.shape, BF16),
            pltpu.SMEM((1,), jnp.int32),
            pltpu.SemaphoreType.DMA((max(GRP.values()) + 1,)),
            pltpu.SemaphoreType.DMA,
        ],
        compiler_params=pltpu.CompilerParams(vmem_limit_bytes=120 * 1024 * 1024, disable_bounds_checks=True),
    )(x.reshape(B * T, D), w_qkv, w_att_out, w_mlp_in, dw_csgu, w_mlp_out, dw_merge, w_merge)
    return out.reshape(B, T, D)
```

```python
import functools

import jax
import jax.numpy as jnp
from jax import lax
import jax.experimental.pallas as pl
import jax.experimental.pallas.tpu as pltpu

F32 = jnp.float32
BF16 = jnp.bfloat16
U32 = jnp.uint32
LOG2E = 1.4426950408889634
NT_DIMS = (((1,), (1,)), ((), ()))

TQ = 400
CK = 256
SLOT = 448
LAG = 16
R1 = 208
R2 = TQ - R1
RA = 288
VSEQ = (3, 4, 1, 5, 7, 2, 6)

PROLOGUE = (
    'sx0 sw0 | x0 sx1 sw1 n0 w0 sx2 sx3 A q x1 w1 sx4 sx5 sw3 sw4 p1 H0 n1 KK0 '
    'x2 x3 x4 sx6 sx7 sw2 sw5 sw6 sw7 sx8 n2 n3 KK2 KK4 KK6 H1 H2 n4 K8 '
    'x5 x6 x7 w3 w4 w2 w5 w6 w7 x8 sx9 p3 p4 p5 p6 n5 K9 Zg KK10 n6 KK12 n7 K15 K14 p2 L0').split()
STEP_A1 = 'q Z Zg W W Mb K Ks D W Ma W Zl L H KK KK Zx n KK Zx n KK Zx n KK Zx n KK KK Ns G'.split()
STEP_A2 = 'q Z Zg W W Mb K Ks D W Ma W Zl L H KK KK KK KK KK KK KK G'.split()
STEP_B = 'q Z Zg W W Mb K Ks W Ma W Zl L KK KK KK KK KK KK KK G'.split()
LAST_A = 'WA E Z WA WA Mb WA Zl Mc Ga'.split()
LAST_B = 'B Z S B B R Zm B S B B R Zm B B B B B B B B B B Zl M1 Gb M2'.split()


def _sem_groups():
    grp, g, prev = {}, -1, False
    for op in PROLOGUE:
        is_wait = op[0] in 'xw'
        if is_wait:
            g += 0 if prev else 1
            grp[op] = g
        prev = is_wait
    grp['x9'] = g + 1
    return grp


GRP = _sem_groups()


def _pk(x):
    return pltpu.bitcast(x, U32)


def _upk(x):
    return pltpu.bitcast(x, BF16)


def _cat0(u, v):
    return jnp.concatenate([u, v], axis=0) if v.shape[0] else u


def _ln(x, eps=1e-5):
    m = jnp.mean(x, axis=-1, keepdims=True)
    xc = x - m
    v = jnp.mean(xc * xc, axis=-1, keepdims=True)
    return xc * jnp.exp2(jnp.log(v + eps) * (-0.5 * LOG2E))


def _gelu(x):
    c = 0.7978845608028654
    hx = 0.5 * x
    return hx + hx * jnp.tanh(x * (c + (c * 0.044715) * (x * x)))


def _ds(base, off, n, align):
    if isinstance(base, int):
        return pl.ds(base + off, n)
    a = align
    while off % a:
        a //= 2
    return pl.ds(pl.multiple_of(base + off, a), n) if a > 1 else pl.ds(base + off, n)


def _conv_direct(buf_ref, g, w_ref, wg, base, off, nrows, K):
    V = nrows // 8
    acc = None
    for p in range(8):
        taps = list(range(p, K, 8))
        nq = V + len(taps) - 1
        slab = buf_ref[g, _ds(base, off + p - K // 2, 8 * nq, 32), :].reshape(nq, 8, 128)
        for qi, i in enumerate(taps):
            term = slab[qi:qi + V] * w_ref[wg, i][None]
            acc = term if acc is None else acc + term
    return acc.reshape(8 * V, 128)


def _conv(buf_ref, g, ge, w_ref, wg, base, off, nrows, K):
    nq = nrows // 32
    outs = []
    q0 = 0
    while q0 < nq:
        Q = min(4, nq - q0)
        am = a0 = a1 = None
        for i in [p + 8 * h for p in range(8) for h in range(2)]:
            r = off + 32 * q0 + i - K // 2 + 16
            xs = buf_ref[g, _ds(base, r, 32 * Q - 16, 32), :]
            xs = jnp.concatenate([xs[32 * k:32 * k + 16] for k in range(Q)], axis=0).reshape(2 * Q, 8, 128)
            t = xs * w_ref[wg, 32 + i][None]
            am = t if am is None else am + t
            if i + 16 < K:
                es = buf_ref[ge, _ds(base, r, 32 * Q, 32), :]
                e2 = jnp.concatenate([es[32 * k + 16:32 * k + 32] for k in range(Q)], axis=0).reshape(2 * Q, 8, 128)
                t = e2 * w_ref[wg, i + 16][None]
                a1 = t if a1 is None else a1 + t
            else:
                es = buf_ref[ge, _ds(base, r, 32 * Q - 16, 32), :]
            e1 = jnp.concatenate([es[32 * k:32 * k + 16] for k in range(Q)], axis=0).reshape(2 * Q, 8, 128)
            t = e1 * w_ref[wg, i][None]
            a0 = t if a0 is None else a0 + t
        y0 = (am - a0).reshape(16 * Q, 128)
        y1 = (am + a1).reshape(16 * Q, 128)
        for k in range(Q):
            outs += [y0[16 * k:16 * k + 16], y1[16 * k:16 * k + 16]]
        q0 += Q
    if nrows % 32:
        outs.append(_conv_direct(buf_ref, g, w_ref, wg, base, off + 32 * nq, nrows - 32 * nq, K))
    return jnp.concatenate(outs, axis=0) if len(outs) > 1 else outs[0]


def _key_combos(alo, ahi, blo, bhi):
    return [alo + bhi, ahi - bhi, blo - alo, alo + ahi, blo + bhi]


class _Tile:
    def __init__(self, t, NT, NS, TP, T):
        if isinstance(t, int):
            b = t // NT
            self.prev = (NS if t % NT == 0 else t - 1) * SLOT
            self.next = (NS if t % NT == NT - 1 else t + 1) * SLOT
        else:
            b = (t >= NT).astype(jnp.int32)
            first = jnp.logical_or(t == 0, t == NT)
            last = jnp.logical_or(t == NT - 1, t == NS - 1)
            self.prev = jnp.where(first, NS, t - 1) * SLOT
            self.next = jnp.where(last, NS, t + 1) * SLOT
        self.cb = t * SLOT
        self.fb = t * TQ
        self.ab = t * (TQ // 2) + b * ((TP - T) // 2)
        self.kb = b * (TP // 2)
        self.cbk = b * (TP // 4)


def _kernel(x_hbm, wqkv_hbm, wao_hbm, wmi_hbm, dwc_hbm, wmo_hbm, dwm_hbm, wm_hbm, o_hbm,
            x_buf, o_buf, xa_ref, wa_p, wvo_p, wmi_p, wmo_p, wm_p, ws_ref, dw_f, g_buf, m_buf, u_ref,
            s_ref, mx_ref, q_ref, qc_ref, kc_ref, mp_ref, lp_ref, acc_ref, acc7_ref, y_ref,
            wqkv_ref, wao_ref, wmi_ref, dwc_ref, wmo_ref, dwm_ref, wm_ref,
            zoff, sem_in, sem_out,
            *, B, T, D, K, TP):
    NT = T // TQ
    NS = B * NT
    G = D // 128
    NC = TP // CK
    NU = TP // 512
    assert B == 2 and D == 256 and K == 31 and T % TQ == 0 and NC == 16
    last = [None]
    first_w = [None]

    def tile(t):
        return _Tile(t, NT, NS, TP, T)

    def x_copy(u):
        r0 = u * 512 if u < NU else (T if u == NU else T + 512)
        n = min(512, T - r0) if u < NU else (512 if u == NU else T - 512)
        return pltpu.make_async_copy(x_hbm.at[pl.ds(r0, n), :], x_buf.at[pl.ds(LAG + r0, n), :],
                                     sem_in.at[GRP['x%d' % u]])

    w_pairs = [(wqkv_hbm.at[:, 0:2 * D], wqkv_ref.at[:, 0:2 * D]), (wmi_hbm, wmi_ref), (wao_hbm, wao_ref),
               (dwc_hbm, dwc_ref), (wmo_hbm, wmo_ref), (dwm_hbm, dwm_ref), (wm_hbm, wm_ref),
               (wqkv_hbm.at[:, 2 * D:3 * D], wqkv_ref.at[:, 2 * D:3 * D])]

    def w_copy(k):
        return pltpu.make_async_copy(w_pairs[k][0], w_pairs[k][1], sem_in.at[GRP['w%d' % k]])

    def dma_start(op):
        (x_copy if op[1] == 'x' else w_copy)(int(op[2:])).start()

    def out_copy(base, off, n):
        return pltpu.make_async_copy(o_buf.at[_ds(base, off, n, 16), :], o_hbm.at[_ds(base, off - LAG, n, 16), :],
                                     sem_out)

    split = PROLOGUE.index('|')
    for op in PROLOGUE[:split]:
        dma_start(op)

    zoff[0] = 0
    z16 = jnp.zeros((16, 128), F32)
    for b in range(B):
        lo, hi = b * NT * SLOT, ((b + 1) * NT - 1) * SLOT
        for gi in range(G):
            g_buf[gi, lo:lo + 16, :] = z16
            g_buf[gi, hi + 416:hi + 432, :] = z16
        for gi in range(2 * G):
            m_buf[gi, lo:lo + 16, :] = z16
            m_buf[gi, lo + 16:lo + 32, :] = z16
            m_buf[2 * G + gi, lo + 16:lo + 32, :] = z16
            m_buf[gi, hi + 432:hi + 448, :] = z16
    x_buf[0:LAG, :] = jnp.zeros((LAG, D), BF16)
    x_buf[LAG + B * T:LAG + B * T + TP - T, :] = jnp.zeros((TP - T, D), BF16)
    q_ref[TQ // 2:, :] = jnp.zeros((q_ref.shape[0] - TQ // 2, D), U32)

    def prep_a():
        a = lax.dot_general(wqkv_ref[:, 0:D], wqkv_ref[:, D:2 * D], NT_DIMS, preferred_element_type=F32)
        a = a * (D ** -0.5 * LOG2E)
        wa_p[...] = _pk(a.astype(BF16))
        b11, b12, b21, b22 = a[0:128, 0:128], a[0:128, 128:256], a[128:256, 0:128], a[128:256, 128:256]
        ws_ref[...] = _pk(jnp.concatenate(
            [b11 + b22, b11, b12 - b22, b21 - b11, b22, b11 + b12, b21 + b22], axis=1).astype(BF16))

    def prep(k):
        if k == 1:
            wmi_p[...] = _pk(wmi_ref[...])
        elif k == 2:
            wvo = jnp.dot(wqkv_ref[:, 2 * D:3 * D], wao_ref[...], preferred_element_type=F32)
            wvo_p[...] = _pk(wvo.astype(BF16))
        elif k == 4:
            wmo_p[...] = _pk(wmo_ref[...])
        elif k == 6:
            wm_p[...] = _pk(wm_ref[...])
        else:
            dw = (dwc_ref if k == 3 else dwm_ref)[...].astype(F32)
            g0 = 2 * G if k == 3 else 0
            if k == 5:
                row = lax.broadcasted_iota(jnp.int32, dw.shape, 0)
                dw = jnp.where(row == K // 2, dw + 1.0, dw)
            for gi in range(dw.shape[1] // 128):
                for i in range(K):
                    dw_f[g0 + gi, i] = jnp.broadcast_to(dw[i:i + 1, gi * 128:(gi + 1) * 128], (8, 128))
                for i in range(16):
                    v = dw_f[g0 + gi, i]
                    dw_f[g0 + gi, 32 + i] = v + dw_f[g0 + gi, i + 16] if i + 16 < K else v

    def ln_unit(u):
        n = min(512, T - u * 512)
        xk = _ln(x_buf[pl.ds(LAG + u * 512, n), :].astype(F32))
        if n < 512:
            xk = jnp.concatenate([xk, jnp.zeros((512 - n, D), F32)], axis=0)
        vs = []
        for r in (0, 256):
            vs.append(jnp.concatenate(_key_combos(xk[r:r + 128, 0:128], xk[r:r + 128, 128:256],
                                                  xk[r + 128:r + 256, 0:128], xk[r + 128:r + 256, 128:256]), axis=1))
        xa_p, kc_p = _pk(xk.astype(BF16)), _pk(jnp.concatenate(vs, axis=0).astype(BF16))
        xa_ref[u * 256:(u + 1) * 256, :] = xa_p
        kc_ref[u * 128:(u + 1) * 128, :] = kc_p

    def xq_of(t):
        return _upk(xa_ref[_ds(t.ab, 0, TQ // 2, 8), :])

    def xa_chunk(t, j):
        return _upk(xa_ref[_ds(t.kb, j * CK // 2, CK // 2, 16), :])

    def kc(t, j, i):
        return kc_ref[_ds(t.cbk, j * 64, 64, 32), i * 128:(i + 1) * 128]

    def k_alo(t, j):
        return xa_ref[_ds(t.kb, j * 128, 64, 16), 0:128]

    def k_bhi(t, j):
        return xa_ref[_ds(t.kb, j * 128 + 64, 64, 16), 128:256]

    def q_strassen(lhs):
        a11, a12, a21, a22 = lhs[0:R1, 0:128], lhs[0:R1, 128:256], lhs[R1:TQ, 0:128], lhs[R1:TQ, 128:256]
        p1 = jnp.concatenate([_cat0(a11[0:R2] + a22, a11[R2:]), a11, a11 + a12, _cat0(a12[0:R2] - a22, a12[R2:])],
                             axis=1).astype(BF16)
        p2 = jnp.concatenate([a21 + a22, a22, a21 - a11[0:R2]], axis=1).astype(BF16)
        lk = {1: p1[:, 0:128], 3: p1[:, 128:256], 5: p1[:, 256:384], 7: p1[:, 384:512],
              2: p2[:, 0:128], 4: p2[:, 128:256], 6: p2[:, 256:384]}

        def job(k, lo=None, hi=None):
            l = lk[k] if lo is None else lk[k][lo:hi]
            return jnp.dot(l, _upk(ws_ref[:, (k - 1) * 128:k * 128]), preferred_element_type=F32)
        s1, s2 = 144, 160
        m3, m5, m2, m4 = job(3), job(5), job(2), job(4)
        m6a = job(6, 0, s2)
        m1b = job(1, s1, R1)
        m1a = job(1, 0, s1)
        m7a = job(7, 0, s1)
        m7b = job(7, s1, R1)
        m6 = _cat0(m6a, job(6, s2, R2))
        m1, m7 = _cat0(m1a, m1b), _cat0(m7a, m7b)
        c12 = m3 + m5
        c21 = m2 + m4
        last[0] = c12[0:16] + c21[0:16]
        c11 = _cat0(m4 - m5[0:R2], -m5[R2:]) + (m1 + m7)
        c22 = ((m3[0:R2] - m2) + m6) + m1[0:R2]
        return jnp.concatenate([jnp.concatenate([c11, c12], axis=1), jnp.concatenate([c21, c22], axis=1)], axis=0)

    def qproj(t, fast=True):
        if fast:
            qf = q_strassen(xq_of(t).astype(F32))
        else:
            qf = jnp.dot(xq_of(t), _upk(wa_p[...]), preferred_element_type=F32)
            last[0] = qf[0:16, 0:128]
        q_ref[0:TQ // 2, :] = _pk(qf.astype(BF16))
        a11, a12 = qf[0:R1, 0:128], qf[0:R1, 128:256]
        a21, a22 = qf[R1:TQ, 0:128], qf[R1:TQ, 128:256]
        qc_ref[0:R1 // 2, 0:384] = _pk(jnp.concatenate(
            [_cat0(a11[0:R2] + a22, a11[R2:]), a12 - a11, _cat0(a12[0:R2] + a22, a12[R2:])], axis=1).astype(BF16))
        qc_ref[0:R2 // 2, 384:640] = _pk(jnp.concatenate([a21 - a22, a11[0:R2] + a21], axis=1).astype(BF16))

    def mlp_in(t):
        hp = jnp.dot(xq_of(t), _upk(wmi_p[...]), preferred_element_type=F32)
        last[0] = hp[0:16, 0:128]
        h = _gelu(hp)
        u_ref[_ds(t.fb, 0, TQ, 16), :] = h[:, :D]
        g = _ln(h[:, D:])
        halo = jnp.concatenate([g_buf[gi, _ds(t.cb, 0, 16, 32), :] for gi in range(G)], axis=1)
        e = jnp.concatenate([g[0:16] - halo, g[16:] - g[:TQ - 16]], axis=0)
        for gi in range(G):
            g_buf[gi, _ds(t.prev, 16 + TQ, 16, 32), :] = g[0:16, gi * 128:(gi + 1) * 128]
        for gi in range(G):
            g_buf[gi, _ds(t.cb, 16, TQ, 32), :] = g[:, gi * 128:(gi + 1) * 128]
            g_buf[G + gi, _ds(t.cb, 16, TQ, 32), :] = e[:, gi * 128:(gi + 1) * 128]
        for gi in range(G):
            g_buf[gi, _ds(t.next, 0, 16, 32), :] = g[TQ - 16:TQ, gi * 128:(gi + 1) * 128]

    def m_store(t, g0, v, r0=0):
        n = v.shape[0]
        halo = jnp.concatenate([m_buf[g0 + gi, _ds(t.cb, 16 + r0, 16, 32), :] for gi in range(G)], axis=1)
        parts = [v[0:16] - halo, v[16:] - v[:n - 16]]
        if r0 + n == TQ:
            parts.append(-v[n - 16:])
        e = jnp.concatenate(parts, axis=0)
        for gi in range(G):
            m_buf[g0 + gi, _ds(t.cb, 32 + r0, n, 32), :] = v[:, gi * 128:(gi + 1) * 128]
            m_buf[2 * G + g0 + gi, _ds(t.cb, 32 + r0, e.shape[0], 32), :] = e[:, gi * 128:(gi + 1) * 128]
        if n == TQ:
            for gi in range(G):
                m_buf[g0 + gi, _ds(t.next, 0, 32, 32), :] = v[TQ - 32:TQ, gi * 128:(gi + 1) * 128]
                m_buf[2 * G + g0 + gi, _ds(t.next, 16, 16, 32), :] = e[TQ - 16:TQ, gi * 128:(gi + 1) * 128]

    def mlp_out(t):
        gc = jnp.concatenate([_conv(g_buf, gi, G + gi, dw_f, 2 * G + gi, t.cb, 16, TQ, K) for gi in range(G)], axis=-1)
        u = u_ref[_ds(t.fb, 0, TQ, 16), :]
        loc = jnp.dot((u * gc).astype(BF16), _upk(wmo_p[...]), preferred_element_type=F32)
        m_store(t, G, loc)

    def merge_half(half, pieces):
        lhs = []
        for (t, off, nrows, _) in pieces:
            ms = [_conv(m_buf, gi, 2 * G + gi, dw_f, gi, t.cb, 32 - LAG + off, nrows, K)
                  for gi in range(half * G, (half + 1) * G)]
            lhs.append(jnp.concatenate(ms, axis=-1))
        lhs = lhs[0] if len(lhs) == 1 else jnp.concatenate(lhs, axis=0)
        return jnp.dot(lhs.astype(BF16), _upk(wm_p[half * D // 2:(half + 1) * D // 2, :]),
                       preferred_element_type=F32)

    def merge_loc(pieces):
        y = merge_half(1, pieces)
        r = 0
        for (t, off, nrows, yo) in pieces:
            y_ref[yo:yo + nrows, :] = x_buf[_ds(t.fb, off, nrows, 16), :].astype(F32) + y[r:r + nrows]
            r += nrows

    def merge_glob(pieces):
        y = merge_half(0, pieces)
        r = 0
        for (t, off, nrows, yo) in pieces:
            o_buf[_ds(t.fb, off, nrows, 16), :] = (y_ref[yo:yo + nrows, :] + y[r:r + nrows]).astype(BF16)
            r += nrows

    def max_update(ml, first, final):
        if final:
            return jnp.maximum(mp_ref[0:TQ], ml)
        mp_ref[0:TQ] = ml if first else jnp.maximum(mp_ref[0:TQ], ml)

    def scores_pair(t, a, b, pos):
        def nt(l, w):
            return lax.dot_general(_upk(l), _upk(w), NT_DIMS, preferred_element_type=F32)
        h1, h2, hs = R1 // 2, R2 // 2, 48
        f = {
            1: lambda j: nt(qc_ref[0:h1, 0:128], kc(t, j, 0)),
            11: lambda j: nt(qc_ref[0:hs, 0:128], kc(t, j, 0)),
            12: lambda j: nt(qc_ref[hs:h1, 0:128], kc(t, j, 0)),
            2: lambda j: nt(q_ref[0:h1, 0:128], kc(t, j, 4)),
            3: lambda j: nt(qc_ref[0:h2, 384:512], k_alo(t, j)),
            4: lambda j: nt(qc_ref[0:h1, 128:256], k_bhi(t, j)),
            5: lambda j: nt(q_ref[h1:TQ // 2, 128:256], kc(t, j, 3)),
            6: lambda j: nt(qc_ref[0:h2, 512:640], kc(t, j, 2)),
            7: lambda j: nt(qc_ref[0:h1, 256:384], kc(t, j, 1)),
            71: lambda j: nt(qc_ref[0:hs, 256:384], kc(t, j, 1)),
            72: lambda j: nt(qc_ref[hs:h1, 256:384], kc(t, j, 1)),
        }
        for j, order in ((a, (2, 4, 3, 5)), (b, (3, 5, 2, 4))):
            m = {k: f[k](j) for k in order}
            c0 = j * CK
            c12 = m[2] + m[4]
            c21 = m[3] + m[5]
            if j == a:
                last[0] = c12[0:16] + c21[0:16]
            s_ref[0:R1, c0 + 128:c0 + 256] = c12
            s_ref[R1:TQ, c0:c0 + 128] = c21
            s_ref[0:R1, c0:c0 + 128] = _cat0(m[4][0:R2] - m[5], m[4][R2:])
            s_ref[R1:TQ, c0 + 128:c0 + 256] = m[3] - m[2][0:R2]

        def off_diag(j):
            return _cat0(s_ref[0:R1, j * CK + 128:j * CK + 256], s_ref[R1:TQ, j * CK:j * CK + 128])

        def diag(j):
            return _cat0(s_ref[0:R1, j * CK:j * CK + 128], s_ref[R1:TQ, j * CK + 128:j * CK + 256])
        m1, m7, m6, m6b = f[1](a), f[7](a), f[6](a), f[6](b)
        c0 = a * CK
        c11 = s_ref[0:R1, c0:c0 + 128] + (m1 + m7)
        c22 = s_ref[R1:TQ, c0 + 128:c0 + 256] + (m1[0:R2] + m6)
        s_ref[0:R1, c0:c0 + 128] = c11
        s_ref[R1:TQ, c0 + 128:c0 + 256] = c22
        c0 = b * CK
        s_ref[R1:TQ, c0 + 128:c0 + 256] += m6b
        m11, m71, m12, m72 = f[11](b), f[71](b), f[12](b), f[72](b)
        m1, m7 = _cat0(m11, m12), _cat0(m71, m72)
        c11 = s_ref[0:R1, c0:c0 + 128] + (m1 + m7)
        c22 = s_ref[R1:TQ, c0 + 128:c0 + 256] + m1[0:R2]
        s_ref[0:R1, c0:c0 + 128] = c11
        s_ref[R1:TQ, c0 + 128:c0 + 256] = c22
        ml = jnp.maximum(_cat0(c11, c22), off_diag(b))
        ml = jnp.maximum(ml, jnp.maximum(off_diag(a), diag(a)))
        return max_update(ml, pos == 0, pos >= NC - 2)

    def scores_chunk(t, j, pos):
        q = _upk(q_ref[0:TQ // 2, :])
        if (j + 1) * CK <= T:
            sj = lax.dot_general(q, xa_chunk(t, j), NT_DIMS, preferred_element_type=F32)
            sts = [sj[:, 0:128], sj[:, 128:256]]
        else:
            nrem = T - j * CK - 128
            assert 0 < nrem < 128 and nrem % 16 == 0
            kf = _upk(xa_ref[_ds(t.kb, j * CK // 2, 64, 16), :])
            sj = jnp.concatenate([lax.dot_general(q[0:R1], kf, NT_DIMS, preferred_element_type=F32),
                                  lax.dot_general(q[R1:TQ], kf, NT_DIMS, preferred_element_type=F32)], axis=0)
            kr = _upk(xa_ref[_ds(t.kb, j * CK // 2 + 64, nrem // 2, 16), :])
            st = lax.dot_general(kr, _upk(q_ref[...]), NT_DIMS, preferred_element_type=F32)
            st = jnp.concatenate([st, jnp.full((128 - nrem, st.shape[1]), -jnp.inf, F32)], axis=0)
            sts = [sj, st.T[0:TQ]]
        last[0] = sj[0:16, 0:128]
        s_ref[:, j * CK:j * CK + 128] = sts[0]
        s_ref[:, j * CK + 128:(j + 1) * CK] = sts[1]
        return max_update(jnp.maximum(sts[0], sts[1]), pos == 0, pos == NC - 1)

    def scores_fin(mpart):
        m = jnp.max(mpart, axis=-1, keepdims=True)
        lam = jnp.sum(jnp.exp2(mpart - m), axis=-1, keepdims=True)
        m = m + jnp.log(lam) * LOG2E
        mx_ref[0:TQ] = jnp.broadcast_to(m, (TQ, 128))

    def pv_group(t, js, first, r0=0, r1=R1, r2=R2):
        ra, rb, rc = r0, r0 + r1, r0 + r1 + r2
        L = {k: [] for k in range(1, 8)}
        l1 = l2 = None
        for j in js:
            c0 = j * CK
            a11 = jnp.exp2(s_ref[ra:rb, c0:c0 + 128] - mx_ref[ra:rb])
            a12 = jnp.exp2(s_ref[ra:rb, c0 + 128:c0 + 256] - mx_ref[ra:rb])
            a21 = jnp.exp2(s_ref[rb:rc, c0:c0 + 128] - mx_ref[rb:rc])
            a22 = jnp.exp2(s_ref[rb:rc, c0 + 128:c0 + 256] - mx_ref[rb:rc])
            s1 = a11 + a12
            s2 = a21 + a22
            l1 = s1 if l1 is None else l1 + s1
            l2 = s2 if l2 is None else l2 + s2
            L[1].append(_cat0(a11[0:r2] + a22, a11[r2:]))
            L[2].append(s2)
            L[3].append(a11)
            L[4].append(a22)
            L[5].append(s1)
            L[6].append(a21 - a11[0:r2])
            L[7].append(_cat0(a12[0:r2] - a22, a12[r2:]))
        W = {1: lambda j: kc(t, j, 0), 2: lambda j: k_alo(t, j), 3: lambda j: kc(t, j, 1), 4: lambda j: kc(t, j, 2),
             5: lambda j: k_bhi(t, j), 6: lambda j: kc(t, j, 3), 7: lambda j: kc(t, j, 4)}
        for i, k in enumerate(VSEQ):
            lhs = jnp.concatenate(L[k], axis=1).astype(BF16)
            rhs = _upk(jnp.concatenate([W[k](j) for j in js], axis=0))
            mk = jnp.dot(lhs, rhs, preferred_element_type=F32)
            last[0] = mk[0:16]
            if i == 0:
                first_w[0] = mk[0:16]
            n = mk.shape[0]
            if first:
                acc7_ref[k, 0:n] = mk
            else:
                acc7_ref[k, 0:n] += mk
        lloc = _cat0(l1, l2)
        if first:
            lp_ref[ra:rc] = lloc
        else:
            lp_ref[ra:rc] += lloc

    def pv_fin(t, r0=0, r1=R1, r2=R2):
        l = jnp.sum(lp_ref[r0:r0 + r1 + r2], axis=-1, keepdims=True)
        m1, m3, m5, m7 = (acc7_ref[k, 0:r1] for k in (1, 3, 5, 7))
        m2, m4, m6 = (acc7_ref[k, 0:r2] for k in (2, 4, 6))
        c11 = m1 + (m7 - m5)
        c11 = _cat0(c11[0:r2] + m4, c11[r2:])
        c12 = m3 + m5
        c21 = m2 + m4
        c22 = (m1[0:r2] - m2) + (m3[0:r2] + m6)
        acc = jnp.concatenate([jnp.concatenate([c11, c12], axis=1), jnp.concatenate([c21, c22], axis=1)], axis=0)
        o = acc * (1.0 / l)
        glob = jnp.dot(o.astype(BF16), _upk(wvo_p[...]), preferred_element_type=F32)
        m_store(t, 0, glob, r0)

    def pv_chunk(t, j, r0, n):
        c0 = j * CK
        pa = jnp.exp2(s_ref[r0:r0 + n, c0:c0 + 128] - mx_ref[r0:r0 + n])
        pb = jnp.exp2(s_ref[r0:r0 + n, c0 + 128:c0 + 256] - mx_ref[r0:r0 + n])
        lloc = pa + pb
        pv = jnp.dot(jnp.concatenate([pa, pb], axis=-1).astype(BF16), xa_chunk(t, j), preferred_element_type=F32)
        last[0] = pv[0:16, 0:128]
        if j == 0:
            lp_ref[r0:r0 + n] = lloc
            acc_ref[r0:r0 + n] = pv
        else:
            lp_ref[r0:r0 + n] += lloc
            acc_ref[r0:r0 + n] += pv

    def pv_chunk_fin(t, r0, n):
        l = jnp.sum(lp_ref[r0:r0 + n], axis=-1, keepdims=True)
        o = (acc_ref[r0:r0 + n] * (1.0 / l)).astype(BF16)
        glob = jnp.dot(o, _upk(wvo_p[...]), preferred_element_type=F32)
        m_store(t, 0, glob, r0)

    def anchor(op):
        if op == 'Zx':
            zrow = pl.multiple_of(zoff[0], 16)
            x_buf[pl.ds(zrow + B * T + LAG + TP - T, 16), 0:128] = last[0].astype(BF16)
            return
        zrow = pl.multiple_of(zoff[0], 8)
        if op in ('Z', 'Zg'):
            (m_buf if op == 'Z' else g_buf)[0, pl.ds(zrow + NS * SLOT + 64, 8), :] = last[0][0:8]
        else:
            (lp_ref if op == 'Zl' else mx_ref)[pl.ds(zrow + TQ, 8), :] = last[0][0:8]

    def step(order, pb, pa, t0, tp, th=None, un=None, dma=None):
        cord, nxt = [], 0
        for op in order:
            if op == 'KK':
                cord += [nxt, nxt + 1]
                nxt += 2
            elif op in ('Ks', 'K'):
                cord.append(NC - 2 if op == 'Ks' else NC - 1)
        assert 4 * order.count('W') == NC and sorted(cord) == list(range(NC))
        mpart = None
        jv = jk = 0
        nq = []
        for op in order:
            if op == 'q':
                qproj(tp)
            elif op == 'W':
                pv_group(t0, cord[jv:jv + 4], jv == 0)
                jv += 4
            elif op == 'G':
                pv_fin(t0)
            elif op in ('K', 'Ks'):
                assert jk < jv
                mpart = scores_chunk(tp, cord[jk], jk)
                jk += 1
            elif op == 'KK':
                assert jk + 1 < jv
                mpart = scores_pair(tp, cord[jk], cord[jk + 1], jk)
                jk += 2
            elif op[0] == 'Z':
                anchor(op)
            elif op == 'Ma':
                merge_loc(pa)
            elif op == 'Mb':
                merge_glob(pb)
            elif op == 'H':
                mlp_in(th)
            elif op == 'L':
                mlp_out(tp)
            elif op == 'n':
                r = (len(nq) // 2) * 256 + (len(nq) % 2) * 64
                xa_, xb_ = (_ln(x_buf[_ds(un * 512, LAG + T + r + o, 64, 16), :].astype(F32)) for o in (0, 128))
                v = jnp.concatenate(
                    [xa_, xb_] + _key_combos(xa_[:, 0:128], xa_[:, 128:256], xb_[:, 0:128], xb_[:, 128:256]), axis=1)
                nq.append((r, _pk(v.astype(BF16))))
            elif op == 'Ns':
                assert len(nq) == 4
                for r, v in nq:
                    xa_ref[_ds(un * 256, TP // 2 + r // 2, 32, 256), :] = v[:, 0:256]
                    xa_ref[_ds(un * 256, TP // 2 + r // 2 + 64, 32, 256), :] = v[:, 256:512]
                    kc_ref[_ds(un * 128, TP // 4 + (r // 256) * 64 + (r % 256) // 2, 32, 128), :] = v[:, 512:1152]
            elif op == 'D':
                dma()
            else:
                raise ValueError(op)
        scores_fin(mpart)

    done, nln = [], 0
    for op in PROLOGUE[split + 1:]:
        if op[0] == 's':
            dma_start(op)
        elif op[0] == 'x':
            x_copy(int(op[1:])).wait()
        elif op[0] == 'w':
            w_copy(int(op[1:])).wait()
        elif op[0] == 'n':
            ln_unit(int(op[1:]))
            nln = int(op[1:]) + 1
        elif op[0] == 'p':
            prep(int(op[1:]))
        elif op == 'A':
            prep_a()
        elif op == 'q':
            qproj(tile(0), False)
        elif op.startswith('KK'):
            j = int(op[2:])
            assert nln * 512 >= (j + 2) * CK
            mpart = scores_pair(tile(0), j, j + 1, len(done))
            done += [j, j + 1]
        elif op[0] == 'K':
            j = int(op[1:])
            assert nln * 512 >= (j + 1) * CK
            mpart = scores_chunk(tile(0), j, len(done))
            done.append(j)
        elif op[0] == 'H':
            assert nln * 512 >= (int(op[1:]) + 1) * TQ
            mlp_in(tile(int(op[1:])))
        elif op == 'L0':
            mlp_out(tile(0))
        elif op[0] == 'Z':
            anchor(op)
        else:
            raise ValueError(op)
    assert sorted(done) == list(range(NC))
    scores_fin(mpart)

    def body_a(order, s, c):
        if 'Ns' in order:
            @pl.when(s == 1)
            def _():
                x_copy(NU + 1).wait()

        w = jnp.maximum(s - 1, 0)
        fb = w * TQ

        def dma():
            @pl.when(s > 0)
            def _():
                out_copy(fb, LAG, TQ - LAG).start()

            @pl.when(jnp.logical_and(s > 1, s != NT + 1))
            def _():
                out_copy(fb, 0, LAG).start()

        step(order, [(tile(w), 0, TQ, 0)], [(tile(s), 0, TQ, 0)], tile(s), tile(s + 1), tile(s + 3), s, dma)
        return c
    lax.fori_loop(0, NU, functools.partial(body_a, STEP_A1), 0)
    lax.fori_loop(NU, NS - 3, functools.partial(body_a, STEP_A2), 0)

    z = zoff[0]
    tail0 = (tile(NT - 1), TQ, LAG, TQ + LAG)
    Y2 = TQ + 3 * LAG

    def body_b(s, c):
        step(STEP_B, [(tile(s - 1), 0, TQ, 0)], [(tile(s), 0, TQ, 0), tail0], tile(s), tile(s + 1))
        out_copy((s - 1) * TQ, 0, TQ).start()
        return c
    lax.fori_loop(NS - 3, NS - 1, body_b, 0)

    def last_block(ops):
        tl = tile(z + (NS - 1))
        j = 0
        saved = None
        for op in ops:
            if op == 'WA':
                pv_group(tl, list(range(j, j + 4)), j == 0, 0, RA // 2, RA // 2)
                j += 4
            elif op == 'B':
                pv_chunk(tl, j, RA, TQ - RA)
                j += 1
            elif op == 'Ga':
                pv_fin(tl, 0, RA // 2, RA // 2)
            elif op == 'Gb':
                pv_chunk_fin(tl, RA, TQ - RA)
            elif op == 'E':
                last[0] = first_w[0]
            elif op == 'S':
                saved = last[0]
            elif op == 'R':
                last[0] = saved
            elif op[0] == 'Z':
                anchor(op)
            elif op == 'Mb':
                merge_glob([(tile(z + (NS - 2)), 0, TQ, 0), tail0])
                out_copy(0, (NS - 2) * TQ, TQ).start()
                out_copy(0, NT * TQ, LAG).start()
            elif op == 'Mc':
                merge_loc([(tl, 0, TQ + LAG, Y2)])
            elif op == 'M1':
                merge_glob([(tl, 0, RA, Y2)])
                out_copy(0, (NS - 1) * TQ, RA).start()
            elif op == 'M2':
                merge_glob([(tl, RA, TQ + LAG - RA, Y2 + RA)])
                out_copy(0, (NS - 1) * TQ + RA, TQ + LAG - RA).start()
            else:
                raise ValueError(op)
        assert j == NC

    pl.when(z < 1)(functools.partial(last_block, LAST_A))
    pl.when(z < 2)(functools.partial(last_block, LAST_B))

    out_copy(0, LAG, B * T).wait()


@jax.jit
def pallas_standalone__conformer_family_e_branchformer__speech_kernel(
    x: jax.Array,
    w_qkv: jax.Array,
    w_att_out: jax.Array,
    w_mlp_in: jax.Array,
    dw_csgu: jax.Array,
    w_mlp_out: jax.Array,
    dw_merge: jax.Array,
    w_merge: jax.Array,
):
    B, T, D = x.shape
    K = dw_csgu.shape[0]
    TP = (T + 511) // 512 * 512
    G = D // 128
    RB = (B * (T // TQ) + 1) * SLOT
    out = pl.pallas_call(
        functools.partial(_kernel, B=B, T=T, D=D, K=K, TP=TP),
        in_specs=[pl.BlockSpec(memory_space=pl.ANY)] * 8,
        out_specs=pl.BlockSpec(memory_space=pl.ANY),
        out_shape=jax.ShapeDtypeStruct((B * T, D), x.dtype),
        scratch_shapes=[
            pltpu.VMEM((B * T + 32 + TP - T, D), BF16),
            pltpu.VMEM((B * T + 32, D), BF16),
            pltpu.VMEM((B * TP // 2, D), U32),
            pltpu.VMEM((D // 2, D), U32),
            pltpu.VMEM((D // 2, D), U32),
            pltpu.VMEM((D // 2, 2 * D), U32),
            pltpu.VMEM((D // 2, D), U32),
            pltpu.VMEM((D, D), U32),
            pltpu.VMEM((64, 896), U32),
            pltpu.VMEM((3 * G, 48, 8, 128), F32),
            pltpu.VMEM((2 * G, RB, 128), F32),
            pltpu.VMEM((4 * G, RB, 128), F32),
            pltpu.VMEM((B * T, D), F32),
            pltpu.VMEM((TQ, TP), F32),
            pltpu.VMEM((TQ + 16, 128), F32),
            pltpu.VMEM((256, D), U32),
            pltpu.VMEM((128, 640), U32),
            pltpu.VMEM((B * TP // 4, 640), U32),
            pltpu.VMEM((TQ + 16, 128), F32),
            pltpu.VMEM((TQ + 16, 128), F32),
            pltpu.VMEM((TQ, D), F32),
            pltpu.VMEM((8, 224, 128), F32),
            pltpu.VMEM((2 * TQ + 4 * LAG, D), F32),
            pltpu.VMEM(w_qkv.shape, BF16),
            pltpu.VMEM(w_att_out.shape, BF16),
            pltpu.VMEM(w_mlp_in.shape, BF16),
            pltpu.VMEM(dw_csgu.shape, BF16),
            pltpu.VMEM(w_mlp_out.shape, BF16),
            pltpu.VMEM(dw_merge.shape, BF16),
            pltpu.VMEM(w_merge.shape, BF16),
            pltpu.SMEM((1,), jnp.int32),
            pltpu.SemaphoreType.DMA((max(GRP.values()) + 1,)),
            pltpu.SemaphoreType.DMA,
        ],
        compiler_params=pltpu.CompilerParams(vmem_limit_bytes=120 * 1024 * 1024, disable_bounds_checks=True),
    )(x.reshape(B * T, D), w_qkv, w_att_out, w_mlp_in, dw_csgu, w_mlp_out, dw_merge, w_merge)
    return out.reshape(B, T, D)
```

```python
import functools

import jax
import jax.numpy as jnp
from jax import lax
import jax.experimental.pallas as pl
import jax.experimental.pallas.tpu as pltpu

F32 = jnp.float32
BF16 = jnp.bfloat16
U32 = jnp.uint32
LOG2E = 1.4426950408889634
NT_DIMS = (((1,), (1,)), ((), ()))

TQ = 400
CK = 256
SLOT = 448
LAG = 16
R1 = 208
R2 = TQ - R1
RA = 288
VSEQ = (3, 4, 1, 5, 7, 2, 6)

PROLOGUE = (
    'sx0 sw0 | x0 sx1 sw1 n0 w0 sx2 sx3 A q x1 w1 sx4 sx5 sw3 sw4 p1 H0 n1 KK0 '
    'x2 x3 x4 sx6 sx7 sw2 sw5 sw6 sw7 sx8 n2 n3 KK2 KK4 KK6 H1 H2 n4 K8 '
    'x5 x6 x7 w3 w4 w2 w5 w6 w7 x8 sx9 p3 p4 p5 p6 n5 K9 Zg KK10 n6 KK12 n7 K15 K14 p2 L0').split()
STEP_A1 = 'q Z Zg W W Mb K Ks D W Ma W Zl L H KK KK Zx n KK Zx n KK Zx n KK Zx n KK KK Ns G'.split()
STEP_A2 = 'q Z Zg W W Mb K Ks D W Ma W Zl L H KK KK KK KK KK KK KK G'.split()
STEP_B = 'q Z Zg W W Mb K Ks W Ma W Zl L KK KK KK KK KK KK KK G'.split()
LAST_A = 'WA E Z WA WA Mb WA Zl Mc Ga'.split()
LAST_B = 'B Z S B B R Zm B S B B R Zm B B B B B B B B B B Zl M1 Gb M2'.split()


def _sem_groups():
    grp, g, prev = {}, -1, False
    for op in PROLOGUE:
        is_wait = op[0] in 'xw'
        if is_wait:
            g += 0 if prev else 1
            grp[op] = g
        prev = is_wait
    grp['x9'] = g + 1
    return grp


GRP = _sem_groups()


def _pk(x):
    return pltpu.bitcast(x, U32)


def _upk(x):
    return pltpu.bitcast(x, BF16)


def _cat0(u, v):
    return jnp.concatenate([u, v], axis=0) if v.shape[0] else u


def _ln(x, eps=1e-5):
    m = jnp.mean(x, axis=-1, keepdims=True)
    xc = x - m
    v = jnp.mean(xc * xc, axis=-1, keepdims=True)
    return xc * jnp.exp2(jnp.log(v + eps) * (-0.5 * LOG2E))


def _gelu(x):
    c = 0.7978845608028654
    hx = 0.5 * x
    return hx + hx * jnp.tanh(x * (c + (c * 0.044715) * (x * x)))


def _ds(base, off, n, align):
    if isinstance(base, int):
        return pl.ds(base + off, n)
    a = align
    while off % a:
        a //= 2
    return pl.ds(pl.multiple_of(base + off, a), n) if a > 1 else pl.ds(base + off, n)


def _conv_direct(buf_ref, g, w_ref, wg, base, off, nrows, K):
    V = nrows // 8
    acc = None
    for p in range(8):
        taps = list(range(p, K, 8))
        nq = V + len(taps) - 1
        slab = buf_ref[g, _ds(base, off + p - K // 2, 8 * nq, 32), :].reshape(nq, 8, 128)
        for qi, i in enumerate(taps):
            term = slab[qi:qi + V] * w_ref[wg, i][None]
            acc = term if acc is None else acc + term
    return acc.reshape(8 * V, 128)


def _conv(buf_ref, g, ge, w_ref, wg, base, off, nrows, K):
    nq = nrows // 32
    outs = []
    q0 = 0
    while q0 < nq:
        Q = min(4, nq - q0)
        am = a0 = a1 = None
        for i in [p + 8 * h for p in range(8) for h in range(2)]:
            r = off + 32 * q0 + i - K // 2 + 16
            xs = buf_ref[g, _ds(base, r, 32 * Q - 16, 32), :]
            xs = jnp.concatenate([xs[32 * k:32 * k + 16] for k in range(Q)], axis=0).reshape(2 * Q, 8, 128)
            t = xs * w_ref[wg, 32 + i][None]
            am = t if am is None else am + t
            if i + 16 < K:
                es = buf_ref[ge, _ds(base, r, 32 * Q, 32), :]
                e2 = jnp.concatenate([es[32 * k + 16:32 * k + 32] for k in range(Q)], axis=0).reshape(2 * Q, 8, 128)
                t = e2 * w_ref[wg, i + 16][None]
                a1 = t if a1 is None else a1 + t
            else:
                es = buf_ref[ge, _ds(base, r, 32 * Q - 16, 32), :]
            e1 = jnp.concatenate([es[32 * k:32 * k + 16] for k in range(Q)], axis=0).reshape(2 * Q, 8, 128)
            t = e1 * w_ref[wg, i][None]
            a0 = t if a0 is None else a0 + t
        y0 = (am - a0).reshape(16 * Q, 128)
        y1 = (am + a1).reshape(16 * Q, 128)
        for k in range(Q):
            outs += [y0[16 * k:16 * k + 16], y1[16 * k:16 * k + 16]]
        q0 += Q
    if nrows % 32:
        outs.append(_conv_direct(buf_ref, g, w_ref, wg, base, off + 32 * nq, nrows - 32 * nq, K))
    return jnp.concatenate(outs, axis=0) if len(outs) > 1 else outs[0]


def _key_combos(alo, ahi, blo, bhi):
    return [alo + bhi, ahi - bhi, blo - alo, alo + ahi, blo + bhi]


class _Tile:
    def __init__(self, t, NT, NS, TP, T):
        if isinstance(t, int):
            b = t // NT
            self.prev = (NS if t % NT == 0 else t - 1) * SLOT
            self.next = (NS if t % NT == NT - 1 else t + 1) * SLOT
        else:
            b = (t >= NT).astype(jnp.int32)
            first = jnp.logical_or(t == 0, t == NT)
            last = jnp.logical_or(t == NT - 1, t == NS - 1)
            self.prev = jnp.where(first, NS, t - 1) * SLOT
            self.next = jnp.where(last, NS, t + 1) * SLOT
        self.cb = t * SLOT
        self.fb = t * TQ
        self.ab = t * (TQ // 2) + b * ((TP - T) // 2)
        self.kb = b * (TP // 2)
        self.cbk = b * (TP // 4)


def _kernel(x_hbm, wqkv_hbm, wao_hbm, wmi_hbm, dwc_hbm, wmo_hbm, dwm_hbm, wm_hbm, o_hbm,
            x_buf, o_buf, xa_ref, wa_p, wvo_p, wmi_p, wmo_p, wm_p, ws_ref, dw_f, g_buf, m_buf, u_ref,
            s_ref, mx_ref, q_ref, qc_ref, kc_ref, mp_ref, lp_ref, acc_ref, acc7_ref, y_ref,
            wqkv_ref, wao_ref, wmi_ref, dwc_ref, wmo_ref, dwm_ref, wm_ref,
            zoff, sem_in, sem_out,
            *, B, T, D, K, TP):
    NT = T // TQ
    NS = B * NT
    G = D // 128
    NC = TP // CK
    NU = TP // 512
    assert B == 2 and D == 256 and K == 31 and T % TQ == 0 and NC == 16
    last = [None]
    first_w = [None]

    def tile(t):
        return _Tile(t, NT, NS, TP, T)

    def x_copy(u):
        r0 = u * 512 if u < NU else (T if u == NU else T + 512)
        n = min(512, T - r0) if u < NU else (512 if u == NU else T - 512)
        return pltpu.make_async_copy(x_hbm.at[pl.ds(r0, n), :], x_buf.at[pl.ds(LAG + r0, n), :],
                                     sem_in.at[GRP['x%d' % u]])

    w_pairs = [(wqkv_hbm.at[:, 0:2 * D], wqkv_ref.at[:, 0:2 * D]), (wmi_hbm, wmi_ref), (wao_hbm, wao_ref),
               (dwc_hbm, dwc_ref), (wmo_hbm, wmo_ref), (dwm_hbm, dwm_ref), (wm_hbm, wm_ref),
               (wqkv_hbm.at[:, 2 * D:3 * D], wqkv_ref.at[:, 2 * D:3 * D])]

    def w_copy(k):
        return pltpu.make_async_copy(w_pairs[k][0], w_pairs[k][1], sem_in.at[GRP['w%d' % k]])

    def dma_start(op):
        (x_copy if op[1] == 'x' else w_copy)(int(op[2:])).start()

    def out_copy(base, off, n):
        return pltpu.make_async_copy(o_buf.at[_ds(base, off, n, 16), :], o_hbm.at[_ds(base, off - LAG, n, 16), :],
                                     sem_out)

    split = PROLOGUE.index('|')
    for op in PROLOGUE[:split]:
        dma_start(op)

    zoff[0] = 0
    z16 = jnp.zeros((16, 128), F32)
    for b in range(B):
        lo, hi = b * NT * SLOT, ((b + 1) * NT - 1) * SLOT
        for gi in range(G):
            g_buf[gi, lo:lo + 16, :] = z16
            g_buf[gi, hi + 416:hi + 432, :] = z16
        for gi in range(2 * G):
            m_buf[gi, lo:lo + 16, :] = z16
            m_buf[gi, lo + 16:lo + 32, :] = z16
            m_buf[2 * G + gi, lo + 16:lo + 32, :] = z16
            m_buf[gi, hi + 432:hi + 448, :] = z16
    for gi in range(G):
        m_buf[gi, 32:32 + TQ, :] = jnp.zeros((TQ, 128), F32)
        m_buf[2 * G + gi, 32:32 + TQ, :] = jnp.zeros((TQ, 128), F32)
    y_ref[0:TQ, :] = jnp.zeros((TQ, D), F32)
    x_buf[0:LAG, :] = jnp.zeros((LAG, D), BF16)
    x_buf[LAG + B * T:LAG + B * T + TP - T, :] = jnp.zeros((TP - T, D), BF16)
    q_ref[TQ // 2:, :] = jnp.zeros((q_ref.shape[0] - TQ // 2, D), U32)

    def prep_a():
        a = lax.dot_general(wqkv_ref[:, 0:D], wqkv_ref[:, D:2 * D], NT_DIMS, preferred_element_type=F32)
        a = a * (D ** -0.5 * LOG2E)
        wa_p[...] = _pk(a.astype(BF16))
        b11, b12, b21, b22 = a[0:128, 0:128], a[0:128, 128:256], a[128:256, 0:128], a[128:256, 128:256]
        ws_ref[...] = _pk(jnp.concatenate(
            [b11 + b22, b11, b12 - b22, b21 - b11, b22, b11 + b12, b21 + b22], axis=1).astype(BF16))

    def prep(k):
        if k == 1:
            wmi_p[...] = _pk(wmi_ref[...])
        elif k == 2:
            wvo = jnp.dot(wqkv_ref[:, 2 * D:3 * D], wao_ref[...], preferred_element_type=F32)
            wvo_p[...] = _pk(wvo.astype(BF16))
        elif k == 4:
            wmo_p[...] = _pk(wmo_ref[...])
        elif k == 6:
            wm_p[...] = _pk(wm_ref[...])
        else:
            dw = (dwc_ref if k == 3 else dwm_ref)[...].astype(F32)
            g0 = 2 * G if k == 3 else 0
            if k == 5:
                row = lax.broadcasted_iota(jnp.int32, dw.shape, 0)
                dw = jnp.where(row == K // 2, dw + 1.0, dw)
            for gi in range(dw.shape[1] // 128):
                for i in range(K):
                    dw_f[g0 + gi, i] = jnp.broadcast_to(dw[i:i + 1, gi * 128:(gi + 1) * 128], (8, 128))
                for i in range(16):
                    v = dw_f[g0 + gi, i]
                    dw_f[g0 + gi, 32 + i] = v + dw_f[g0 + gi, i + 16] if i + 16 < K else v

    def ln_unit(u):
        n = min(512, T - u * 512)
        xk = _ln(x_buf[pl.ds(LAG + u * 512, n), :].astype(F32))
        if n < 512:
            xk = jnp.concatenate([xk, jnp.zeros((512 - n, D), F32)], axis=0)
        vs = []
        for r in (0, 256):
            vs.append(jnp.concatenate(_key_combos(xk[r:r + 128, 0:128], xk[r:r + 128, 128:256],
                                                  xk[r + 128:r + 256, 0:128], xk[r + 128:r + 256, 128:256]), axis=1))
        xa_p, kc_p = _pk(xk.astype(BF16)), _pk(jnp.concatenate(vs, axis=0).astype(BF16))
        xa_ref[u * 256:(u + 1) * 256, :] = xa_p
        kc_ref[u * 128:(u + 1) * 128, :] = kc_p

    def xq_of(t):
        return _upk(xa_ref[_ds(t.ab, 0, TQ // 2, 8), :])

    def xa_chunk(t, j):
        return _upk(xa_ref[_ds(t.kb, j * CK // 2, CK // 2, 16), :])

    def kc(t, j, i):
        return kc_ref[_ds(t.cbk, j * 64, 64, 32), i * 128:(i + 1) * 128]

    def k_alo(t, j):
        return xa_ref[_ds(t.kb, j * 128, 64, 16), 0:128]

    def k_bhi(t, j):
        return xa_ref[_ds(t.kb, j * 128 + 64, 64, 16), 128:256]

    def q_strassen(lhs):
        a11, a12, a21, a22 = lhs[0:R1, 0:128], lhs[0:R1, 128:256], lhs[R1:TQ, 0:128], lhs[R1:TQ, 128:256]
        p1 = jnp.concatenate([_cat0(a11[0:R2] + a22, a11[R2:]), a11, a11 + a12, _cat0(a12[0:R2] - a22, a12[R2:])],
                             axis=1).astype(BF16)
        p2 = jnp.concatenate([a21 + a22, a22, a21 - a11[0:R2]], axis=1).astype(BF16)
        lk = {1: p1[:, 0:128], 3: p1[:, 128:256], 5: p1[:, 256:384], 7: p1[:, 384:512],
              2: p2[:, 0:128], 4: p2[:, 128:256], 6: p2[:, 256:384]}

        def job(k, lo=None, hi=None):
            l = lk[k] if lo is None else lk[k][lo:hi]
            return jnp.dot(l, _upk(ws_ref[:, (k - 1) * 128:k * 128]), preferred_element_type=F32)
        s1, s2 = 144, 160
        m3, m5, m2, m4 = job(3), job(5), job(2), job(4)
        m6a = job(6, 0, s2)
        m1b = job(1, s1, R1)
        m1a = job(1, 0, s1)
        m7a = job(7, 0, s1)
        m7b = job(7, s1, R1)
        m6 = _cat0(m6a, job(6, s2, R2))
        m1, m7 = _cat0(m1a, m1b), _cat0(m7a, m7b)
        c12 = m3 + m5
        c21 = m2 + m4
        last[0] = c12[0:16] + c21[0:16]
        c11 = _cat0(m4 - m5[0:R2], -m5[R2:]) + (m1 + m7)
        c22 = ((m3[0:R2] - m2) + m6) + m1[0:R2]
        return jnp.concatenate([jnp.concatenate([c11, c12], axis=1), jnp.concatenate([c21, c22], axis=1)], axis=0)

    def qproj(t, fast=True):
        if fast:
            qf = q_strassen(xq_of(t).astype(F32))
        else:
            qf = jnp.dot(xq_of(t), _upk(wa_p[...]), preferred_element_type=F32)
            last[0] = qf[0:16, 0:128]
        q_ref[0:TQ // 2, :] = _pk(qf.astype(BF16))
        a11, a12 = qf[0:R1, 0:128], qf[0:R1, 128:256]
        a21, a22 = qf[R1:TQ, 0:128], qf[R1:TQ, 128:256]
        qc_ref[0:R1 // 2, 0:384] = _pk(jnp.concatenate(
            [_cat0(a11[0:R2] + a22, a11[R2:]), a12 - a11, _cat0(a12[0:R2] + a22, a12[R2:])], axis=1).astype(BF16))
        qc_ref[0:R2 // 2, 384:640] = _pk(jnp.concatenate([a21 - a22, a11[0:R2] + a21], axis=1).astype(BF16))

    def mlp_in(t):
        hp = jnp.dot(xq_of(t), _upk(wmi_p[...]), preferred_element_type=F32)
        last[0] = hp[0:16, 0:128]
        h = _gelu(hp)
        u_ref[_ds(t.fb, 0, TQ, 16), :] = h[:, :D]
        g = _ln(h[:, D:])
        halo = jnp.concatenate([g_buf[gi, _ds(t.cb, 0, 16, 32), :] for gi in range(G)], axis=1)
        e = jnp.concatenate([g[0:16] - halo, g[16:] - g[:TQ - 16]], axis=0)
        for gi in range(G):
            g_buf[gi, _ds(t.prev, 16 + TQ, 16, 32), :] = g[0:16, gi * 128:(gi + 1) * 128]
        for gi in range(G):
            g_buf[gi, _ds(t.cb, 16, TQ, 32), :] = g[:, gi * 128:(gi + 1) * 128]
            g_buf[G + gi, _ds(t.cb, 16, TQ, 32), :] = e[:, gi * 128:(gi + 1) * 128]
        for gi in range(G):
            g_buf[gi, _ds(t.next, 0, 16, 32), :] = g[TQ - 16:TQ, gi * 128:(gi + 1) * 128]

    def m_store(t, g0, v, r0=0):
        n = v.shape[0]
        halo = jnp.concatenate([m_buf[g0 + gi, _ds(t.cb, 16 + r0, 16, 32), :] for gi in range(G)], axis=1)
        parts = [v[0:16] - halo, v[16:] - v[:n - 16]]
        if r0 + n == TQ:
            parts.append(-v[n - 16:])
        e = jnp.concatenate(parts, axis=0)
        for gi in range(G):
            m_buf[g0 + gi, _ds(t.cb, 32 + r0, n, 32), :] = v[:, gi * 128:(gi + 1) * 128]
            m_buf[2 * G + g0 + gi, _ds(t.cb, 32 + r0, e.shape[0], 32), :] = e[:, gi * 128:(gi + 1) * 128]
        if n == TQ:
            for gi in range(G):
                m_buf[g0 + gi, _ds(t.next, 0, 32, 32), :] = v[TQ - 32:TQ, gi * 128:(gi + 1) * 128]
                m_buf[2 * G + g0 + gi, _ds(t.next, 16, 16, 32), :] = e[TQ - 16:TQ, gi * 128:(gi + 1) * 128]

    def mlp_out(t):
        gc = jnp.concatenate([_conv(g_buf, gi, G + gi, dw_f, 2 * G + gi, t.cb, 16, TQ, K) for gi in range(G)], axis=-1)
        u = u_ref[_ds(t.fb, 0, TQ, 16), :]
        loc = jnp.dot((u * gc).astype(BF16), _upk(wmo_p[...]), preferred_element_type=F32)
        m_store(t, G, loc)

    def merge_half(half, pieces):
        lhs = []
        for (t, off, nrows, _) in pieces:
            ms = [_conv(m_buf, gi, 2 * G + gi, dw_f, gi, t.cb, 32 - LAG + off, nrows, K)
                  for gi in range(half * G, (half + 1) * G)]
            lhs.append(jnp.concatenate(ms, axis=-1))
        lhs = lhs[0] if len(lhs) == 1 else jnp.concatenate(lhs, axis=0)
        return jnp.dot(lhs.astype(BF16), _upk(wm_p[half * D // 2:(half + 1) * D // 2, :]),
                       preferred_element_type=F32)

    def merge_loc(pieces):
        y = merge_half(1, pieces)
        r = 0
        for (t, off, nrows, yo) in pieces:
            y_ref[yo:yo + nrows, :] = x_buf[_ds(t.fb, off, nrows, 16), :].astype(F32) + y[r:r + nrows]
            r += nrows

    def merge_glob(pieces):
        y = merge_half(0, pieces)
        r = 0
        for (t, off, nrows, yo) in pieces:
            o_buf[_ds(t.fb, off, nrows, 16), :] = (y_ref[yo:yo + nrows, :] + y[r:r + nrows]).astype(BF16)
            r += nrows

    def max_update(ml, first, final):
        if final:
            return jnp.maximum(mp_ref[0:TQ], ml)
        mp_ref[0:TQ] = ml if first else jnp.maximum(mp_ref[0:TQ], ml)

    def scores_pair(t, a, b, pos):
        def nt(l, w):
            return lax.dot_general(_upk(l), _upk(w), NT_DIMS, preferred_element_type=F32)
        h1, h2, hs = R1 // 2, R2 // 2, 48
        f = {
            1: lambda j: nt(qc_ref[0:h1, 0:128], kc(t, j, 0)),
            11: lambda j: nt(qc_ref[0:hs, 0:128], kc(t, j, 0)),
            12: lambda j: nt(qc_ref[hs:h1, 0:128], kc(t, j, 0)),
            2: lambda j: nt(q_ref[0:h1, 0:128], kc(t, j, 4)),
            3: lambda j: nt(qc_ref[0:h2, 384:512], k_alo(t, j)),
            4: lambda j: nt(qc_ref[0:h1, 128:256], k_bhi(t, j)),
            5: lambda j: nt(q_ref[h1:TQ // 2, 128:256], kc(t, j, 3)),
            6: lambda j: nt(qc_ref[0:h2, 512:640], kc(t, j, 2)),
            7: lambda j: nt(qc_ref[0:h1, 256:384], kc(t, j, 1)),
            71: lambda j: nt(qc_ref[0:hs, 256:384], kc(t, j, 1)),
            72: lambda j: nt(qc_ref[hs:h1, 256:384], kc(t, j, 1)),
        }
        for j, order in ((a, (2, 4, 3, 5)), (b, (3, 5, 2, 4))):
            m = {k: f[k](j) for k in order}
            c0 = j * CK
            c12 = m[2] + m[4]
            c21 = m[3] + m[5]
            if j == a:
                last[0] = c12[0:16] + c21[0:16]
            s_ref[0:R1, c0 + 128:c0 + 256] = c12
            s_ref[R1:TQ, c0:c0 + 128] = c21
            s_ref[0:R1, c0:c0 + 128] = _cat0(m[4][0:R2] - m[5], m[4][R2:])
            s_ref[R1:TQ, c0 + 128:c0 + 256] = m[3] - m[2][0:R2]

        def off_diag(j):
            return _cat0(s_ref[0:R1, j * CK + 128:j * CK + 256], s_ref[R1:TQ, j * CK:j * CK + 128])

        def diag(j):
            return _cat0(s_ref[0:R1, j * CK:j * CK + 128], s_ref[R1:TQ, j * CK + 128:j * CK + 256])
        m1, m7, m6, m6b = f[1](a), f[7](a), f[6](a), f[6](b)
        c0 = a * CK
        c11 = s_ref[0:R1, c0:c0 + 128] + (m1 + m7)
        c22 = s_ref[R1:TQ, c0 + 128:c0 + 256] + (m1[0:R2] + m6)
        s_ref[0:R1, c0:c0 + 128] = c11
        s_ref[R1:TQ, c0 + 128:c0 + 256] = c22
        c0 = b * CK
        s_ref[R1:TQ, c0 + 128:c0 + 256] += m6b
        m11, m71, m12, m72 = f[11](b), f[71](b), f[12](b), f[72](b)
        m1, m7 = _cat0(m11, m12), _cat0(m71, m72)
        c11 = s_ref[0:R1, c0:c0 + 128] + (m1 + m7)
        c22 = s_ref[R1:TQ, c0 + 128:c0 + 256] + m1[0:R2]
        s_ref[0:R1, c0:c0 + 128] = c11
        s_ref[R1:TQ, c0 + 128:c0 + 256] = c22
        ml = jnp.maximum(_cat0(c11, c22), off_diag(b))
        ml = jnp.maximum(ml, jnp.maximum(off_diag(a), diag(a)))
        return max_update(ml, pos == 0, pos >= NC - 2)

    def scores_chunk(t, j, pos):
        q = _upk(q_ref[0:TQ // 2, :])
        if (j + 1) * CK <= T:
            sj = lax.dot_general(q, xa_chunk(t, j), NT_DIMS, preferred_element_type=F32)
            sts = [sj[:, 0:128], sj[:, 128:256]]
        else:
            nrem = T - j * CK - 128
            assert 0 < nrem < 128 and nrem % 16 == 0
            kf = _upk(xa_ref[_ds(t.kb, j * CK // 2, 64, 16), :])
            sj = jnp.concatenate([lax.dot_general(q[0:R1], kf, NT_DIMS, preferred_element_type=F32),
                                  lax.dot_general(q[R1:TQ], kf, NT_DIMS, preferred_element_type=F32)], axis=0)
            kr = _upk(xa_ref[_ds(t.kb, j * CK // 2 + 64, nrem // 2, 16), :])
            st = lax.dot_general(kr, _upk(q_ref[...]), NT_DIMS, preferred_element_type=F32)
            st = jnp.concatenate([st, jnp.full((128 - nrem, st.shape[1]), -jnp.inf, F32)], axis=0)
            sts = [sj, st.T[0:TQ]]
        last[0] = sj[0:16, 0:128]
        s_ref[:, j * CK:j * CK + 128] = sts[0]
        s_ref[:, j * CK + 128:(j + 1) * CK] = sts[1]
        return max_update(jnp.maximum(sts[0], sts[1]), pos == 0, pos == NC - 1)

    def scores_fin(mpart):
        m = jnp.max(mpart, axis=-1, keepdims=True)
        lam = jnp.sum(jnp.exp2(mpart - m), axis=-1, keepdims=True)
        m = m + jnp.log(lam) * LOG2E
        mx_ref[0:TQ] = jnp.broadcast_to(m, (TQ, 128))

    def pv_group(t, js, first, r0=0, r1=R1, r2=R2):
        ra, rb, rc = r0, r0 + r1, r0 + r1 + r2
        L = {k: [] for k in range(1, 8)}
        l1 = l2 = None
        for j in js:
            c0 = j * CK
            a11 = jnp.exp2(s_ref[ra:rb, c0:c0 + 128] - mx_ref[ra:rb])
            a12 = jnp.exp2(s_ref[ra:rb, c0 + 128:c0 + 256] - mx_ref[ra:rb])
            a21 = jnp.exp2(s_ref[rb:rc, c0:c0 + 128] - mx_ref[rb:rc])
            a22 = jnp.exp2(s_ref[rb:rc, c0 + 128:c0 + 256] - mx_ref[rb:rc])
            s1 = a11 + a12
            s2 = a21 + a22
            l1 = s1 if l1 is None else l1 + s1
            l2 = s2 if l2 is None else l2 + s2
            L[1].append(_cat0(a11[0:r2] + a22, a11[r2:]))
            L[2].append(s2)
            L[3].append(a11)
            L[4].append(a22)
            L[5].append(s1)
            L[6].append(a21 - a11[0:r2])
            L[7].append(_cat0(a12[0:r2] - a22, a12[r2:]))
        W = {1: lambda j: kc(t, j, 0), 2: lambda j: k_alo(t, j), 3: lambda j: kc(t, j, 1), 4: lambda j: kc(t, j, 2),
             5: lambda j: k_bhi(t, j), 6: lambda j: kc(t, j, 3), 7: lambda j: kc(t, j, 4)}
        for i, k in enumerate(VSEQ):
            lhs = jnp.concatenate(L[k], axis=1).astype(BF16)
            rhs = _upk(jnp.concatenate([W[k](j) for j in js], axis=0))
            mk = jnp.dot(lhs, rhs, preferred_element_type=F32)
            last[0] = mk[0:16]
            if i == 0:
                first_w[0] = mk[0:16]
            n = mk.shape[0]
            if first:
                acc7_ref[k, 0:n] = mk
            else:
                acc7_ref[k, 0:n] += mk
        lloc = _cat0(l1, l2)
        if first:
            lp_ref[ra:rc] = lloc
        else:
            lp_ref[ra:rc] += lloc

    def pv_fin(t, r0=0, r1=R1, r2=R2):
        l = jnp.sum(lp_ref[r0:r0 + r1 + r2], axis=-1, keepdims=True)
        m1, m3, m5, m7 = (acc7_ref[k, 0:r1] for k in (1, 3, 5, 7))
        m2, m4, m6 = (acc7_ref[k, 0:r2] for k in (2, 4, 6))
        c11 = m1 + (m7 - m5)
        c11 = _cat0(c11[0:r2] + m4, c11[r2:])
        c12 = m3 + m5
        c21 = m2 + m4
        c22 = (m1[0:r2] - m2) + (m3[0:r2] + m6)
        acc = jnp.concatenate([jnp.concatenate([c11, c12], axis=1), jnp.concatenate([c21, c22], axis=1)], axis=0)
        o = acc * (1.0 / l)
        glob = jnp.dot(o.astype(BF16), _upk(wvo_p[...]), preferred_element_type=F32)
        m_store(t, 0, glob, r0)

    def pv_chunk(t, j, r0, n):
        c0 = j * CK
        pa = jnp.exp2(s_ref[r0:r0 + n, c0:c0 + 128] - mx_ref[r0:r0 + n])
        pb = jnp.exp2(s_ref[r0:r0 + n, c0 + 128:c0 + 256] - mx_ref[r0:r0 + n])
        lloc = pa + pb
        pv = jnp.dot(jnp.concatenate([pa, pb], axis=-1).astype(BF16), xa_chunk(t, j), preferred_element_type=F32)
        last[0] = pv[0:16, 0:128]
        if j == 0:
            lp_ref[r0:r0 + n] = lloc
            acc_ref[r0:r0 + n] = pv
        else:
            lp_ref[r0:r0 + n] += lloc
            acc_ref[r0:r0 + n] += pv

    def pv_chunk_fin(t, r0, n):
        l = jnp.sum(lp_ref[r0:r0 + n], axis=-1, keepdims=True)
        o = (acc_ref[r0:r0 + n] * (1.0 / l)).astype(BF16)
        glob = jnp.dot(o, _upk(wvo_p[...]), preferred_element_type=F32)
        m_store(t, 0, glob, r0)

    def anchor(op):
        if op == 'Zx':
            zrow = pl.multiple_of(zoff[0], 16)
            x_buf[pl.ds(zrow + B * T + LAG + TP - T, 16), 0:128] = last[0].astype(BF16)
            return
        zrow = pl.multiple_of(zoff[0], 8)
        if op in ('Z', 'Zg'):
            (m_buf if op == 'Z' else g_buf)[0, pl.ds(zrow + NS * SLOT + 64, 8), :] = last[0][0:8]
        else:
            (lp_ref if op == 'Zl' else mx_ref)[pl.ds(zrow + TQ, 8), :] = last[0][0:8]

    def step(order, pb, pa, t0, tp, th=None, un=None, dma=None):
        cord, nxt = [], 0
        for op in order:
            if op == 'KK':
                cord += [nxt, nxt + 1]
                nxt += 2
            elif op in ('Ks', 'K'):
                cord.append(NC - 2 if op == 'Ks' else NC - 1)
        assert 4 * order.count('W') == NC and sorted(cord) == list(range(NC))
        mpart = None
        jv = jk = 0
        nq = []
        for op in order:
            if op == 'q':
                qproj(tp)
            elif op == 'W':
                pv_group(t0, cord[jv:jv + 4], jv == 0)
                jv += 4
            elif op == 'G':
                pv_fin(t0)
            elif op in ('K', 'Ks'):
                assert jk < jv
                mpart = scores_chunk(tp, cord[jk], jk)
                jk += 1
            elif op == 'KK':
                assert jk + 1 < jv
                mpart = scores_pair(tp, cord[jk], cord[jk + 1], jk)
                jk += 2
            elif op[0] == 'Z':
                anchor(op)
            elif op == 'Ma':
                merge_loc(pa)
            elif op == 'Mb':
                merge_glob(pb)
            elif op == 'H':
                mlp_in(th)
            elif op == 'L':
                mlp_out(tp)
            elif op == 'n':
                r = (len(nq) // 2) * 256 + (len(nq) % 2) * 64
                xa_, xb_ = (_ln(x_buf[_ds(un * 512, LAG + T + r + o, 64, 16), :].astype(F32)) for o in (0, 128))
                v = jnp.concatenate(
                    [xa_, xb_] + _key_combos(xa_[:, 0:128], xa_[:, 128:256], xb_[:, 0:128], xb_[:, 128:256]), axis=1)
                nq.append((r, _pk(v.astype(BF16))))
            elif op == 'Ns':
                assert len(nq) == 4
                for r, v in nq:
                    xa_ref[_ds(un * 256, TP // 2 + r // 2, 32, 256), :] = v[:, 0:256]
                    xa_ref[_ds(un * 256, TP // 2 + r // 2 + 64, 32, 256), :] = v[:, 256:512]
                    kc_ref[_ds(un * 128, TP // 4 + (r // 256) * 64 + (r % 256) // 2, 32, 128), :] = v[:, 512:1152]
            elif op == 'D':
                dma()
            else:
                raise ValueError(op)
        scores_fin(mpart)

    done, nln = [], 0
    for op in PROLOGUE[split + 1:]:
        if op[0] == 's':
            dma_start(op)
        elif op[0] == 'x':
            x_copy(int(op[1:])).wait()
        elif op[0] == 'w':
            w_copy(int(op[1:])).wait()
        elif op[0] == 'n':
            ln_unit(int(op[1:]))
            nln = int(op[1:]) + 1
        elif op[0] == 'p':
            prep(int(op[1:]))
        elif op == 'A':
            prep_a()
        elif op == 'q':
            qproj(tile(0), False)
        elif op.startswith('KK'):
            j = int(op[2:])
            assert nln * 512 >= (j + 2) * CK
            mpart = scores_pair(tile(0), j, j + 1, len(done))
            done += [j, j + 1]
        elif op[0] == 'K':
            j = int(op[1:])
            assert nln * 512 >= (j + 1) * CK
            mpart = scores_chunk(tile(0), j, len(done))
            done.append(j)
        elif op[0] == 'H':
            assert nln * 512 >= (int(op[1:]) + 1) * TQ
            mlp_in(tile(int(op[1:])))
        elif op == 'L0':
            mlp_out(tile(0))
        elif op[0] == 'Z':
            anchor(op)
        else:
            raise ValueError(op)
    assert sorted(done) == list(range(NC))
    scores_fin(mpart)

    def body_a(order, s, c):
        if 'Ns' in order:
            @pl.when(s == 1)
            def _():
                x_copy(NU + 1).wait()

        w = jnp.maximum(s - 1, 0)
        fb = w * TQ

        def dma():
            @pl.when(s > 0)
            def _():
                out_copy(fb, LAG, TQ - LAG).start()

            @pl.when(jnp.logical_and(s > 1, s != NT + 1))
            def _():
                out_copy(fb, 0, LAG).start()

        step(order, [(tile(w), 0, TQ, 0)], [(tile(s), 0, TQ, 0)], tile(s), tile(s + 1), tile(s + 3), s, dma)
        return c
    lax.fori_loop(0, NU, functools.partial(body_a, STEP_A1), 0)
    lax.fori_loop(NU, NS - 3, functools.partial(body_a, STEP_A2), 0)

    z = zoff[0]
    tail0 = (tile(NT - 1), TQ, LAG, TQ + LAG)
    Y2 = TQ + 3 * LAG

    def body_b(s, c):
        step(STEP_B, [(tile(s - 1), 0, TQ, 0)], [(tile(s), 0, TQ, 0), tail0], tile(s), tile(s + 1))
        out_copy((s - 1) * TQ, 0, TQ).start()
        return c
    lax.fori_loop(NS - 3, NS - 1, body_b, 0)

    def last_block(ops):
        tl = tile(z + (NS - 1))
        j = 0
        saved = None
        for op in ops:
            if op == 'WA':
                pv_group(tl, list(range(j, j + 4)), j == 0, 0, RA // 2, RA // 2)
                j += 4
            elif op == 'B':
                pv_chunk(tl, j, RA, TQ - RA)
                j += 1
            elif op == 'Ga':
                pv_fin(tl, 0, RA // 2, RA // 2)
            elif op == 'Gb':
                pv_chunk_fin(tl, RA, TQ - RA)
            elif op == 'E':
                last[0] = first_w[0]
            elif op == 'S':
                saved = last[0]
            elif op == 'R':
                last[0] = saved
            elif op[0] == 'Z':
                anchor(op)
            elif op == 'Mb':
                merge_glob([(tile(z + (NS - 2)), 0, TQ, 0), tail0])
                out_copy(0, (NS - 2) * TQ, TQ).start()
                out_copy(0, NT * TQ, LAG).start()
            elif op == 'Mc':
                merge_loc([(tl, 0, TQ + LAG, Y2)])
            elif op == 'M1':
                merge_glob([(tl, 0, RA, Y2)])
                out_copy(0, (NS - 1) * TQ, RA).start()
            elif op == 'M2':
                merge_glob([(tl, RA, TQ + LAG - RA, Y2 + RA)])
                out_copy(0, (NS - 1) * TQ + RA, TQ + LAG - RA).start()
            else:
                raise ValueError(op)
        assert j == NC

    pl.when(z < 1)(functools.partial(last_block, LAST_A))
    pl.when(z < 2)(functools.partial(last_block, LAST_B))

    out_copy(0, LAG, B * T).wait()


@jax.jit
def pallas_standalone__conformer_family_e_branchformer__speech_kernel(
    x: jax.Array,
    w_qkv: jax.Array,
    w_att_out: jax.Array,
    w_mlp_in: jax.Array,
    dw_csgu: jax.Array,
    w_mlp_out: jax.Array,
    dw_merge: jax.Array,
    w_merge: jax.Array,
):
    B, T, D = x.shape
    K = dw_csgu.shape[0]
    TP = (T + 511) // 512 * 512
    G = D // 128
    RB = (B * (T // TQ) + 1) * SLOT
    out = pl.pallas_call(
        functools.partial(_kernel, B=B, T=T, D=D, K=K, TP=TP),
        in_specs=[pl.BlockSpec(memory_space=pl.ANY)] * 8,
        out_specs=pl.BlockSpec(memory_space=pl.ANY),
        out_shape=jax.ShapeDtypeStruct((B * T, D), x.dtype),
        scratch_shapes=[
            pltpu.VMEM((B * T + 32 + TP - T, D), BF16),
            pltpu.VMEM((B * T + 32, D), BF16),
            pltpu.VMEM((B * TP // 2, D), U32),
            pltpu.VMEM((D // 2, D), U32),
            pltpu.VMEM((D // 2, D), U32),
            pltpu.VMEM((D // 2, 2 * D), U32),
            pltpu.VMEM((D // 2, D), U32),
            pltpu.VMEM((D, D), U32),
            pltpu.VMEM((64, 896), U32),
            pltpu.VMEM((3 * G, 48, 8, 128), F32),
            pltpu.VMEM((2 * G, RB, 128), F32),
            pltpu.VMEM((4 * G, RB, 128), F32),
            pltpu.VMEM((B * T, D), F32),
            pltpu.VMEM((TQ, TP), F32),
            pltpu.VMEM((TQ + 16, 128), F32),
            pltpu.VMEM((256, D), U32),
            pltpu.VMEM((128, 640), U32),
            pltpu.VMEM((B * TP // 4, 640), U32),
            pltpu.VMEM((TQ + 16, 128), F32),
            pltpu.VMEM((TQ + 16, 128), F32),
            pltpu.VMEM((TQ, D), F32),
            pltpu.VMEM((8, 224, 128), F32),
            pltpu.VMEM((2 * TQ + 4 * LAG, D), F32),
            pltpu.VMEM(w_qkv.shape, BF16),
            pltpu.VMEM(w_att_out.shape, BF16),
            pltpu.VMEM(w_mlp_in.shape, BF16),
            pltpu.VMEM(dw_csgu.shape, BF16),
            pltpu.VMEM(w_mlp_out.shape, BF16),
            pltpu.VMEM(dw_merge.shape, BF16),
            pltpu.VMEM(w_merge.shape, BF16),
            pltpu.SMEM((1,), jnp.int32),
            pltpu.SemaphoreType.DMA((max(GRP.values()) + 1,)),
            pltpu.SemaphoreType.DMA,
        ],
        compiler_params=pltpu.CompilerParams(vmem_limit_bytes=120 * 1024 * 1024, disable_bounds_checks=True),
    )(x.reshape(B * T, D), w_qkv, w_att_out, w_mlp_in, dw_csgu, w_mlp_out, dw_merge, w_merge)
    return out.reshape(B, T, D)
```

```python
import functools

import jax
import jax.numpy as jnp
from jax import lax
import jax.experimental.pallas as pl
import jax.experimental.pallas.tpu as pltpu

F32 = jnp.float32
BF16 = jnp.bfloat16
U32 = jnp.uint32
LOG2E = 1.4426950408889634
NT_DIMS = (((1,), (1,)), ((), ()))

TQ = 400
CK = 256
SLOT = 448
LAG = 16
R1 = 208
R2 = TQ - R1
RA = 288
VSEQ = (3, 4, 1, 5, 7, 2, 6)

PROLOGUE = (
    'sx0 sw0 | x0 sx1 sw1 n0 w0 sx2 sx3 A q x1 w1 sx4 sx5 sw3 sw4 p1 H0 n1 KK0 '
    'x2 x3 x4 sx6 sx7 sw2 sw5 sw6 sw7 sx8 n2 n3 KK2 KK4 KK6 H1 H2 n4 K8 '
    'x5 x6 x7 w3 w4 w2 w5 w6 w7 x8 sx9 p3 p4 p5 p6 n5 K9 Zg KK10 n6 KK12 n7 K15 K14 p2 L0').split()
STEP_A1 = 'q Z Zg W W Mb K Ks D W Ma W Zl L H KK KK Zx n KK Zx n KK Zx n KK Zx n KK KK Ns G'.split()
STEP_A2 = 'q Z Zg W W Mb K Ks D W Ma W Zl L H KK KK KK KK KK KK KK G'.split()
STEP_B = 'q Z Zg W W Mb K Ks W Ma W Zl L KK KK KK KK KK KK KK G'.split()
LAST_A = 'WA E Z WA WA Mb WA Zl Mc Ga'.split()
LAST_B = 'B Z S B B R Zm B S B B R Zm B B B B B B B B B B Zl M1 Gb M2'.split()


def _sem_groups():
    grp, g, prev = {}, -1, False
    for op in PROLOGUE:
        is_wait = op[0] in 'xw'
        if is_wait:
            g += 0 if prev else 1
            grp[op] = g
        prev = is_wait
    grp['x9'] = g + 1
    return grp


GRP = _sem_groups()


def _pk(x):
    return pltpu.bitcast(x, U32)


def _upk(x):
    return pltpu.bitcast(x, BF16)


def _cat0(u, v):
    return jnp.concatenate([u, v], axis=0) if v.shape[0] else u


def _ln(x, eps=1e-5):
    m = jnp.mean(x, axis=-1, keepdims=True)
    xc = x - m
    v = jnp.mean(xc * xc, axis=-1, keepdims=True)
    return xc * jnp.exp2(jnp.log(v + eps) * (-0.5 * LOG2E))


def _gelu(x):
    c = 0.7978845608028654
    hx = 0.5 * x
    return hx + hx * jnp.tanh(x * (c + (c * 0.044715) * (x * x)))


def _ds(base, off, n, align):
    if isinstance(base, int):
        return pl.ds(base + off, n)
    a = align
    while off % a:
        a //= 2
    return pl.ds(pl.multiple_of(base + off, a), n) if a > 1 else pl.ds(base + off, n)


def _conv_direct(buf_ref, g, w_ref, wg, base, off, nrows, K):
    V = nrows // 8
    acc = None
    for p in range(8):
        taps = list(range(p, K, 8))
        nq = V + len(taps) - 1
        slab = buf_ref[g, _ds(base, off + p - K // 2, 8 * nq, 32), :].reshape(nq, 8, 128)
        for qi, i in enumerate(taps):
            term = slab[qi:qi + V] * w_ref[wg, i][None]
            acc = term if acc is None else acc + term
    return acc.reshape(8 * V, 128)


def _conv(buf_ref, g, ge, w_ref, wg, base, off, nrows, K):
    nq = nrows // 32
    outs = []
    q0 = 0
    while q0 < nq:
        Q = min(4, nq - q0)
        am = a0 = a1 = None
        for i in [p + 8 * h for p in range(8) for h in range(2)]:
            r = off + 32 * q0 + i - K // 2 + 16
            xs = buf_ref[g, _ds(base, r, 32 * Q - 16, 32), :]
            xs = jnp.concatenate([xs[32 * k:32 * k + 16] for k in range(Q)], axis=0).reshape(2 * Q, 8, 128)
            t = xs * w_ref[wg, 32 + i][None]
            am = t if am is None else am + t
            if i + 16 < K:
                es = buf_ref[ge, _ds(base, r, 32 * Q, 32), :]
                e2 = jnp.concatenate([es[32 * k + 16:32 * k + 32] for k in range(Q)], axis=0).reshape(2 * Q, 8, 128)
                t = e2 * w_ref[wg, i + 16][None]
                a1 = t if a1 is None else a1 + t
            else:
                es = buf_ref[ge, _ds(base, r, 32 * Q - 16, 32), :]
            e1 = jnp.concatenate([es[32 * k:32 * k + 16] for k in range(Q)], axis=0).reshape(2 * Q, 8, 128)
            t = e1 * w_ref[wg, i][None]
            a0 = t if a0 is None else a0 + t
        y0 = (am - a0).reshape(16 * Q, 128)
        y1 = (am + a1).reshape(16 * Q, 128)
        for k in range(Q):
            outs += [y0[16 * k:16 * k + 16], y1[16 * k:16 * k + 16]]
        q0 += Q
    if nrows % 32:
        outs.append(_conv_direct(buf_ref, g, w_ref, wg, base, off + 32 * nq, nrows - 32 * nq, K))
    return jnp.concatenate(outs, axis=0) if len(outs) > 1 else outs[0]


def _key_combos(alo, ahi, blo, bhi):
    return [alo + bhi, ahi - bhi, blo - alo, alo + ahi, blo + bhi]


class _Tile:
    def __init__(self, t, NT, NS, TP, T):
        if isinstance(t, int):
            b = t // NT
            self.prev = (NS if t % NT == 0 else t - 1) * SLOT
            self.next = (NS if t % NT == NT - 1 else t + 1) * SLOT
        else:
            b = (t >= NT).astype(jnp.int32)
            first = jnp.logical_or(t == 0, t == NT)
            last = jnp.logical_or(t == NT - 1, t == NS - 1)
            self.prev = jnp.where(first, NS, t - 1) * SLOT
            self.next = jnp.where(last, NS, t + 1) * SLOT
        self.cb = t * SLOT
        self.fb = t * TQ
        self.ab = t * (TQ // 2) + b * ((TP - T) // 2)
        self.kb = b * (TP // 2)
        self.cbk = b * (TP // 4)


def _kernel(x_hbm, wqkv_hbm, wao_hbm, wmi_hbm, dwc_hbm, wmo_hbm, dwm_hbm, wm_hbm, o_hbm,
            x_buf, o_buf, xa_ref, wa_p, wvo_p, wmi_p, wmo_p, wm_p, ws_ref, dw_f, g_buf, m_buf, u_ref,
            s_ref, mx_ref, q_ref, qc_ref, kc_ref, mp_ref, lp_ref, acc_ref, acc7_ref, y_ref,
            wqkv_ref, wao_ref, wmi_ref, dwc_ref, wmo_ref, dwm_ref, wm_ref,
            zoff, sem_in, sem_out,
            *, B, T, D, K, TP):
    NT = T // TQ
    NS = B * NT
    G = D // 128
    NC = TP // CK
    NU = TP // 512
    assert B == 2 and D == 256 and K == 31 and T % TQ == 0 and NC == 16
    last = [None]
    first_w = [None]

    def tile(t):
        return _Tile(t, NT, NS, TP, T)

    def x_copy(u):
        r0 = u * 512 if u < NU else (T if u == NU else T + 512)
        n = min(512, T - r0) if u < NU else (512 if u == NU else T - 512)
        return pltpu.make_async_copy(x_hbm.at[pl.ds(r0, n), :], x_buf.at[pl.ds(LAG + r0, n), :],
                                     sem_in.at[GRP['x%d' % u]])

    w_pairs = [(wqkv_hbm.at[:, 0:2 * D], wqkv_ref.at[:, 0:2 * D]), (wmi_hbm, wmi_ref), (wao_hbm, wao_ref),
               (dwc_hbm, dwc_ref), (wmo_hbm, wmo_ref), (dwm_hbm, dwm_ref), (wm_hbm, wm_ref),
               (wqkv_hbm.at[:, 2 * D:3 * D], wqkv_ref.at[:, 2 * D:3 * D])]

    def w_copy(k):
        return pltpu.make_async_copy(w_pairs[k][0], w_pairs[k][1], sem_in.at[GRP['w%d' % k]])

    def dma_start(op):
        (x_copy if op[1] == 'x' else w_copy)(int(op[2:])).start()

    def out_copy(base, off, n):
        return pltpu.make_async_copy(o_buf.at[_ds(base, off, n, 16), :], o_hbm.at[_ds(base, off - LAG, n, 16), :],
                                     sem_out)

    split = PROLOGUE.index('|')
    for op in PROLOGUE[:split]:
        dma_start(op)

    zoff[0] = 0
    z16 = jnp.zeros((16, 128), F32)
    for b in range(B):
        lo, hi = b * NT * SLOT, ((b + 1) * NT - 1) * SLOT
        for gi in range(G):
            g_buf[gi, lo:lo + 16, :] = z16
            g_buf[gi, hi + 416:hi + 432, :] = z16
        for gi in range(2 * G):
            m_buf[gi, lo:lo + 16, :] = z16
            m_buf[gi, lo + 16:lo + 32, :] = z16
            m_buf[2 * G + gi, lo + 16:lo + 32, :] = z16
            m_buf[gi, hi + 432:hi + 448, :] = z16
    for gi in range(G):
        m_buf[gi, 32:32 + TQ, :] = jnp.zeros((TQ, 128), F32)
        m_buf[2 * G + gi, 32:32 + TQ, :] = jnp.zeros((TQ, 128), F32)
    y_ref[0:TQ, :] = jnp.zeros((TQ, D), F32)
    x_buf[0:LAG, :] = jnp.zeros((LAG, D), BF16)
    x_buf[LAG + B * T:LAG + B * T + TP - T, :] = jnp.zeros((TP - T, D), BF16)
    q_ref[TQ // 2:, :] = jnp.zeros((q_ref.shape[0] - TQ // 2, D), U32)

    def prep_a():
        a = lax.dot_general(wqkv_ref[:, 0:D], wqkv_ref[:, D:2 * D], NT_DIMS, preferred_element_type=F32)
        a = a * (D ** -0.5 * LOG2E)
        wa_p[...] = _pk(a.astype(BF16))
        b11, b12, b21, b22 = a[0:128, 0:128], a[0:128, 128:256], a[128:256, 0:128], a[128:256, 128:256]
        ws_ref[...] = _pk(jnp.concatenate(
            [b11 + b22, b11, b12 - b22, b21 - b11, b22, b11 + b12, b21 + b22], axis=1).astype(BF16))

    def prep(k):
        if k == 1:
            wmi_p[...] = _pk(wmi_ref[...])
        elif k == 2:
            wvo = jnp.dot(wqkv_ref[:, 2 * D:3 * D], wao_ref[...], preferred_element_type=F32)
            wvo_p[...] = _pk(wvo.astype(BF16))
        elif k == 4:
            wmo_p[...] = _pk(wmo_ref[...])
        elif k == 6:
            wm_p[...] = _pk(wm_ref[...])
        else:
            dw = (dwc_ref if k == 3 else dwm_ref)[...].astype(F32)
            g0 = 2 * G if k == 3 else 0
            if k == 5:
                row = lax.broadcasted_iota(jnp.int32, dw.shape, 0)
                dw = jnp.where(row == K // 2, dw + 1.0, dw)
            for gi in range(dw.shape[1] // 128):
                for i in range(K):
                    dw_f[g0 + gi, i] = jnp.broadcast_to(dw[i:i + 1, gi * 128:(gi + 1) * 128], (8, 128))
                for i in range(16):
                    v = dw_f[g0 + gi, i]
                    dw_f[g0 + gi, 32 + i] = v + dw_f[g0 + gi, i + 16] if i + 16 < K else v

    def ln_unit(u):
        n = min(512, T - u * 512)
        xk = _ln(x_buf[pl.ds(LAG + u * 512, n), :].astype(F32))
        if n < 512:
            xk = jnp.concatenate([xk, jnp.zeros((512 - n, D), F32)], axis=0)
        vs = []
        for r in (0, 256):
            vs.append(jnp.concatenate(_key_combos(xk[r:r + 128, 0:128], xk[r:r + 128, 128:256],
                                                  xk[r + 128:r + 256, 0:128], xk[r + 128:r + 256, 128:256]), axis=1))
        xa_p, kc_p = _pk(xk.astype(BF16)), _pk(jnp.concatenate(vs, axis=0).astype(BF16))
        xa_ref[u * 256:(u + 1) * 256, :] = xa_p
        kc_ref[u * 128:(u + 1) * 128, :] = kc_p

    def xq_of(t):
        return _upk(xa_ref[_ds(t.ab, 0, TQ // 2, 8), :])

    def xa_chunk(t, j):
        return _upk(xa_ref[_ds(t.kb, j * CK // 2, CK // 2, 16), :])

    def kc(t, j, i):
        return kc_ref[_ds(t.cbk, j * 64, 64, 32), i * 128:(i + 1) * 128]

    def k_alo(t, j):
        return xa_ref[_ds(t.kb, j * 128, 64, 16), 0:128]

    def k_bhi(t, j):
        return xa_ref[_ds(t.kb, j * 128 + 64, 64, 16), 128:256]

    def q_strassen(lhs):
        a11, a12, a21, a22 = lhs[0:R1, 0:128], lhs[0:R1, 128:256], lhs[R1:TQ, 0:128], lhs[R1:TQ, 128:256]
        p1 = jnp.concatenate([_cat0(a11[0:R2] + a22, a11[R2:]), a11, a11 + a12, _cat0(a12[0:R2] - a22, a12[R2:])],
                             axis=1).astype(BF16)
        p2 = jnp.concatenate([a21 + a22, a22, a21 - a11[0:R2]], axis=1).astype(BF16)
        lk = {1: p1[:, 0:128], 3: p1[:, 128:256], 5: p1[:, 256:384], 7: p1[:, 384:512],
              2: p2[:, 0:128], 4: p2[:, 128:256], 6: p2[:, 256:384]}

        def job(k, lo=None, hi=None):
            l = lk[k] if lo is None else lk[k][lo:hi]
            return jnp.dot(l, _upk(ws_ref[:, (k - 1) * 128:k * 128]), preferred_element_type=F32)
        s1, s2 = 144, 160
        m3, m5, m2, m4 = job(3), job(5), job(2), job(4)
        m6a = job(6, 0, s2)
        m1b = job(1, s1, R1)
        m1a = job(1, 0, s1)
        m7a = job(7, 0, s1)
        m7b = job(7, s1, R1)
        m6 = _cat0(m6a, job(6, s2, R2))
        m1, m7 = _cat0(m1a, m1b), _cat0(m7a, m7b)
        c12 = m3 + m5
        c21 = m2 + m4
        last[0] = c12[0:16] + c21[0:16]
        c11 = _cat0(m4 - m5[0:R2], -m5[R2:]) + (m1 + m7)
        c22 = ((m3[0:R2] - m2) + m6) + m1[0:R2]
        return jnp.concatenate([jnp.concatenate([c11, c12], axis=1), jnp.concatenate([c21, c22], axis=1)], axis=0)

    def qproj(t, fast=True):
        if fast:
            qf = q_strassen(xq_of(t).astype(F32))
        else:
            qf = jnp.dot(xq_of(t), _upk(wa_p[...]), preferred_element_type=F32)
            last[0] = qf[0:16, 0:128]
        q_ref[0:TQ // 2, :] = _pk(qf.astype(BF16))
        a11, a12 = qf[0:R1, 0:128], qf[0:R1, 128:256]
        a21, a22 = qf[R1:TQ, 0:128], qf[R1:TQ, 128:256]
        qc_ref[0:R1 // 2, 0:384] = _pk(jnp.concatenate(
            [_cat0(a11[0:R2] + a22, a11[R2:]), a12 - a11, _cat0(a12[0:R2] + a22, a12[R2:])], axis=1).astype(BF16))
        qc_ref[0:R2 // 2, 384:640] = _pk(jnp.concatenate([a21 - a22, a11[0:R2] + a21], axis=1).astype(BF16))

    def mlp_in(t):
        hp = jnp.dot(xq_of(t), _upk(wmi_p[...]), preferred_element_type=F32)
        last[0] = hp[0:16, 0:128]
        h = _gelu(hp)
        u_ref[_ds(t.fb, 0, TQ, 16), :] = h[:, :D]
        g = _ln(h[:, D:])
        halo = jnp.concatenate([g_buf[gi, _ds(t.cb, 0, 16, 32), :] for gi in range(G)], axis=1)
        e = jnp.concatenate([g[0:16] - halo, g[16:] - g[:TQ - 16]], axis=0)
        for gi in range(G):
            g_buf[gi, _ds(t.prev, 16 + TQ, 16, 32), :] = g[0:16, gi * 128:(gi + 1) * 128]
        for gi in range(G):
            g_buf[gi, _ds(t.cb, 16, TQ, 32), :] = g[:, gi * 128:(gi + 1) * 128]
            g_buf[G + gi, _ds(t.cb, 16, TQ, 32), :] = e[:, gi * 128:(gi + 1) * 128]
        for gi in range(G):
            g_buf[gi, _ds(t.next, 0, 16, 32), :] = g[TQ - 16:TQ, gi * 128:(gi + 1) * 128]

    def m_store(t, g0, v, r0=0):
        n = v.shape[0]
        halo = jnp.concatenate([m_buf[g0 + gi, _ds(t.cb, 16 + r0, 16, 32), :] for gi in range(G)], axis=1)
        parts = [v[0:16] - halo, v[16:] - v[:n - 16]]
        if r0 + n == TQ:
            parts.append(-v[n - 16:])
        e = jnp.concatenate(parts, axis=0)
        for gi in range(G):
            m_buf[g0 + gi, _ds(t.cb, 32 + r0, n, 32), :] = v[:, gi * 128:(gi + 1) * 128]
            m_buf[2 * G + g0 + gi, _ds(t.cb, 32 + r0, e.shape[0], 32), :] = e[:, gi * 128:(gi + 1) * 128]
        if n == TQ:
            for gi in range(G):
                m_buf[g0 + gi, _ds(t.next, 0, 32, 32), :] = v[TQ - 32:TQ, gi * 128:(gi + 1) * 128]
                m_buf[2 * G + g0 + gi, _ds(t.next, 16, 16, 32), :] = e[TQ - 16:TQ, gi * 128:(gi + 1) * 128]

    def mlp_out(t):
        gc = jnp.concatenate([_conv(g_buf, gi, G + gi, dw_f, 2 * G + gi, t.cb, 16, TQ, K) for gi in range(G)], axis=-1)
        u = u_ref[_ds(t.fb, 0, TQ, 16), :]
        loc = jnp.dot((u * gc).astype(BF16), _upk(wmo_p[...]), preferred_element_type=F32)
        m_store(t, G, loc)

    def merge_half(half, pieces):
        lhs = []
        for (t, off, nrows, _) in pieces:
            ms = [_conv(m_buf, gi, 2 * G + gi, dw_f, gi, t.cb, 32 - LAG + off, nrows, K)
                  for gi in range(half * G, (half + 1) * G)]
            lhs.append(jnp.concatenate(ms, axis=-1))
        lhs = lhs[0] if len(lhs) == 1 else jnp.concatenate(lhs, axis=0)
        return jnp.dot(lhs.astype(BF16), _upk(wm_p[half * D // 2:(half + 1) * D // 2, :]),
                       preferred_element_type=F32)

    def merge_loc(pieces):
        y = merge_half(1, pieces)
        r = 0
        for (t, off, nrows, yo) in pieces:
            y_ref[yo:yo + nrows, :] = x_buf[_ds(t.fb, off, nrows, 16), :].astype(F32) + y[r:r + nrows]
            r += nrows

    def merge_glob(pieces):
        y = merge_half(0, pieces)
        r = 0
        for (t, off, nrows, yo) in pieces:
            o_buf[_ds(t.fb, off, nrows, 16), :] = (y_ref[yo:yo + nrows, :] + y[r:r + nrows]).astype(BF16)
            r += nrows

    def max_update(ml, first, final):
        if final:
            return jnp.maximum(mp_ref[0:TQ], ml)
        mp_ref[0:TQ] = ml if first else jnp.maximum(mp_ref[0:TQ], ml)

    def scores_pair(t, a, b, pos):
        def nt(l, w):
            return lax.dot_general(_upk(l), _upk(w), NT_DIMS, preferred_element_type=F32)
        h1, h2, hs = R1 // 2, R2 // 2, 48
        f = {
            1: lambda j: nt(qc_ref[0:h1, 0:128], kc(t, j, 0)),
            11: lambda j: nt(qc_ref[0:hs, 0:128], kc(t, j, 0)),
            12: lambda j: nt(qc_ref[hs:h1, 0:128], kc(t, j, 0)),
            2: lambda j: nt(q_ref[0:h1, 0:128], kc(t, j, 4)),
            3: lambda j: nt(qc_ref[0:h2, 384:512], k_alo(t, j)),
            4: lambda j: nt(qc_ref[0:h1, 128:256], k_bhi(t, j)),
            5: lambda j: nt(q_ref[h1:TQ // 2, 128:256], kc(t, j, 3)),
            6: lambda j: nt(qc_ref[0:h2, 512:640], kc(t, j, 2)),
            7: lambda j: nt(qc_ref[0:h1, 256:384], kc(t, j, 1)),
            71: lambda j: nt(qc_ref[0:hs, 256:384], kc(t, j, 1)),
            72: lambda j: nt(qc_ref[hs:h1, 256:384], kc(t, j, 1)),
        }
        for j, order in ((a, (2, 4, 3, 5)), (b, (3, 5, 2, 4))):
            m = {k: f[k](j) for k in order}
            c0 = j * CK
            c12 = m[2] + m[4]
            c21 = m[3] + m[5]
            if j == a:
                last[0] = c12[0:16] + c21[0:16]
            s_ref[0:R1, c0 + 128:c0 + 256] = c12
            s_ref[R1:TQ, c0:c0 + 128] = c21
            s_ref[0:R1, c0:c0 + 128] = _cat0(m[4][0:R2] - m[5], m[4][R2:])
            s_ref[R1:TQ, c0 + 128:c0 + 256] = m[3] - m[2][0:R2]

        def off_diag(j):
            return _cat0(s_ref[0:R1, j * CK + 128:j * CK + 256], s_ref[R1:TQ, j * CK:j * CK + 128])

        def diag(j):
            return _cat0(s_ref[0:R1, j * CK:j * CK + 128], s_ref[R1:TQ, j * CK + 128:j * CK + 256])
        m1, m7, m6, m6b = f[1](a), f[7](a), f[6](a), f[6](b)
        c0 = a * CK
        c11 = s_ref[0:R1, c0:c0 + 128] + (m1 + m7)
        c22 = s_ref[R1:TQ, c0 + 128:c0 + 256] + (m1[0:R2] + m6)
        s_ref[0:R1, c0:c0 + 128] = c11
        s_ref[R1:TQ, c0 + 128:c0 + 256] = c22
        c0 = b * CK
        s_ref[R1:TQ, c0 + 128:c0 + 256] += m6b
        m11, m71, m12, m72 = f[11](b), f[71](b), f[12](b), f[72](b)
        m1, m7 = _cat0(m11, m12), _cat0(m71, m72)
        c11 = s_ref[0:R1, c0:c0 + 128] + (m1 + m7)
        c22 = s_ref[R1:TQ, c0 + 128:c0 + 256] + m1[0:R2]
        s_ref[0:R1, c0:c0 + 128] = c11
        s_ref[R1:TQ, c0 + 128:c0 + 256] = c22
        ml = jnp.maximum(_cat0(c11, c22), off_diag(b))
        ml = jnp.maximum(ml, jnp.maximum(off_diag(a), diag(a)))
        return max_update(ml, pos == 0, pos >= NC - 2)

    def scores_chunk(t, j, pos):
        q = _upk(q_ref[0:TQ // 2, :])
        if (j + 1) * CK <= T:
            sj = lax.dot_general(q, xa_chunk(t, j), NT_DIMS, preferred_element_type=F32)
            sts = [sj[:, 0:128], sj[:, 128:256]]
        else:
            nrem = T - j * CK - 128
            assert 0 < nrem < 128 and nrem % 16 == 0
            kf = _upk(xa_ref[_ds(t.kb, j * CK // 2, 64, 16), :])
            sj = jnp.concatenate([lax.dot_general(q[0:R1], kf, NT_DIMS, preferred_element_type=F32),
                                  lax.dot_general(q[R1:TQ], kf, NT_DIMS, preferred_element_type=F32)], axis=0)
            kr = _upk(xa_ref[_ds(t.kb, j * CK // 2 + 64, nrem // 2, 16), :])
            st = lax.dot_general(kr, _upk(q_ref[...]), NT_DIMS, preferred_element_type=F32)
            st = jnp.concatenate([st, jnp.full((128 - nrem, st.shape[1]), -jnp.inf, F32)], axis=0)
            sts = [sj, st.T[0:TQ]]
        last[0] = sj[0:16, 0:128]
        s_ref[:, j * CK:j * CK + 128] = sts[0]
        s_ref[:, j * CK + 128:(j + 1) * CK] = sts[1]
        return max_update(jnp.maximum(sts[0], sts[1]), pos == 0, pos == NC - 1)

    def scores_fin(mpart):
        m = jnp.max(mpart, axis=-1, keepdims=True)
        lam = jnp.sum(jnp.exp2(mpart - m), axis=-1, keepdims=True)
        m = m + jnp.log(lam) * LOG2E
        mx_ref[0:TQ] = jnp.broadcast_to(m, (TQ, 128))

    def pv_group(t, js, first, r0=0, r1=R1, r2=R2):
        ra, rb, rc = r0, r0 + r1, r0 + r1 + r2
        W = {1: lambda j: kc(t, j, 0), 2: lambda j: k_alo(t, j), 3: lambda j: kc(t, j, 1), 4: lambda j: kc(t, j, 2),
             5: lambda j: k_bhi(t, j), 6: lambda j: kc(t, j, 3), 7: lambda j: kc(t, j, 4)}
        done = set()

        def blk(r, c, j):
            lo, hi = (ra, rb) if r == 1 else (rb, rc)
            c0 = j * CK + (c - 1) * 128
            if (r, c, j) in done:
                return s_ref[lo:hi, c0:c0 + 128]
            done.add((r, c, j))
            p = jnp.exp2(s_ref[lo:hi, c0:c0 + 128] - mx_ref[lo:hi])
            s_ref[lo:hi, c0:c0 + 128] = p
            return p

        def lhs_of(k, j):
            if k == 1:
                a11 = blk(1, 1, j)
                return _cat0(a11[0:r2] + blk(2, 2, j), a11[r2:])
            if k == 2:
                return blk(2, 1, j) + blk(2, 2, j)
            if k == 3:
                return blk(1, 1, j)
            if k == 4:
                return blk(2, 2, j)
            if k == 5:
                return blk(1, 1, j) + blk(1, 2, j)
            if k == 6:
                return blk(2, 1, j) - blk(1, 1, j)[0:r2]
            a12 = blk(1, 2, j)
            return _cat0(a12[0:r2] - blk(2, 2, j), a12[r2:])
        for i, k in enumerate(VSEQ):
            ls = [lhs_of(k, j) for j in js]
            if k in (2, 5):
                lo, hi = (ra, rb) if k == 5 else (rb, rc)
                lsum = (ls[0] + ls[1]) + (ls[2] + ls[3])
                if first:
                    lp_ref[lo:hi] = lsum
                else:
                    lp_ref[lo:hi] += lsum
            lhs = jnp.concatenate(ls, axis=1).astype(BF16)
            rhs = _upk(jnp.concatenate([W[k](j) for j in js], axis=0))
            mk = jnp.dot(lhs, rhs, preferred_element_type=F32)
            last[0] = mk[0:16]
            if i == 0:
                first_w[0] = mk[0:16]
            n = mk.shape[0]
            if first:
                acc7_ref[k, 0:n] = mk
            else:
                acc7_ref[k, 0:n] += mk

    def pv_fin(t, r0=0, r1=R1, r2=R2):
        l = jnp.sum(lp_ref[r0:r0 + r1 + r2], axis=-1, keepdims=True)
        m1, m3, m5, m7 = (acc7_ref[k, 0:r1] for k in (1, 3, 5, 7))
        m2, m4, m6 = (acc7_ref[k, 0:r2] for k in (2, 4, 6))
        c11 = m1 + (m7 - m5)
        c11 = _cat0(c11[0:r2] + m4, c11[r2:])
        c12 = m3 + m5
        c21 = m2 + m4
        c22 = (m1[0:r2] - m2) + (m3[0:r2] + m6)
        acc = jnp.concatenate([jnp.concatenate([c11, c12], axis=1), jnp.concatenate([c21, c22], axis=1)], axis=0)
        o = acc * (1.0 / l)
        glob = jnp.dot(o.astype(BF16), _upk(wvo_p[...]), preferred_element_type=F32)
        m_store(t, 0, glob, r0)

    def pv_chunk(t, j, r0, n):
        c0 = j * CK
        pa = jnp.exp2(s_ref[r0:r0 + n, c0:c0 + 128] - mx_ref[r0:r0 + n])
        pb = jnp.exp2(s_ref[r0:r0 + n, c0 + 128:c0 + 256] - mx_ref[r0:r0 + n])
        lloc = pa + pb
        pv = jnp.dot(jnp.concatenate([pa, pb], axis=-1).astype(BF16), xa_chunk(t, j), preferred_element_type=F32)
        last[0] = pv[0:16, 0:128]
        if j == 0:
            lp_ref[r0:r0 + n] = lloc
            acc_ref[r0:r0 + n] = pv
        else:
            lp_ref[r0:r0 + n] += lloc
            acc_ref[r0:r0 + n] += pv

    def pv_chunk_fin(t, r0, n):
        l = jnp.sum(lp_ref[r0:r0 + n], axis=-1, keepdims=True)
        o = (acc_ref[r0:r0 + n] * (1.0 / l)).astype(BF16)
        glob = jnp.dot(o, _upk(wvo_p[...]), preferred_element_type=F32)
        m_store(t, 0, glob, r0)

    def anchor(op):
        if op == 'Zx':
            zrow = pl.multiple_of(zoff[0], 16)
            x_buf[pl.ds(zrow + B * T + LAG + TP - T, 16), 0:128] = last[0].astype(BF16)
            return
        zrow = pl.multiple_of(zoff[0], 8)
        if op in ('Z', 'Zg'):
            (m_buf if op == 'Z' else g_buf)[0, pl.ds(zrow + NS * SLOT + 64, 8), :] = last[0][0:8]
        else:
            (lp_ref if op == 'Zl' else mx_ref)[pl.ds(zrow + TQ, 8), :] = last[0][0:8]

    def step(order, pb, pa, t0, tp, th=None, un=None, dma=None):
        cord, nxt = [], 0
        for op in order:
            if op == 'KK':
                cord += [nxt, nxt + 1]
                nxt += 2
            elif op in ('Ks', 'K'):
                cord.append(NC - 2 if op == 'Ks' else NC - 1)
        assert 4 * order.count('W') == NC and sorted(cord) == list(range(NC))
        mpart = None
        jv = jk = 0
        nq = []
        for op in order:
            if op == 'q':
                qproj(tp)
            elif op == 'W':
                pv_group(t0, cord[jv:jv + 4], jv == 0)
                jv += 4
            elif op == 'G':
                pv_fin(t0)
            elif op in ('K', 'Ks'):
                assert jk < jv
                mpart = scores_chunk(tp, cord[jk], jk)
                jk += 1
            elif op == 'KK':
                assert jk + 1 < jv
                mpart = scores_pair(tp, cord[jk], cord[jk + 1], jk)
                jk += 2
            elif op[0] == 'Z':
                anchor(op)
            elif op == 'Ma':
                merge_loc(pa)
            elif op == 'Mb':
                merge_glob(pb)
            elif op == 'H':
                mlp_in(th)
            elif op == 'L':
                mlp_out(tp)
            elif op == 'n':
                r = (len(nq) // 2) * 256 + (len(nq) % 2) * 64
                xa_, xb_ = (_ln(x_buf[_ds(un * 512, LAG + T + r + o, 64, 16), :].astype(F32)) for o in (0, 128))
                v = jnp.concatenate(
                    [xa_, xb_] + _key_combos(xa_[:, 0:128], xa_[:, 128:256], xb_[:, 0:128], xb_[:, 128:256]), axis=1)
                nq.append((r, _pk(v.astype(BF16))))
            elif op == 'Ns':
                assert len(nq) == 4
                for r, v in nq:
                    xa_ref[_ds(un * 256, TP // 2 + r // 2, 32, 256), :] = v[:, 0:256]
                    xa_ref[_ds(un * 256, TP // 2 + r // 2 + 64, 32, 256), :] = v[:, 256:512]
                    kc_ref[_ds(un * 128, TP // 4 + (r // 256) * 64 + (r % 256) // 2, 32, 128), :] = v[:, 512:1152]
            elif op == 'D':
                dma()
            else:
                raise ValueError(op)
        scores_fin(mpart)

    done, nln = [], 0
    for op in PROLOGUE[split + 1:]:
        if op[0] == 's':
            dma_start(op)
        elif op[0] == 'x':
            x_copy(int(op[1:])).wait()
        elif op[0] == 'w':
            w_copy(int(op[1:])).wait()
        elif op[0] == 'n':
            ln_unit(int(op[1:]))
            nln = int(op[1:]) + 1
        elif op[0] == 'p':
            prep(int(op[1:]))
        elif op == 'A':
            prep_a()
        elif op == 'q':
            qproj(tile(0), False)
        elif op.startswith('KK'):
            j = int(op[2:])
            assert nln * 512 >= (j + 2) * CK
            mpart = scores_pair(tile(0), j, j + 1, len(done))
            done += [j, j + 1]
        elif op[0] == 'K':
            j = int(op[1:])
            assert nln * 512 >= (j + 1) * CK
            mpart = scores_chunk(tile(0), j, len(done))
            done.append(j)
        elif op[0] == 'H':
            assert nln * 512 >= (int(op[1:]) + 1) * TQ
            mlp_in(tile(int(op[1:])))
        elif op == 'L0':
            mlp_out(tile(0))
        elif op[0] == 'Z':
            anchor(op)
        else:
            raise ValueError(op)
    assert sorted(done) == list(range(NC))
    scores_fin(mpart)

    def body_a(order, s, c):
        if 'Ns' in order:
            @pl.when(s == 1)
            def _():
                x_copy(NU + 1).wait()

        w = jnp.maximum(s - 1, 0)
        fb = w * TQ

        def dma():
            @pl.when(s > 0)
            def _():
                out_copy(fb, LAG, TQ - LAG).start()

            @pl.when(jnp.logical_and(s > 1, s != NT + 1))
            def _():
                out_copy(fb, 0, LAG).start()

        step(order, [(tile(w), 0, TQ, 0)], [(tile(s), 0, TQ, 0)], tile(s), tile(s + 1), tile(s + 3), s, dma)
        return c
    lax.fori_loop(0, NU, functools.partial(body_a, STEP_A1), 0)
    lax.fori_loop(NU, NS - 3, functools.partial(body_a, STEP_A2), 0)

    z = zoff[0]
    tail0 = (tile(NT - 1), TQ, LAG, TQ + LAG)
    Y2 = TQ + 3 * LAG

    def body_b(s, c):
        step(STEP_B, [(tile(s - 1), 0, TQ, 0)], [(tile(s), 0, TQ, 0), tail0], tile(s), tile(s + 1))
        out_copy((s - 1) * TQ, 0, TQ).start()
        return c
    lax.fori_loop(NS - 3, NS - 1, body_b, 0)

    def last_block(ops):
        tl = tile(z + (NS - 1))
        j = 0
        saved = None
        for op in ops:
            if op == 'WA':
                pv_group(tl, list(range(j, j + 4)), j == 0, 0, RA // 2, RA // 2)
                j += 4
            elif op == 'B':
                pv_chunk(tl, j, RA, TQ - RA)
                j += 1
            elif op == 'Ga':
                pv_fin(tl, 0, RA // 2, RA // 2)
            elif op == 'Gb':
                pv_chunk_fin(tl, RA, TQ - RA)
            elif op == 'E':
                last[0] = first_w[0]
            elif op == 'S':
                saved = last[0]
            elif op == 'R':
                last[0] = saved
            elif op[0] == 'Z':
                anchor(op)
            elif op == 'Mb':
                merge_glob([(tile(z + (NS - 2)), 0, TQ, 0), tail0])
                out_copy(0, (NS - 2) * TQ, TQ).start()
                out_copy(0, NT * TQ, LAG).start()
            elif op == 'Mc':
                merge_loc([(tl, 0, TQ + LAG, Y2)])
            elif op == 'M1':
                merge_glob([(tl, 0, RA, Y2)])
                out_copy(0, (NS - 1) * TQ, RA).start()
            elif op == 'M2':
                merge_glob([(tl, RA, TQ + LAG - RA, Y2 + RA)])
                out_copy(0, (NS - 1) * TQ + RA, TQ + LAG - RA).start()
            else:
                raise ValueError(op)
        assert j == NC

    pl.when(z < 1)(functools.partial(last_block, LAST_A))
    pl.when(z < 2)(functools.partial(last_block, LAST_B))

    out_copy(0, LAG, B * T).wait()


@jax.jit
def pallas_standalone__conformer_family_e_branchformer__speech_kernel(
    x: jax.Array,
    w_qkv: jax.Array,
    w_att_out: jax.Array,
    w_mlp_in: jax.Array,
    dw_csgu: jax.Array,
    w_mlp_out: jax.Array,
    dw_merge: jax.Array,
    w_merge: jax.Array,
):
    B, T, D = x.shape
    K = dw_csgu.shape[0]
    TP = (T + 511) // 512 * 512
    G = D // 128
    RB = (B * (T // TQ) + 1) * SLOT
    out = pl.pallas_call(
        functools.partial(_kernel, B=B, T=T, D=D, K=K, TP=TP),
        in_specs=[pl.BlockSpec(memory_space=pl.ANY)] * 8,
        out_specs=pl.BlockSpec(memory_space=pl.ANY),
        out_shape=jax.ShapeDtypeStruct((B * T, D), x.dtype),
        scratch_shapes=[
            pltpu.VMEM((B * T + 32 + TP - T, D), BF16),
            pltpu.VMEM((B * T + 32, D), BF16),
            pltpu.VMEM((B * TP // 2, D), U32),
            pltpu.VMEM((D // 2, D), U32),
            pltpu.VMEM((D // 2, D), U32),
            pltpu.VMEM((D // 2, 2 * D), U32),
            pltpu.VMEM((D // 2, D), U32),
            pltpu.VMEM((D, D), U32),
            pltpu.VMEM((64, 896), U32),
            pltpu.VMEM((3 * G, 48, 8, 128), F32),
            pltpu.VMEM((2 * G, RB, 128), F32),
            pltpu.VMEM((4 * G, RB, 128), F32),
            pltpu.VMEM((B * T, D), F32),
            pltpu.VMEM((TQ, TP), F32),
            pltpu.VMEM((TQ + 16, 128), F32),
            pltpu.VMEM((256, D), U32),
            pltpu.VMEM((128, 640), U32),
            pltpu.VMEM((B * TP // 4, 640), U32),
            pltpu.VMEM((TQ + 16, 128), F32),
            pltpu.VMEM((TQ + 16, 128), F32),
            pltpu.VMEM((TQ, D), F32),
            pltpu.VMEM((8, 224, 128), F32),
            pltpu.VMEM((2 * TQ + 4 * LAG, D), F32),
            pltpu.VMEM(w_qkv.shape, BF16),
            pltpu.VMEM(w_att_out.shape, BF16),
            pltpu.VMEM(w_mlp_in.shape, BF16),
            pltpu.VMEM(dw_csgu.shape, BF16),
            pltpu.VMEM(w_mlp_out.shape, BF16),
            pltpu.VMEM(dw_merge.shape, BF16),
            pltpu.VMEM(w_merge.shape, BF16),
            pltpu.SMEM((1,), jnp.int32),
            pltpu.SemaphoreType.DMA((max(GRP.values()) + 1,)),
            pltpu.SemaphoreType.DMA,
        ],
        compiler_params=pltpu.CompilerParams(vmem_limit_bytes=120 * 1024 * 1024, disable_bounds_checks=True),
    )(x.reshape(B * T, D), w_qkv, w_att_out, w_mlp_in, dw_csgu, w_mlp_out, dw_merge, w_merge)
    return out.reshape(B, T, D)
```

```python
import functools

import jax
import jax.numpy as jnp
from jax import lax
import jax.experimental.pallas as pl
import jax.experimental.pallas.tpu as pltpu

F32 = jnp.float32
BF16 = jnp.bfloat16
U32 = jnp.uint32
LOG2E = 1.4426950408889634
NT_DIMS = (((1,), (1,)), ((), ()))

TQ = 400
CK = 256
SLOT = 448
LAG = 16
R1 = 208
R2 = TQ - R1
RA = 288
VSEQ = (3, 4, 1, 5, 7, 2, 6)

PROLOGUE = (
    'sx0 sw0 | x0 sx1 sw1 n0 w0 sx2 sx3 A q x1 w1 sx4 sx5 sw3 sw4 p1 H0 n1 KK0 '
    'x2 x3 x4 sx6 sx7 sw2 sw5 sw6 sw7 sx8 n2 n3 KK2 KK4 KK6 H1 H2 n4 J8 '
    'x5 x6 x7 w3 w4 w2 w5 w6 w7 x8 sx9 p3 p4 p5 p6 n5 K9 Zg KK10 n6 KK12 n7 K15 K14 p2 L0').split()
STEP_A1 = 'q Z Zg W W Mb D W Ma W Zl L K K1 H KK KK Zx n KK Zx n KK Zx n KK Zx n KK KK Ns G'.split()
STEP_A2 = 'q Z Zg W W Mb D W Ma W Zl L H KK K K1 KK KK KK KK KK KK G'.split()
STEP_B = 'q Z Zg W W Mb K W Ma W Zl L K1 KK KK KK KK KK KK KK G'.split()
LAST_A = 'WA E Z WA WA Mb WA Zl Mc Ga'.split()
LAST_B = 'B Z S B B R Zm B S B B R Zm B B B B B B B B B B Zl M1 Gb M2'.split()


def _sem_groups():
    grp, g, prev = {}, -1, False
    for op in PROLOGUE:
        is_wait = op[0] in 'xw'
        if is_wait:
            g += 0 if prev else 1
            grp[op] = g
        prev = is_wait
    grp['x9'] = g + 1
    return grp


GRP = _sem_groups()


def _pk(x):
    return pltpu.bitcast(x, U32)


def _upk(x):
    return pltpu.bitcast(x, BF16)


def _cat0(u, v):
    return jnp.concatenate([u, v], axis=0) if v.shape[0] else u


def _ln(x, eps=1e-5):
    m = jnp.mean(x, axis=-1, keepdims=True)
    xc = x - m
    v = jnp.mean(xc * xc, axis=-1, keepdims=True)
    return xc * jnp.exp2(jnp.log(v + eps) * (-0.5 * LOG2E))


def _gelu(x):
    c = 0.7978845608028654
    hx = 0.5 * x
    return hx + hx * jnp.tanh(x * (c + (c * 0.044715) * (x * x)))


def _ds(base, off, n, align):
    if isinstance(base, int):
        return pl.ds(base + off, n)
    a = align
    while off % a:
        a //= 2
    return pl.ds(pl.multiple_of(base + off, a), n) if a > 1 else pl.ds(base + off, n)


def _conv_direct(buf_ref, g, w_ref, wg, base, off, nrows, K):
    V = nrows // 8
    acc = None
    for p in range(8):
        taps = list(range(p, K, 8))
        nq = V + len(taps) - 1
        slab = buf_ref[g, _ds(base, off + p - K // 2, 8 * nq, 32), :].reshape(nq, 8, 128)
        for qi, i in enumerate(taps):
            term = slab[qi:qi + V] * w_ref[wg, i][None]
            acc = term if acc is None else acc + term
    return acc.reshape(8 * V, 128)


def _conv(buf_ref, g, ge, w_ref, wg, base, off, nrows, K):
    nq = nrows // 32
    outs = []
    q0 = 0
    while q0 < nq:
        Q = min(4, nq - q0)
        am = a0 = a1 = None
        for i in [p + 8 * h for p in range(8) for h in range(2)]:
            r = off + 32 * q0 + i - K // 2 + 16
            xs = buf_ref[g, _ds(base, r, 32 * Q - 16, 32), :]
            xs = jnp.concatenate([xs[32 * k:32 * k + 16] for k in range(Q)], axis=0).reshape(2 * Q, 8, 128)
            t = xs * w_ref[wg, 32 + i][None]
            am = t if am is None else am + t
            if i + 16 < K:
                es = buf_ref[ge, _ds(base, r, 32 * Q, 32), :]
                e2 = jnp.concatenate([es[32 * k + 16:32 * k + 32] for k in range(Q)], axis=0).reshape(2 * Q, 8, 128)
                t = e2 * w_ref[wg, i + 16][None]
                a1 = t if a1 is None else a1 + t
            else:
                es = buf_ref[ge, _ds(base, r, 32 * Q - 16, 32), :]
            e1 = jnp.concatenate([es[32 * k:32 * k + 16] for k in range(Q)], axis=0).reshape(2 * Q, 8, 128)
            t = e1 * w_ref[wg, i][None]
            a0 = t if a0 is None else a0 + t
        y0 = (am - a0).reshape(16 * Q, 128)
        y1 = (am + a1).reshape(16 * Q, 128)
        for k in range(Q):
            outs += [y0[16 * k:16 * k + 16], y1[16 * k:16 * k + 16]]
        q0 += Q
    if nrows % 32:
        outs.append(_conv_direct(buf_ref, g, w_ref, wg, base, off + 32 * nq, nrows - 32 * nq, K))
    return jnp.concatenate(outs, axis=0) if len(outs) > 1 else outs[0]


def _key_combos(alo, ahi, blo, bhi):
    return [alo + bhi, ahi - bhi, blo - alo, alo + ahi, blo + bhi]


class _Tile:
    def __init__(self, t, NT, NS, TP, T):
        if isinstance(t, int):
            b = t // NT
            self.prev = (NS if t % NT == 0 else t - 1) * SLOT
            self.next = (NS if t % NT == NT - 1 else t + 1) * SLOT
        else:
            b = (t >= NT).astype(jnp.int32)
            first = jnp.logical_or(t == 0, t == NT)
            last = jnp.logical_or(t == NT - 1, t == NS - 1)
            self.prev = jnp.where(first, NS, t - 1) * SLOT
            self.next = jnp.where(last, NS, t + 1) * SLOT
        self.cb = t * SLOT
        self.fb = t * TQ
        self.ab = t * (TQ // 2) + b * ((TP - T) // 2)
        self.kb = b * (TP // 2)
        self.cbk = b * (TP // 4)


def _kernel(x_hbm, wqkv_hbm, wao_hbm, wmi_hbm, dwc_hbm, wmo_hbm, dwm_hbm, wm_hbm, o_hbm,
            x_buf, o_buf, xa_ref, wa_p, wvo_p, wmi_p, wmo_p, wm_p, ws_ref, dw_f, g_buf, m_buf, u_ref,
            s_ref, mx_ref, q_ref, qc_ref, kc_ref, mp_ref, lp_ref, acc_ref, acc7_ref, y_ref,
            wqkv_ref, wao_ref, wmi_ref, dwc_ref, wmo_ref, dwm_ref, wm_ref,
            zoff, sem_in, sem_out,
            *, B, T, D, K, TP):
    NT = T // TQ
    NS = B * NT
    G = D // 128
    NC = TP // CK
    NU = TP // 512
    assert B == 2 and D == 256 and K == 31 and T % TQ == 0 and NC == 16
    last = [None]
    first_w = [None]

    def tile(t):
        return _Tile(t, NT, NS, TP, T)

    def x_copy(u):
        r0 = u * 512 if u < NU else (T if u == NU else T + 512)
        n = min(512, T - r0) if u < NU else (512 if u == NU else T - 512)
        return pltpu.make_async_copy(x_hbm.at[pl.ds(r0, n), :], x_buf.at[pl.ds(LAG + r0, n), :],
                                     sem_in.at[GRP['x%d' % u]])

    w_pairs = [(wqkv_hbm.at[:, 0:2 * D], wqkv_ref.at[:, 0:2 * D]), (wmi_hbm, wmi_ref), (wao_hbm, wao_ref),
               (dwc_hbm, dwc_ref), (wmo_hbm, wmo_ref), (dwm_hbm, dwm_ref), (wm_hbm, wm_ref),
               (wqkv_hbm.at[:, 2 * D:3 * D], wqkv_ref.at[:, 2 * D:3 * D])]

    def w_copy(k):
        return pltpu.make_async_copy(w_pairs[k][0], w_pairs[k][1], sem_in.at[GRP['w%d' % k]])

    def dma_start(op):
        (x_copy if op[1] == 'x' else w_copy)(int(op[2:])).start()

    def out_copy(base, off, n):
        return pltpu.make_async_copy(o_buf.at[_ds(base, off, n, 16), :], o_hbm.at[_ds(base, off - LAG, n, 16), :],
                                     sem_out)

    split = PROLOGUE.index('|')
    for op in PROLOGUE[:split]:
        dma_start(op)

    zoff[0] = 0
    z16 = jnp.zeros((16, 128), F32)
    for b in range(B):
        lo, hi = b * NT * SLOT, ((b + 1) * NT - 1) * SLOT
        for gi in range(G):
            g_buf[gi, lo:lo + 16, :] = z16
            g_buf[gi, hi + 416:hi + 432, :] = z16
        for gi in range(2 * G):
            m_buf[gi, lo:lo + 16, :] = z16
            m_buf[gi, lo + 16:lo + 32, :] = z16
            m_buf[2 * G + gi, lo + 16:lo + 32, :] = z16
            m_buf[gi, hi + 432:hi + 448, :] = z16
    for gi in range(G):
        m_buf[gi, 32:32 + TQ, :] = jnp.zeros((TQ, 128), F32)
        m_buf[2 * G + gi, 32:32 + TQ, :] = jnp.zeros((TQ, 128), F32)
    y_ref[0:TQ, :] = jnp.zeros((TQ, D), F32)
    x_buf[0:LAG, :] = jnp.zeros((LAG, D), BF16)
    x_buf[LAG + B * T:LAG + B * T + TP - T, :] = jnp.zeros((TP - T, D), BF16)
    q_ref[TQ // 2:, :] = jnp.zeros((q_ref.shape[0] - TQ // 2, D), U32)

    def prep_a():
        a = lax.dot_general(wqkv_ref[:, 0:D], wqkv_ref[:, D:2 * D], NT_DIMS, preferred_element_type=F32)
        a = a * (D ** -0.5 * LOG2E)
        wa_p[...] = _pk(a.astype(BF16))
        b11, b12, b21, b22 = a[0:128, 0:128], a[0:128, 128:256], a[128:256, 0:128], a[128:256, 128:256]
        ws_ref[...] = _pk(jnp.concatenate(
            [b11 + b22, b11, b12 - b22, b21 - b11, b22, b11 + b12, b21 + b22], axis=1).astype(BF16))

    def prep(k):
        if k == 1:
            wmi_p[...] = _pk(wmi_ref[...])
        elif k == 2:
            wvo = jnp.dot(wqkv_ref[:, 2 * D:3 * D], wao_ref[...], preferred_element_type=F32)
            wvo_p[...] = _pk(wvo.astype(BF16))
        elif k == 4:
            wmo_p[...] = _pk(wmo_ref[...])
        elif k == 6:
            wm_p[...] = _pk(wm_ref[...])
        else:
            dw = (dwc_ref if k == 3 else dwm_ref)[...].astype(F32)
            g0 = 2 * G if k == 3 else 0
            if k == 5:
                row = lax.broadcasted_iota(jnp.int32, dw.shape, 0)
                dw = jnp.where(row == K // 2, dw + 1.0, dw)
            for gi in range(dw.shape[1] // 128):
                for i in range(K):
                    dw_f[g0 + gi, i] = jnp.broadcast_to(dw[i:i + 1, gi * 128:(gi + 1) * 128], (8, 128))
                for i in range(16):
                    v = dw_f[g0 + gi, i]
                    dw_f[g0 + gi, 32 + i] = v + dw_f[g0 + gi, i + 16] if i + 16 < K else v

    def ln_unit(u):
        n = min(512, T - u * 512)
        xk = _ln(x_buf[pl.ds(LAG + u * 512, n), :].astype(F32))
        if n < 512:
            xk = jnp.concatenate([xk, jnp.zeros((512 - n, D), F32)], axis=0)
        vs = []
        for r in (0, 256):
            vs.append(jnp.concatenate(_key_combos(xk[r:r + 128, 0:128], xk[r:r + 128, 128:256],
                                                  xk[r + 128:r + 256, 0:128], xk[r + 128:r + 256, 128:256]), axis=1))
        xa_p, kc_p = _pk(xk.astype(BF16)), _pk(jnp.concatenate(vs, axis=0).astype(BF16))
        xa_ref[u * 256:(u + 1) * 256, :] = xa_p
        kc_ref[u * 128:(u + 1) * 128, :] = kc_p

    def xq_of(t):
        return _upk(xa_ref[_ds(t.ab, 0, TQ // 2, 8), :])

    def xa_chunk(t, j):
        return _upk(xa_ref[_ds(t.kb, j * CK // 2, CK // 2, 16), :])

    def kc(t, j, i):
        return kc_ref[_ds(t.cbk, j * 64, 64, 32), i * 128:(i + 1) * 128]

    def k_alo(t, j):
        return xa_ref[_ds(t.kb, j * 128, 64, 16), 0:128]

    def k_bhi(t, j):
        return xa_ref[_ds(t.kb, j * 128 + 64, 64, 16), 128:256]

    def q_strassen(lhs):
        a11, a12, a21, a22 = lhs[0:R1, 0:128], lhs[0:R1, 128:256], lhs[R1:TQ, 0:128], lhs[R1:TQ, 128:256]
        p1 = jnp.concatenate([_cat0(a11[0:R2] + a22, a11[R2:]), a11, a11 + a12, _cat0(a12[0:R2] - a22, a12[R2:])],
                             axis=1).astype(BF16)
        p2 = jnp.concatenate([a21 + a22, a22, a21 - a11[0:R2]], axis=1).astype(BF16)
        lk = {1: p1[:, 0:128], 3: p1[:, 128:256], 5: p1[:, 256:384], 7: p1[:, 384:512],
              2: p2[:, 0:128], 4: p2[:, 128:256], 6: p2[:, 256:384]}

        def job(k, lo=None, hi=None):
            l = lk[k] if lo is None else lk[k][lo:hi]
            return jnp.dot(l, _upk(ws_ref[:, (k - 1) * 128:k * 128]), preferred_element_type=F32)
        s1, s2 = 144, 160
        m3, m5, m2, m4 = job(3), job(5), job(2), job(4)
        m6a = job(6, 0, s2)
        m1b = job(1, s1, R1)
        m1a = job(1, 0, s1)
        m7a = job(7, 0, s1)
        m7b = job(7, s1, R1)
        m6 = _cat0(m6a, job(6, s2, R2))
        m1, m7 = _cat0(m1a, m1b), _cat0(m7a, m7b)
        c12 = m3 + m5
        c21 = m2 + m4
        last[0] = c12[0:16] + c21[0:16]
        c11 = _cat0(m4 - m5[0:R2], -m5[R2:]) + (m1 + m7)
        c22 = ((m3[0:R2] - m2) + m6) + m1[0:R2]
        return jnp.concatenate([jnp.concatenate([c11, c12], axis=1), jnp.concatenate([c21, c22], axis=1)], axis=0)

    def qproj(t, fast=True):
        if fast:
            qf = q_strassen(xq_of(t).astype(F32))
        else:
            qf = jnp.dot(xq_of(t), _upk(wa_p[...]), preferred_element_type=F32)
            last[0] = qf[0:16, 0:128]
        q_ref[0:TQ // 2, :] = _pk(qf.astype(BF16))
        a11, a12 = qf[0:R1, 0:128], qf[0:R1, 128:256]
        a21, a22 = qf[R1:TQ, 0:128], qf[R1:TQ, 128:256]
        qc_ref[0:R1 // 2, 0:384] = _pk(jnp.concatenate(
            [_cat0(a11[0:R2] + a22, a11[R2:]), a12 - a11, _cat0(a12[0:R2] + a22, a12[R2:])], axis=1).astype(BF16))
        qc_ref[0:R2 // 2, 384:640] = _pk(jnp.concatenate([a21 - a22, a11[0:R2] + a21], axis=1).astype(BF16))

    def mlp_in(t):
        hp = jnp.dot(xq_of(t), _upk(wmi_p[...]), preferred_element_type=F32)
        last[0] = hp[0:16, 0:128]
        h = _gelu(hp)
        u_ref[_ds(t.fb, 0, TQ, 16), :] = h[:, :D]
        g = _ln(h[:, D:])
        halo = jnp.concatenate([g_buf[gi, _ds(t.cb, 0, 16, 32), :] for gi in range(G)], axis=1)
        e = jnp.concatenate([g[0:16] - halo, g[16:] - g[:TQ - 16]], axis=0)
        for gi in range(G):
            g_buf[gi, _ds(t.prev, 16 + TQ, 16, 32), :] = g[0:16, gi * 128:(gi + 1) * 128]
        for gi in range(G):
            g_buf[gi, _ds(t.cb, 16, TQ, 32), :] = g[:, gi * 128:(gi + 1) * 128]
            g_buf[G + gi, _ds(t.cb, 16, TQ, 32), :] = e[:, gi * 128:(gi + 1) * 128]
        for gi in range(G):
            g_buf[gi, _ds(t.next, 0, 16, 32), :] = g[TQ - 16:TQ, gi * 128:(gi + 1) * 128]

    def m_store(t, g0, v, r0=0):
        n = v.shape[0]
        halo = jnp.concatenate([m_buf[g0 + gi, _ds(t.cb, 16 + r0, 16, 32), :] for gi in range(G)], axis=1)
        parts = [v[0:16] - halo, v[16:] - v[:n - 16]]
        if r0 + n == TQ:
            parts.append(-v[n - 16:])
        e = jnp.concatenate(parts, axis=0)
        for gi in range(G):
            m_buf[g0 + gi, _ds(t.cb, 32 + r0, n, 32), :] = v[:, gi * 128:(gi + 1) * 128]
            m_buf[2 * G + g0 + gi, _ds(t.cb, 32 + r0, e.shape[0], 32), :] = e[:, gi * 128:(gi + 1) * 128]
        if n == TQ:
            for gi in range(G):
                m_buf[g0 + gi, _ds(t.next, 0, 32, 32), :] = v[TQ - 32:TQ, gi * 128:(gi + 1) * 128]
                m_buf[2 * G + g0 + gi, _ds(t.next, 16, 16, 32), :] = e[TQ - 16:TQ, gi * 128:(gi + 1) * 128]

    def mlp_out(t):
        gc = jnp.concatenate([_conv(g_buf, gi, G + gi, dw_f, 2 * G + gi, t.cb, 16, TQ, K) for gi in range(G)], axis=-1)
        u = u_ref[_ds(t.fb, 0, TQ, 16), :]
        loc = jnp.dot((u * gc).astype(BF16), _upk(wmo_p[...]), preferred_element_type=F32)
        m_store(t, G, loc)

    def merge_half(half, pieces):
        lhs = []
        for (t, off, nrows, _) in pieces:
            ms = [_conv(m_buf, gi, 2 * G + gi, dw_f, gi, t.cb, 32 - LAG + off, nrows, K)
                  for gi in range(half * G, (half + 1) * G)]
            lhs.append(jnp.concatenate(ms, axis=-1))
        lhs = lhs[0] if len(lhs) == 1 else jnp.concatenate(lhs, axis=0)
        return jnp.dot(lhs.astype(BF16), _upk(wm_p[half * D // 2:(half + 1) * D // 2, :]),
                       preferred_element_type=F32)

    def merge_loc(pieces):
        y = merge_half(1, pieces)
        r = 0
        for (t, off, nrows, yo) in pieces:
            y_ref[yo:yo + nrows, :] = x_buf[_ds(t.fb, off, nrows, 16), :].astype(F32) + y[r:r + nrows]
            r += nrows

    def merge_glob(pieces):
        y = merge_half(0, pieces)
        r = 0
        for (t, off, nrows, yo) in pieces:
            o_buf[_ds(t.fb, off, nrows, 16), :] = (y_ref[yo:yo + nrows, :] + y[r:r + nrows]).astype(BF16)
            r += nrows

    def max_update(ml, first, final):
        if final:
            return jnp.maximum(mp_ref[0:TQ], ml)
        mp_ref[0:TQ] = ml if first else jnp.maximum(mp_ref[0:TQ], ml)

    def scores_pair(t, a, b, pos):
        def nt(l, w):
            return lax.dot_general(_upk(l), _upk(w), NT_DIMS, preferred_element_type=F32)
        h1, h2, hs = R1 // 2, R2 // 2, 48
        f = {
            1: lambda j: nt(qc_ref[0:h1, 0:128], kc(t, j, 0)),
            11: lambda j: nt(qc_ref[0:hs, 0:128], kc(t, j, 0)),
            12: lambda j: nt(qc_ref[hs:h1, 0:128], kc(t, j, 0)),
            2: lambda j: nt(q_ref[0:h1, 0:128], kc(t, j, 4)),
            3: lambda j: nt(qc_ref[0:h2, 384:512], k_alo(t, j)),
            4: lambda j: nt(qc_ref[0:h1, 128:256], k_bhi(t, j)),
            5: lambda j: nt(q_ref[h1:TQ // 2, 128:256], kc(t, j, 3)),
            6: lambda j: nt(qc_ref[0:h2, 512:640], kc(t, j, 2)),
            7: lambda j: nt(qc_ref[0:h1, 256:384], kc(t, j, 1)),
            71: lambda j: nt(qc_ref[0:hs, 256:384], kc(t, j, 1)),
            72: lambda j: nt(qc_ref[hs:h1, 256:384], kc(t, j, 1)),
        }
        for j, order in ((a, (2, 4, 3, 5)), (b, (3, 5, 2, 4))):
            m = {k: f[k](j) for k in order}
            c0 = j * CK
            c12 = m[2] + m[4]
            c21 = m[3] + m[5]
            if j == a:
                last[0] = c12[0:16] + c21[0:16]
            s_ref[0:R1, c0 + 128:c0 + 256] = c12
            s_ref[R1:TQ, c0:c0 + 128] = c21
            s_ref[0:R1, c0:c0 + 128] = _cat0(m[4][0:R2] - m[5], m[4][R2:])
            s_ref[R1:TQ, c0 + 128:c0 + 256] = m[3] - m[2][0:R2]

        def off_diag(j):
            return _cat0(s_ref[0:R1, j * CK + 128:j * CK + 256], s_ref[R1:TQ, j * CK:j * CK + 128])

        def diag(j):
            return _cat0(s_ref[0:R1, j * CK:j * CK + 128], s_ref[R1:TQ, j * CK + 128:j * CK + 256])
        m1, m7, m6, m6b = f[1](a), f[7](a), f[6](a), f[6](b)
        c0 = a * CK
        c11 = s_ref[0:R1, c0:c0 + 128] + (m1 + m7)
        c22 = s_ref[R1:TQ, c0 + 128:c0 + 256] + (m1[0:R2] + m6)
        s_ref[0:R1, c0:c0 + 128] = c11
        s_ref[R1:TQ, c0 + 128:c0 + 256] = c22
        c0 = b * CK
        s_ref[R1:TQ, c0 + 128:c0 + 256] += m6b
        m11, m71, m12, m72 = f[11](b), f[71](b), f[12](b), f[72](b)
        m1, m7 = _cat0(m11, m12), _cat0(m71, m72)
        c11 = s_ref[0:R1, c0:c0 + 128] + (m1 + m7)
        c22 = s_ref[R1:TQ, c0 + 128:c0 + 256] + m1[0:R2]
        s_ref[0:R1, c0:c0 + 128] = c11
        s_ref[R1:TQ, c0 + 128:c0 + 256] = c22
        ml = jnp.maximum(_cat0(c11, c22), off_diag(b))
        ml = jnp.maximum(ml, jnp.maximum(off_diag(a), diag(a)))
        return max_update(ml, pos == 0, pos >= NC - 2)

    def scores_single(t, j, pos):
        def nt(l, w):
            return lax.dot_general(_upk(l), _upk(w), NT_DIMS, preferred_element_type=F32)
        h1, h2 = R1 // 2, R2 // 2
        m2 = nt(q_ref[0:h1, 0:128], kc(t, j, 4))
        m4 = nt(qc_ref[0:h1, 128:256], k_bhi(t, j))
        m3 = nt(qc_ref[0:h2, 384:512], k_alo(t, j))
        m5 = nt(q_ref[h1:TQ // 2, 128:256], kc(t, j, 3))
        last[0] = m2[0:16]
        c0 = j * CK
        s_ref[0:R1, c0 + 128:c0 + 256] = m2 + m4
        s_ref[R1:TQ, c0:c0 + 128] = m3 + m5
        s_ref[0:R1, c0:c0 + 128] = _cat0(m4[0:R2] - m5, m4[R2:])
        s_ref[R1:TQ, c0 + 128:c0 + 256] = m3 - m2[0:R2]
        m1a = nt(qc_ref[0:48, 0:128], kc(t, j, 0))
        m7a = nt(qc_ref[0:48, 256:384], kc(t, j, 1))
        m6a = nt(qc_ref[0:48, 512:640], kc(t, j, 2))
        m6b = nt(qc_ref[48:h2, 512:640], kc(t, j, 2))
        m1b = nt(qc_ref[48:72, 0:128], kc(t, j, 0))
        m7b = nt(qc_ref[48:72, 256:384], kc(t, j, 1))
        m1c = nt(qc_ref[72:h1, 0:128], kc(t, j, 0))
        m7c = nt(qc_ref[72:h1, 256:384], kc(t, j, 1))
        m1, m7, m6 = _cat0(_cat0(m1a, m1b), m1c), _cat0(_cat0(m7a, m7b), m7c), _cat0(m6a, m6b)
        c11 = s_ref[0:R1, c0:c0 + 128] + (m1 + m7)
        c22 = s_ref[R1:TQ, c0 + 128:c0 + 256] + (m1[0:R2] + m6)
        s_ref[0:R1, c0:c0 + 128] = c11
        s_ref[R1:TQ, c0 + 128:c0 + 256] = c22
        ml = jnp.maximum(_cat0(c11, c22), _cat0(s_ref[0:R1, c0 + 128:c0 + 256], s_ref[R1:TQ, c0:c0 + 128]))
        return max_update(ml, pos == 0, pos == NC - 1)

    def scores_chunk(t, j, pos):
        q = _upk(q_ref[0:TQ // 2, :])
        if (j + 1) * CK <= T:
            sj = lax.dot_general(q, xa_chunk(t, j), NT_DIMS, preferred_element_type=F32)
            sts = [sj[:, 0:128], sj[:, 128:256]]
        else:
            nrem = T - j * CK - 128
            assert 0 < nrem < 128 and nrem % 16 == 0
            kf = _upk(xa_ref[_ds(t.kb, j * CK // 2, 64, 16), :])
            sj = jnp.concatenate([lax.dot_general(q[0:R1], kf, NT_DIMS, preferred_element_type=F32),
                                  lax.dot_general(q[R1:TQ], kf, NT_DIMS, preferred_element_type=F32)], axis=0)
            kr = _upk(xa_ref[_ds(t.kb, j * CK // 2 + 64, nrem // 2, 16), :])
            st = lax.dot_general(kr, _upk(q_ref[...]), NT_DIMS, preferred_element_type=F32)
            st = jnp.concatenate([st, jnp.full((128 - nrem, st.shape[1]), -jnp.inf, F32)], axis=0)
            sts = [sj, st.T[0:TQ]]
        last[0] = sj[0:16, 0:128]
        s_ref[:, j * CK:j * CK + 128] = sts[0]
        s_ref[:, j * CK + 128:(j + 1) * CK] = sts[1]
        return max_update(jnp.maximum(sts[0], sts[1]), pos == 0, pos == NC - 1)

    def scores_fin(mpart):
        m = jnp.max(mpart, axis=-1, keepdims=True)
        lam = jnp.sum(jnp.exp2(mpart - m), axis=-1, keepdims=True)
        m = m + jnp.log(lam) * LOG2E
        mx_ref[0:TQ] = jnp.broadcast_to(m, (TQ, 128))

    def pv_group(t, js, first, r0=0, r1=R1, r2=R2):
        ra, rb, rc = r0, r0 + r1, r0 + r1 + r2
        W = {1: lambda j: kc(t, j, 0), 2: lambda j: k_alo(t, j), 3: lambda j: kc(t, j, 1), 4: lambda j: kc(t, j, 2),
             5: lambda j: k_bhi(t, j), 6: lambda j: kc(t, j, 3), 7: lambda j: kc(t, j, 4)}
        done = set()

        def blk(r, c, j):
            lo, hi = (ra, rb) if r == 1 else (rb, rc)
            c0 = j * CK + (c - 1) * 128
            if (r, c, j) in done:
                return s_ref[lo:hi, c0:c0 + 128]
            done.add((r, c, j))
            p = jnp.exp2(s_ref[lo:hi, c0:c0 + 128] - mx_ref[lo:hi])
            s_ref[lo:hi, c0:c0 + 128] = p
            return p

        def lhs_of(k, j):
            if k == 1:
                a11 = blk(1, 1, j)
                return _cat0(a11[0:r2] + blk(2, 2, j), a11[r2:])
            if k == 2:
                return blk(2, 1, j) + blk(2, 2, j)
            if k == 3:
                return blk(1, 1, j)
            if k == 4:
                return blk(2, 2, j)
            if k == 5:
                return blk(1, 1, j) + blk(1, 2, j)
            if k == 6:
                return blk(2, 1, j) - blk(1, 1, j)[0:r2]
            a12 = blk(1, 2, j)
            return _cat0(a12[0:r2] - blk(2, 2, j), a12[r2:])
        for i, k in enumerate(VSEQ):
            ls = [lhs_of(k, j) for j in js]
            if k in (2, 5):
                lo, hi = (ra, rb) if k == 5 else (rb, rc)
                lsum = (ls[0] + ls[1]) + (ls[2] + ls[3])
                if first:
                    lp_ref[lo:hi] = lsum
                else:
                    lp_ref[lo:hi] += lsum
            lhs = jnp.concatenate(ls, axis=1).astype(BF16)
            rhs = _upk(jnp.concatenate([W[k](j) for j in js], axis=0))
            mk = jnp.dot(lhs, rhs, preferred_element_type=F32)
            last[0] = mk[0:16]
            if i == 0:
                first_w[0] = mk[0:16]
            n = mk.shape[0]
            if first:
                acc7_ref[k, 0:n] = mk
            else:
                acc7_ref[k, 0:n] += mk

    def pv_fin(t, r0=0, r1=R1, r2=R2):
        l = jnp.sum(lp_ref[r0:r0 + r1 + r2], axis=-1, keepdims=True)
        m1, m3, m5, m7 = (acc7_ref[k, 0:r1] for k in (1, 3, 5, 7))
        m2, m4, m6 = (acc7_ref[k, 0:r2] for k in (2, 4, 6))
        c11 = m1 + (m7 - m5)
        c11 = _cat0(c11[0:r2] + m4, c11[r2:])
        c12 = m3 + m5
        c21 = m2 + m4
        c22 = (m1[0:r2] - m2) + (m3[0:r2] + m6)
        acc = jnp.concatenate([jnp.concatenate([c11, c12], axis=1), jnp.concatenate([c21, c22], axis=1)], axis=0)
        o = acc * (1.0 / l)
        glob = jnp.dot(o.astype(BF16), _upk(wvo_p[...]), preferred_element_type=F32)
        m_store(t, 0, glob, r0)

    def pv_chunk(t, j, r0, n):
        c0 = j * CK
        pa = jnp.exp2(s_ref[r0:r0 + n, c0:c0 + 128] - mx_ref[r0:r0 + n])
        pb = jnp.exp2(s_ref[r0:r0 + n, c0 + 128:c0 + 256] - mx_ref[r0:r0 + n])
        lloc = pa + pb
        pv = jnp.dot(jnp.concatenate([pa, pb], axis=-1).astype(BF16), xa_chunk(t, j), preferred_element_type=F32)
        last[0] = pv[0:16, 0:128]
        if j == 0:
            lp_ref[r0:r0 + n] = lloc
            acc_ref[r0:r0 + n] = pv
        else:
            lp_ref[r0:r0 + n] += lloc
            acc_ref[r0:r0 + n] += pv

    def pv_chunk_fin(t, r0, n):
        l = jnp.sum(lp_ref[r0:r0 + n], axis=-1, keepdims=True)
        o = (acc_ref[r0:r0 + n] * (1.0 / l)).astype(BF16)
        glob = jnp.dot(o, _upk(wvo_p[...]), preferred_element_type=F32)
        m_store(t, 0, glob, r0)

    def anchor(op):
        if op == 'Zx':
            zrow = pl.multiple_of(zoff[0], 16)
            x_buf[pl.ds(zrow + B * T + LAG + TP - T, 16), 0:128] = last[0].astype(BF16)
            return
        zrow = pl.multiple_of(zoff[0], 8)
        if op in ('Z', 'Zg'):
            (m_buf if op == 'Z' else g_buf)[0, pl.ds(zrow + NS * SLOT + 64, 8), :] = last[0][0:8]
        else:
            (lp_ref if op == 'Zl' else mx_ref)[pl.ds(zrow + TQ, 8), :] = last[0][0:8]

    def step(order, pb, pa, t0, tp, th=None, un=None, dma=None):
        cord, nxt = [], 0
        for op in order:
            if op == 'KK':
                cord += [nxt, nxt + 1]
                nxt += 2
            elif op in ('K1', 'K'):
                cord.append(NC - 2 if op == 'K1' else NC - 1)
        assert 4 * order.count('W') == NC and sorted(cord) == list(range(NC))
        mpart = None
        jv = jk = 0
        nq = []
        for op in order:
            if op == 'q':
                qproj(tp)
            elif op == 'W':
                pv_group(t0, cord[jv:jv + 4], jv == 0)
                jv += 4
            elif op == 'G':
                pv_fin(t0)
            elif op in ('K', 'K1'):
                assert jk < jv
                mpart = (scores_chunk if op == 'K' else scores_single)(tp, cord[jk], jk)
                jk += 1
            elif op == 'KK':
                assert jk + 1 < jv
                mpart = scores_pair(tp, cord[jk], cord[jk + 1], jk)
                jk += 2
            elif op[0] == 'Z':
                anchor(op)
            elif op == 'Ma':
                merge_loc(pa)
            elif op == 'Mb':
                merge_glob(pb)
            elif op == 'H':
                mlp_in(th)
            elif op == 'L':
                mlp_out(tp)
            elif op == 'n':
                r = (len(nq) // 2) * 256 + (len(nq) % 2) * 64
                xa_, xb_ = (_ln(x_buf[_ds(un * 512, LAG + T + r + o, 64, 16), :].astype(F32)) for o in (0, 128))
                v = jnp.concatenate(
                    [xa_, xb_] + _key_combos(xa_[:, 0:128], xa_[:, 128:256], xb_[:, 0:128], xb_[:, 128:256]), axis=1)
                nq.append((r, _pk(v.astype(BF16))))
            elif op == 'Ns':
                assert len(nq) == 4
                for r, v in nq:
                    xa_ref[_ds(un * 256, TP // 2 + r // 2, 32, 256), :] = v[:, 0:256]
                    xa_ref[_ds(un * 256, TP // 2 + r // 2 + 64, 32, 256), :] = v[:, 256:512]
                    kc_ref[_ds(un * 128, TP // 4 + (r // 256) * 64 + (r % 256) // 2, 32, 128), :] = v[:, 512:1152]
            elif op == 'D':
                dma()
            else:
                raise ValueError(op)
        scores_fin(mpart)

    done, nln = [], 0
    for op in PROLOGUE[split + 1:]:
        if op[0] == 's':
            dma_start(op)
        elif op[0] == 'x':
            x_copy(int(op[1:])).wait()
        elif op[0] == 'w':
            w_copy(int(op[1:])).wait()
        elif op[0] == 'n':
            ln_unit(int(op[1:]))
            nln = int(op[1:]) + 1
        elif op[0] == 'p':
            prep(int(op[1:]))
        elif op == 'A':
            prep_a()
        elif op == 'q':
            qproj(tile(0), False)
        elif op.startswith('KK'):
            j = int(op[2:])
            assert nln * 512 >= (j + 2) * CK
            mpart = scores_pair(tile(0), j, j + 1, len(done))
            done += [j, j + 1]
        elif op[0] in 'KJ':
            j = int(op[1:])
            assert nln * 512 >= (j + 1) * CK
            mpart = (scores_chunk if op[0] == 'K' else scores_single)(tile(0), j, len(done))
            done.append(j)
        elif op[0] == 'H':
            assert nln * 512 >= (int(op[1:]) + 1) * TQ
            mlp_in(tile(int(op[1:])))
        elif op == 'L0':
            mlp_out(tile(0))
        elif op[0] == 'Z':
            anchor(op)
        else:
            raise ValueError(op)
    assert sorted(done) == list(range(NC))
    scores_fin(mpart)

    def body_a(order, s, c):
        if 'Ns' in order:
            @pl.when(s == 1)
            def _():
                x_copy(NU + 1).wait()

        w = jnp.maximum(s - 1, 0)
        fb = w * TQ

        def dma():
            @pl.when(s > 0)
            def _():
                out_copy(fb, LAG, TQ - LAG).start()

            @pl.when(jnp.logical_and(s > 1, s != NT + 1))
            def _():
                out_copy(fb, 0, LAG).start()

        step(order, [(tile(w), 0, TQ, 0)], [(tile(s), 0, TQ, 0)], tile(s), tile(s + 1), tile(s + 3), s, dma)
        return c
    lax.fori_loop(0, NU, functools.partial(body_a, STEP_A1), 0)
    lax.fori_loop(NU, NS - 3, functools.partial(body_a, STEP_A2), 0)

    z = zoff[0]
    tail0 = (tile(NT - 1), TQ, LAG, TQ + LAG)
    Y2 = TQ + 3 * LAG

    def body_b(s, c):
        step(STEP_B, [(tile(s - 1), 0, TQ, 0)], [(tile(s), 0, TQ, 0), tail0], tile(s), tile(s + 1))
        out_copy((s - 1) * TQ, 0, TQ).start()
        return c
    lax.fori_loop(NS - 3, NS - 1, body_b, 0)

    def last_block(ops):
        tl = tile(z + (NS - 1))
        j = 0
        saved = None
        for op in ops:
            if op == 'WA':
                pv_group(tl, list(range(j, j + 4)), j == 0, 0, RA // 2, RA // 2)
                j += 4
            elif op == 'B':
                pv_chunk(tl, j, RA, TQ - RA)
                j += 1
            elif op == 'Ga':
                pv_fin(tl, 0, RA // 2, RA // 2)
            elif op == 'Gb':
                pv_chunk_fin(tl, RA, TQ - RA)
            elif op == 'E':
                last[0] = first_w[0]
            elif op == 'S':
                saved = last[0]
            elif op == 'R':
                last[0] = saved
            elif op[0] == 'Z':
                anchor(op)
            elif op == 'Mb':
                merge_glob([(tile(z + (NS - 2)), 0, TQ, 0), tail0])
                out_copy(0, (NS - 2) * TQ, TQ).start()
                out_copy(0, NT * TQ, LAG).start()
            elif op == 'Mc':
                merge_loc([(tl, 0, TQ + LAG, Y2)])
            elif op == 'M1':
                merge_glob([(tl, 0, RA, Y2)])
                out_copy(0, (NS - 1) * TQ, RA).start()
            elif op == 'M2':
                merge_glob([(tl, RA, TQ + LAG - RA, Y2 + RA)])
                out_copy(0, (NS - 1) * TQ + RA, TQ + LAG - RA).start()
            else:
                raise ValueError(op)
        assert j == NC

    pl.when(z < 1)(functools.partial(last_block, LAST_A))
    pl.when(z < 2)(functools.partial(last_block, LAST_B))

    out_copy(0, LAG, B * T).wait()


@jax.jit
def pallas_standalone__conformer_family_e_branchformer__speech_kernel(
    x: jax.Array,
    w_qkv: jax.Array,
    w_att_out: jax.Array,
    w_mlp_in: jax.Array,
    dw_csgu: jax.Array,
    w_mlp_out: jax.Array,
    dw_merge: jax.Array,
    w_merge: jax.Array,
):
    B, T, D = x.shape
    K = dw_csgu.shape[0]
    TP = (T + 511) // 512 * 512
    G = D // 128
    RB = (B * (T // TQ) + 1) * SLOT
    out = pl.pallas_call(
        functools.partial(_kernel, B=B, T=T, D=D, K=K, TP=TP),
        in_specs=[pl.BlockSpec(memory_space=pl.ANY)] * 8,
        out_specs=pl.BlockSpec(memory_space=pl.ANY),
        out_shape=jax.ShapeDtypeStruct((B * T, D), x.dtype),
        scratch_shapes=[
            pltpu.VMEM((B * T + 32 + TP - T, D), BF16),
            pltpu.VMEM((B * T + 32, D), BF16),
            pltpu.VMEM((B * TP // 2, D), U32),
            pltpu.VMEM((D // 2, D), U32),
            pltpu.VMEM((D // 2, D), U32),
            pltpu.VMEM((D // 2, 2 * D), U32),
            pltpu.VMEM((D // 2, D), U32),
            pltpu.VMEM((D, D), U32),
            pltpu.VMEM((64, 896), U32),
            pltpu.VMEM((3 * G, 48, 8, 128), F32),
            pltpu.VMEM((2 * G, RB, 128), F32),
            pltpu.VMEM((4 * G, RB, 128), F32),
            pltpu.VMEM((B * T, D), F32),
            pltpu.VMEM((TQ, TP), F32),
            pltpu.VMEM((TQ + 16, 128), F32),
            pltpu.VMEM((256, D), U32),
            pltpu.VMEM((128, 640), U32),
            pltpu.VMEM((B * TP // 4, 640), U32),
            pltpu.VMEM((TQ + 16, 128), F32),
            pltpu.VMEM((TQ + 16, 128), F32),
            pltpu.VMEM((TQ, D), F32),
            pltpu.VMEM((8, 224, 128), F32),
            pltpu.VMEM((2 * TQ + 4 * LAG, D), F32),
            pltpu.VMEM(w_qkv.shape, BF16),
            pltpu.VMEM(w_att_out.shape, BF16),
            pltpu.VMEM(w_mlp_in.shape, BF16),
            pltpu.VMEM(dw_csgu.shape, BF16),
            pltpu.VMEM(w_mlp_out.shape, BF16),
            pltpu.VMEM(dw_merge.shape, BF16),
            pltpu.VMEM(w_merge.shape, BF16),
            pltpu.SMEM((1,), jnp.int32),
            pltpu.SemaphoreType.DMA((max(GRP.values()) + 1,)),
            pltpu.SemaphoreType.DMA,
        ],
        compiler_params=pltpu.CompilerParams(vmem_limit_bytes=120 * 1024 * 1024, disable_bounds_checks=True),
    )(x.reshape(B * T, D), w_qkv, w_att_out, w_mlp_in, dw_csgu, w_mlp_out, dw_merge, w_merge)
    return out.reshape(B, T, D)
```
